```python
import jax
import jax.numpy as jnp

def _softmax(x, axis=-1):
    return jax.nn.softmax(x, axis=axis)
def _gelu(x):
    return jax.nn.gelu(x, approximate=True)
def _silu(x):
    return jax.nn.silu(x)
def _sigmoid(x):
    return jax.nn.sigmoid(x)
def _layernorm(x, axis=-1, eps=1e-5):
    m = jnp.mean(x, axis=axis, keepdims=True)
    v = jnp.var(x, axis=axis, keepdims=True)
    return (x - m) / jnp.sqrt(v + eps)
def _scatter_add(tgt, idx, src, axis=0):
    return tgt.at[idx].add(src)
def _segment_sum(src, seg, n):
    return jax.ops.segment_sum(src, seg, n)
class _Rng:
    def __init__(self, key):
        self._k = key
    def _next(self):
        self._k, sub = jax.random.split(self._k)
        return sub
    def normal(self, shape):
        return jax.random.normal(self._next(), shape, dtype=jnp.bfloat16)
    def randint(self, lo, hi, shape):
        return jax.random.randint(self._next(), shape, lo, hi, dtype=jnp.int32)
    def uniform(self, shape, lo=0.0, hi=1.0):
        return jax.random.uniform(self._next(), shape, jnp.bfloat16, lo, hi)
    def permutation(self, n):
        return jax.random.permutation(self._next(), n)


kernel_name = 'interleave_layers__sliding_local_dilated__softmax_full_mha__prompt'

def setup_inputs():
    _rng = _Rng(jax.random.key(int.from_bytes(__import__("os").urandom(4), "little")))
    _w = (lambda a: (lambda t: t.astype(jnp.bfloat16) if jnp.issubdtype(t.dtype, jnp.floating) else t)(jnp.asarray(a)))
    def _A_setup():
        B, S, D = 1, 2048, 1024
        return {
            "x": _w((lambda *s: _rng.normal(s) * 0.05)(B, S, D)),
            "wqkv": _w((lambda *s: _rng.normal(s) * 0.05)(D, 3 * D)),
            "wo": _w((lambda *s: _rng.normal(s) * 0.05)(D, D)),
        }
    _A_in = _A_setup()

    def _B_setup():
        B, S, D = 1, 2048, 1024
        return {
            "x": _w((lambda *s: _rng.normal(s) * 0.05)(B, S, D)),
            "wqkv": _w((lambda *s: _rng.normal(s) * 0.05)(D, 3 * D)),
            "wo": _w((lambda *s: _rng.normal(s) * 0.05)(D, D)),
        }
    _B_in = _B_setup()

    return {
        "A_x": _A_in["x"],
        "A_wqkv": _A_in["wqkv"],
        "A_wo": _A_in["wo"],
        "B_x": _B_in["x"],
        "B_wqkv": _B_in["wqkv"],
        "B_wo": _B_in["wo"],
    }

def reference(A_x, A_wqkv, A_wo, B_x, B_wqkv, B_wo):
    def _A_ref(x, wqkv, wo):
        B, S, D = x.shape
        H = 32; Dh = D // H
        W, dil = 8, 2
        qkv = (lambda x, *d: x.transpose(*d))((x @ wqkv).reshape(B, S, 3, H, Dh), 2, 0, 3, 1, 4)
        q, k, v = qkv[0], qkv[1], qkv[2]
        scale = Dh ** -0.5
        pos = jnp.arange(S)
        off = jnp.arange(W) * dil
        idx = pos[:, None] - off[None, :]
        mask = idx >= 0
        idx_c = jnp.where(mask, idx, 0).reshape(-1)
        kg = k[:, :, idx_c, :].reshape(B, H, S, W, Dh)
        vg = v[:, :, idx_c, :].reshape(B, H, S, W, Dh)
        logits = jnp.einsum("bhsd,bhswd->bhsw", q, kg) * scale
        logits = jnp.where(mask[None, None, :, :], logits, -1e9)
        attn = _softmax(logits, axis=-1)
        o = jnp.einsum("bhsw,bhswd->bhsd", attn, vg)
        return (lambda x, *d: x.transpose(*d))(o, 0, 2, 1, 3).reshape(B, S, D) @ wo

    def _B_ref(x, wqkv, wo):
        B, S, D = x.shape
        H = 32; Dh = D // H
        qkv = (lambda x, *d: x.transpose(*d))((x @ wqkv).reshape(B, S, 3, H, Dh), 2, 0, 3, 1, 4)
        q, k, v = qkv[0], qkv[1], qkv[2]
        scale = Dh ** -0.5
        scores = jnp.einsum("bhqd,bhkd->bhqk", q, k) * scale
        p = _softmax(scores, axis=-1)
        o = jnp.einsum("bhqk,bhkd->bhqd", p, v)
        return (lambda x, *d: x.transpose(*d))(o, 0, 2, 1, 3).reshape(B, S, D) @ wo

    x = A_x
    x = x + _A_ref(_layernorm(x, axis=-1), A_wqkv, A_wo)
    x = x + _B_ref(_layernorm(x, axis=-1), B_wqkv, B_wo)
    x = x + _A_ref(_layernorm(x, axis=-1), A_wqkv, A_wo)
    x = x + _B_ref(_layernorm(x, axis=-1), B_wqkv, B_wo)
    return x
```

```python
import functools
import math

import jax
import jax.numpy as jnp
from jax import lax
import jax.experimental.pallas as pl
import jax.experimental.pallas.tpu as pltpu

S = 2048
D = 1024
H = 32
DH = D // H
NT = D // 128
HPT = 128 // DH
WIN = 8
DIL = 2
HALO = 16
EPS = 1e-5
LOG2E = math.log2(math.e)
QSCALE = (DH ** -0.5) * LOG2E
MASKED = -1e9 * LOG2E

BM = 256
CM = 128
RG = 16
KC = 256
FQ = 256

L_LO = 2.0 ** -40
L_HI = 2.0 ** 90
O_HI = 3.0e38

F32 = jnp.float32
BF16 = jnp.bfloat16


def _layernorm(x):
    mu = jnp.mean(x, axis=-1, keepdims=True)
    xc = x - mu
    var = jnp.mean(xc * xc, axis=-1, keepdims=True)
    return xc * lax.rsqrt(var + EPS)


def _permute_cols(w32):
    rows = w32.shape[0]
    lane = lax.broadcasted_iota(jnp.int32, (rows, 128), 1)
    tiles = [w32[:, t * 128:(t + 1) * 128] for t in range(NT)]
    for b in range(3):
        sh = 4 << b
        low = (lane & sh) == 0
        for a in range(NT):
            if a & (1 << b):
                continue
            c = a | (1 << b)
            ta, tc = tiles[a], tiles[c]
            tiles[a] = jnp.where(low, ta, pltpu.roll(tc, sh, 1))
            tiles[c] = jnp.where(low, pltpu.roll(ta, 128 - sh, 1), tc)
    return jnp.concatenate(tiles, axis=1)


def _permute_rows(w_ref, c0, ncols):
    w32 = pltpu.bitcast(w_ref[:, pl.ds(c0, ncols)], jnp.uint32)
    nv = D // 16
    v = [w32[i * 8:(i + 1) * 8, :] for i in range(nv)]
    sub = lax.broadcasted_iota(jnp.int32, (8, ncols), 0)
    for vb, sh in ((8, 2), (16, 4)):
        low = (sub & sh) == 0
        for a in range(nv):
            if a & vb:
                continue
            c = a | vb
            ta, tc = v[a], v[c]
            v[a] = jnp.where(low, ta, pltpu.roll(tc, sh, 0))
            v[c] = jnp.where(low, pltpu.roll(ta, 8 - sh, 0), tc)
    def src(i):
        b0, b5 = i & 1, (i >> 5) & 1
        return (i & ~33) | (b0 << 5) | b5
    out = jnp.concatenate([v[src(i)] for i in range(nv)], axis=0)
    w_ref[:, pl.ds(c0, ncols)] = pltpu.bitcast(out, BF16)


def _group_sum4(x, lane):
    b0 = (lane & 1) == 0
    x = x + jnp.where(b0, pltpu.roll(x, 127, 1), pltpu.roll(x, 1, 1))
    b1 = (lane & 2) == 0
    return x + jnp.where(b1, pltpu.roll(x, 126, 1), pltpu.roll(x, 2, 1))


def _kernel(x_hbm, wa_hbm, woa_hbm, wb_hbm, wob_hbm, out_hbm,
            xin, xres, wa, woa, wb, wob, kbuf, vbuf, qs, ks, vt, ot, obuf,
            sems, osems):
    nblk = S // BM
    nch = BM // CM

    copies = [
        pltpu.make_async_copy(wa_hbm, wa, sems.at[0]),
        pltpu.make_async_copy(x_hbm, xin, sems.at[1]),
        pltpu.make_async_copy(woa_hbm, woa, sems.at[2]),
        pltpu.make_async_copy(wb_hbm, wb, sems.at[3]),
        pltpu.make_async_copy(wob_hbm, wob, sems.at[4]),
    ]
    for cp in copies:
        cp.start()

    kbuf[...] = jnp.zeros(kbuf.shape, F32)
    vbuf[...] = jnp.zeros(vbuf.shape, F32)

    copies[0].wait()
    pr = 64

    def perm_body(i, c):
        r = pl.multiple_of(i * pr, pr)
        for sec in range(3):
            w32 = pltpu.bitcast(wa[pl.ds(r, pr), sec * D:(sec + 1) * D], jnp.uint32)
            wa[pl.ds(r, pr), sec * D:(sec + 1) * D] = pltpu.bitcast(_permute_cols(w32), BF16)
        return c

    lax.fori_loop(0, D // pr, perm_body, 0)

    copies[2].wait()

    def permo_body(i, c):
        _permute_rows(woa, pl.multiple_of(i * 128, 128), 128)
        return c

    lax.fori_loop(0, NT, permo_body, 0)
    copies[1].wait()
    copies[3].wait()
    copies[4].wait()

    lane = lax.broadcasted_iota(jnp.int32, (RG, 128), 1)
    rowi = lax.broadcasted_iota(jnp.int32, (RG, 128), 0)

    def local_qkv(h, off, i):
        qkv = jnp.dot(h, wa[...], preferred_element_type=F32)
        for t in range(NT):
            kbuf[t, HALO + off:HALO + off + CM, :] = qkv[:, D + t * 128:D + (t + 1) * 128]
            v_t = qkv[:, 2 * D + t * 128:2 * D + (t + 1) * 128]
            vbuf[t, HALO + off:HALO + off + CM, :] = v_t
            if off == 0:
                first = jnp.broadcast_to(v_t[0:1, :], (HALO, 128))
                vbuf[t, 0:HALO, :] = jnp.where(i == 0, first, vbuf[t, 0:HALO, :])
        return qkv[:, 0:D]

    def local_attn(q, off, i):
        outs = []
        for g in range(CM // RG):
            base = HALO + off + g * RG
            qg = [q[g * RG:(g + 1) * RG, t * 128:(t + 1) * 128] for t in range(NT)]
            logit = []
            for w in range(WIN):
                a = base - DIL * w
                part = qg[0] * kbuf[0, a:a + RG, :]
                for t in range(1, NT):
                    part = part + qg[t] * kbuf[t, a:a + RG, :]
                lg = _group_sum4(part, lane) * QSCALE
                if off == 0 and g == 0 and w > 0:
                    lg = jnp.where(rowi + i * BM >= DIL * w, lg, MASKED)
                logit.append(lg)
            m = functools.reduce(jnp.maximum, logit)
            p = [jnp.exp2(lg - m) for lg in logit]
            inv = 1.0 / functools.reduce(lambda u, v: u + v, p)
            og = []
            for t in range(NT):
                acc = p[0] * vbuf[t, base:base + RG, :]
                for w in range(1, WIN):
                    a = base - DIL * w
                    acc = acc + p[w] * vbuf[t, a:a + RG, :]
                og.append((acc * inv).astype(BF16))
            outs.append(jnp.concatenate(og, axis=1))
        return jnp.concatenate(outs, axis=0)

    def full_qkv(h, r):
        qkv = jnp.dot(h, wb[...], preferred_element_type=F32)
        for t in range(NT):
            qs[t, pl.ds(r, CM), :] = (qkv[:, t * 128:(t + 1) * 128] * QSCALE).astype(BF16)
            ks[t, pl.ds(r, CM), :] = qkv[:, D + t * 128:D + (t + 1) * 128].astype(BF16)
        vt[:, pl.ds(r, CM)] = qkv[:, 2 * D:3 * D].T.astype(BF16)

    def full_oproj(r):
        o = ot[:, pl.ds(r, CM)].T.astype(BF16)
        return xres[pl.ds(r, CM), :] + jnp.dot(o, wob[...], preferred_element_type=F32)

    def row_phase(first):
        def body(i, c):
            r0 = pl.multiple_of(i * BM, BM)
            rs = [pl.multiple_of(r0 + ch * CM, CM) for ch in range(nch)]
            for t in range(NT):
                kbuf[t, 0:HALO, :] = kbuf[t, BM:BM + HALO, :]
                vbuf[t, 0:HALO, :] = vbuf[t, BM:BM + HALO, :]
            if first:
                xs = [xin[pl.ds(r, CM), :].astype(F32) for r in rs]
            else:
                xs = [full_oproj(r) for r in rs]
            qv = [local_qkv(_layernorm(xs[ch]).astype(BF16), ch * CM, i) for ch in range(nch)]
            for ch in range(nch):
                o = local_attn(qv[ch], ch * CM, i)
                xs[ch] = xs[ch] + jnp.dot(o, woa[...], preferred_element_type=F32)
                xres[pl.ds(rs[ch], CM), :] = xs[ch]
            for ch in range(nch):
                full_qkv(_layernorm(xs[ch]).astype(BF16), rs[ch])
            return c

        lax.fori_loop(0, nblk, body, 0)

    nt_dims = (((1,), (1,)), ((), ()))

    def masked_q(q, hp):
        q32 = pltpu.bitcast(q, jnp.uint32)
        head = lax.broadcasted_iota(jnp.int32, q32.shape, 1) // DH
        return pltpu.bitcast(jnp.where(head == hp, q32, jnp.uint32(0)), BF16)

    def full_attn():
        def body(g, bad):
            for hp in range(HPT):
                w = masked_q(qs[g], hp)
                r0 = pl.multiple_of(g * 128 + hp * DH, DH)
                acc = jnp.zeros((DH, S), F32)
                l8 = jnp.zeros((8, S), F32)
                for t in range(S // KC):
                    s = lax.dot_general(ks[g, t * KC:(t + 1) * KC, :], w, nt_dims,
                                        preferred_element_type=F32)
                    p = jnp.exp2(s)
                    l8 = l8 + jnp.sum(p.reshape(KC // 8, 8, S), axis=0)
                    acc = acc + jnp.dot(vt[pl.ds(r0, DH), t * KC:(t + 1) * KC], p.astype(BF16),
                                        preferred_element_type=F32)
                l = jnp.sum(l8, axis=0, keepdims=True)
                o = acc * (1.0 / l)
                ot[pl.ds(r0, DH), :] = o
                ok = (jnp.abs(o) < O_HI) & (l > L_LO) & (l < L_HI)
                nbad = jnp.where(ok, 0.0, 1.0)
                bad = jnp.maximum(bad, jnp.max(nbad.reshape(DH // 8, 8, S), axis=0))
            return bad

        bad = lax.fori_loop(0, NT, body, jnp.zeros((8, S), F32))

        @pl.when(jnp.max(bad) > 0.0)
        def _():
            nq = S // FQ

            def fb_body(it, c):
                hd = it // nq
                g = hd // HPT
                q0 = pl.multiple_of((it % nq) * FQ, FQ)
                r0 = pl.multiple_of(hd * DH, DH)
                w = masked_q(qs[g, pl.ds(q0, FQ), :], hd % HPT)
                s = lax.dot_general(ks[g], w, nt_dims, preferred_element_type=F32)
                p = jnp.exp2(s - jnp.max(s, axis=0, keepdims=True))
                l = jnp.sum(p, axis=0, keepdims=True)
                acc = jnp.dot(vt[pl.ds(r0, DH), :], p.astype(BF16), preferred_element_type=F32)
                ot[pl.ds(r0, DH), pl.ds(q0, FQ)] = acc * (1.0 / l)
                return c

            lax.fori_loop(0, H * nq, fb_body, 0)

    def pair_body(pair, c):
        @pl.when(pair == 0)
        def _():
            row_phase(True)

        @pl.when(pair == 1)
        def _():
            row_phase(False)

        full_attn()
        return c

    lax.fori_loop(0, 2, pair_body, 0)

    def out_copy(i):
        r0 = pl.multiple_of(i * BM, BM)
        return pltpu.make_async_copy(obuf.at[pl.ds(r0, BM), :], out_hbm.at[pl.ds(r0, BM), :],
                                     osems.at[i])

    def out_body(i, c):
        r0 = pl.multiple_of(i * BM, BM)
        for ch in range(nch):
            r = pl.multiple_of(r0 + ch * CM, CM)
            obuf[pl.ds(r, CM), :] = full_oproj(r).astype(BF16)
        out_copy(i).start()
        return c

    lax.fori_loop(0, nblk, out_body, 0)
    for i in range(nblk):
        out_copy(i).wait()


@jax.jit
def pallas_interleave_layers__sliding_local_dilated__softmax_full_mha__prompt_kernel(
    A_x: jax.Array,
    A_wqkv: jax.Array,
    A_wo: jax.Array,
    B_x: jax.Array,
    B_wqkv: jax.Array,
    B_wo: jax.Array,
):
    del B_x
    x = A_x.reshape(S, D)
    hbm = pl.BlockSpec(memory_space=pl.ANY)
    out = pl.pallas_call(
        _kernel,
        out_shape=jax.ShapeDtypeStruct((S, D), BF16),
        in_specs=[hbm] * 5,
        out_specs=hbm,
        scratch_shapes=[
            pltpu.VMEM((S, D), BF16),
            pltpu.VMEM((S, D), F32),
            pltpu.VMEM((D, 3 * D), BF16),
            pltpu.VMEM((D, D), BF16),
            pltpu.VMEM((D, 3 * D), BF16),
            pltpu.VMEM((D, D), BF16),
            pltpu.VMEM((NT, HALO + BM, 128), F32),
            pltpu.VMEM((NT, HALO + BM, 128), F32),
            pltpu.VMEM((NT, S, 128), BF16),
            pltpu.VMEM((NT, S, 128), BF16),
            pltpu.VMEM((D, S), BF16),
            pltpu.VMEM((D, S), F32),
            pltpu.VMEM((S, D), BF16),
            pltpu.SemaphoreType.DMA((5,)),
            pltpu.SemaphoreType.DMA((S // BM,)),
        ],
        compiler_params=pltpu.CompilerParams(vmem_limit_bytes=110 * 1024 * 1024),
        name="interleaved_attention_stack",
    )(x, A_wqkv, A_wo, B_wqkv, B_wo)
    return out.reshape(1, S, D)
```

```python
import functools
import math

import jax
import jax.numpy as jnp
from jax import lax
import jax.experimental.pallas as pl
import jax.experimental.pallas.tpu as pltpu

S = 2048
D = 1024
H = 32
DH = D // H
NT = D // 128
HPT = 128 // DH
WIN = 8
DIL = 2
HALO = 16
EPS = 1e-5
LOG2E = math.log2(math.e)
QSCALE = (DH ** -0.5) * LOG2E
MASKED = -1e9 * LOG2E

BM = 256
CM = 128
RG = 16
KC = 512
QB = 1024
OS = 128
FQ = 128

L_LO = 2.0 ** -40
L_HI = 2.0 ** 90
O_HI = 3.0e38

F32 = jnp.float32
BF16 = jnp.bfloat16
U32 = jnp.uint32


def _layernorm(x):
    mu = jnp.mean(x, axis=-1, keepdims=True)
    xc = x - mu
    var = jnp.mean(xc * xc, axis=-1, keepdims=True)
    return xc * lax.rsqrt(var + EPS)


def _permute_cols(w32):
    rows = w32.shape[0]
    lane = lax.broadcasted_iota(jnp.int32, (rows, 128), 1)
    tiles = [w32[:, t * 128:(t + 1) * 128] for t in range(NT)]
    for b in range(3):
        sh = 4 << b
        low = (lane & sh) == 0
        for a in range(NT):
            if a & (1 << b):
                continue
            c = a | (1 << b)
            ta, tc = tiles[a], tiles[c]
            tiles[a] = jnp.where(low, ta, pltpu.roll(tc, sh, 1))
            tiles[c] = jnp.where(low, pltpu.roll(ta, 128 - sh, 1), tc)
    return jnp.concatenate(tiles, axis=1)


def _permute_rows(w32):
    ncols = w32.shape[1]
    nv = D // 16
    v = [w32[i * 8:(i + 1) * 8, :] for i in range(nv)]
    sub = lax.broadcasted_iota(jnp.int32, (8, ncols), 0)
    for vb, sh in ((8, 2), (16, 4)):
        low = (sub & sh) == 0
        for a in range(nv):
            if a & vb:
                continue
            c = a | vb
            ta, tc = v[a], v[c]
            v[a] = jnp.where(low, ta, pltpu.roll(tc, sh, 0))
            v[c] = jnp.where(low, pltpu.roll(ta, 8 - sh, 0), tc)
    def src(i):
        b0, b5 = i & 1, (i >> 5) & 1
        return (i & ~33) | (b0 << 5) | b5
    return jnp.concatenate([v[src(i)] for i in range(nv)], axis=0)


def _group_sum4(x, lane):
    b0 = (lane & 1) == 0
    x = x + jnp.where(b0, pltpu.roll(x, 127, 1), pltpu.roll(x, 1, 1))
    b1 = (lane & 2) == 0
    return x + jnp.where(b1, pltpu.roll(x, 126, 1), pltpu.roll(x, 2, 1))


def _pack(x):
    return pltpu.bitcast(x.astype(BF16), U32)


def _unpack(x):
    return pltpu.bitcast(x, BF16)


def _kernel(x_hbm, wa_hbm, woa_hbm, wb_hbm, wob_hbm, out_hbm,
            xio, xres, xsave, wst, wost, wst2, wost2, wa, woa, wb, wob, hnext, kbuf, vbuf,
            qs, ks, vt, ots, sems, osems):
    nblk = S // BM
    nch = BM // CM
    nwc = 4
    wr = D // nwc

    def wcopy(src, dst, c, k):
        return pltpu.make_async_copy(src.at[pl.ds(c * wr, wr), :], dst.at[pl.ds(c * wr, wr), :],
                                     sems.at[k])

    cp_wa = [wcopy(wa_hbm, wst, c, c) for c in range(nwc)]
    cp_wb = [wcopy(wb_hbm, wst2, c, nwc + c) for c in range(nwc)]
    cp_x = pltpu.make_async_copy(x_hbm, xio, sems.at[2 * nwc])
    cp_woa = pltpu.make_async_copy(woa_hbm, wost, sems.at[2 * nwc + 1])
    cp_wob = pltpu.make_async_copy(wob_hbm, wost2, sems.at[2 * nwc + 2])
    for cp in cp_wa + [cp_x, cp_woa] + cp_wb + [cp_wob]:
        cp.start()

    kbuf[...] = jnp.zeros(kbuf.shape, F32)
    vbuf[...] = jnp.zeros(vbuf.shape, F32)

    pr = 128

    with jax.named_scope("perm_cols"):
        for c in range(nwc):
            cp_wa[c].wait()

            def perm_body(i, carry, c=c):
                r = pl.multiple_of(c * wr + (i // 3) * pr, pr)
                c0 = pl.multiple_of((i % 3) * D, D)
                w32 = _pack(wst[pl.ds(r, pr), pl.ds(c0, D)])
                wa[pl.ds(pl.multiple_of(r // 2, pr // 2), pr // 2), pl.ds(c0, D)] = _permute_cols(w32)
                return carry

            lax.fori_loop(0, 3 * wr // pr, perm_body, 0)

    with jax.named_scope("x_in"):
        cp_x.wait()

        def xin_body(i, carry):
            r = pl.multiple_of(i * 64, 64)
            xres[pl.ds(r, 64), :] = xio[pl.ds(r, 64), :].astype(F32)
            return carry

        lax.fori_loop(0, S // 64, xin_body, 0)

    with jax.named_scope("perm_rows"):
        cp_woa.wait()

        def permo_body(i, carry):
            c0 = pl.multiple_of(i * 128, 128)
            woa[:, pl.ds(c0, 128)] = _permute_rows(_pack(wost[:, pl.ds(c0, 128)]))
            return carry

        lax.fori_loop(0, NT, permo_body, 0)

    def repack(src, dst, r0, nrows):
        step = 32

        def body(i, carry):
            r = pl.multiple_of(r0 + i * step, step)
            dst[pl.ds(pl.multiple_of(r // 2, step // 2), step // 2), :] = _pack(src[pl.ds(r, step), :])
            return carry

        lax.fori_loop(0, nrows // step, body, 0)

    with jax.named_scope("repack"):
        for c in range(nwc):
            cp_wb[c].wait()
            repack(wst2, wb, c * wr, wr)
        cp_wob.wait()
        repack(wost2, wob, 0, D)

    lane = lax.broadcasted_iota(jnp.int32, (RG, 128), 1)
    rowi = lax.broadcasted_iota(jnp.int32, (RG, 128), 0)

    def local_qkv(h, off, i):
        qkv = jnp.dot(h, _unpack(wa[...]), preferred_element_type=F32)
        for t in range(NT):
            kbuf[t, HALO + off:HALO + off + CM, :] = qkv[:, D + t * 128:D + (t + 1) * 128]
            v_t = qkv[:, 2 * D + t * 128:2 * D + (t + 1) * 128]
            vbuf[t, HALO + off:HALO + off + CM, :] = v_t
            if off == 0:
                first = jnp.broadcast_to(v_t[0:1, :], (HALO, 128))
                vbuf[t, 0:HALO, :] = jnp.where(i == 0, first, vbuf[t, 0:HALO, :])
        return qkv[:, 0:D]

    def local_attn(q, off, i):
        outs = []
        for g in range(CM // RG):
            base = HALO + off + g * RG
            qg = [q[g * RG:(g + 1) * RG, t * 128:(t + 1) * 128] for t in range(NT)]
            logit = []
            for w in range(WIN):
                a = base - DIL * w
                part = qg[0] * kbuf[0, a:a + RG, :]
                for t in range(1, NT):
                    part = part + qg[t] * kbuf[t, a:a + RG, :]
                lg = _group_sum4(part, lane) * QSCALE
                if off == 0 and g == 0 and w > 0:
                    lg = jnp.where(rowi + i * BM >= DIL * w, lg, MASKED)
                logit.append(lg)
            m = functools.reduce(jnp.maximum, logit)
            p = [jnp.exp2(lg - m) for lg in logit]
            inv = 1.0 / functools.reduce(lambda u, v: u + v, p)
            og = []
            for t in range(NT):
                acc = p[0] * vbuf[t, base:base + RG, :]
                for w in range(1, WIN):
                    a = base - DIL * w
                    acc = acc + p[w] * vbuf[t, a:a + RG, :]
                og.append((acc * inv).astype(BF16))
            outs.append(jnp.concatenate(og, axis=1))
        return jnp.concatenate(outs, axis=0)

    def full_qkv(h, r):
        r2 = pl.multiple_of(r // 2, CM // 2)
        v = jnp.dot(h, _unpack(wb[:, 2 * D:3 * D]), preferred_element_type=F32)
        vt[:, pl.ds(r, CM)] = _pack(v.T)
        qk = jnp.dot(h, _unpack(wb[:, 0:2 * D]), preferred_element_type=F32)
        for t in range(NT):
            qs[t, pl.ds(r2, CM // 2), :] = _pack(qk[:, t * 128:(t + 1) * 128] * QSCALE)
            ks[t, pl.ds(r2, CM // 2), :] = _pack(qk[:, D + t * 128:D + (t + 1) * 128])

    def row_phase():
        hnext[...] = _pack(_layernorm(xres[0:CM, :]))

        def body(i, c):
            r0 = pl.multiple_of(i * BM, BM)
            rs = [pl.multiple_of(r0 + ch * CM, CM) for ch in range(nch)]
            for t in range(NT):
                kbuf[t, 0:HALO, :] = kbuf[t, BM:BM + HALO, :]
                vbuf[t, 0:HALO, :] = vbuf[t, BM:BM + HALO, :]
            qv = [local_qkv(_unpack(hnext[...]), 0, i)]
            for ch in range(1, nch):
                h = _layernorm(xres[pl.ds(rs[ch], CM), :]).astype(BF16)
                qv.append(local_qkv(h, ch * CM, i))
            xs = []
            for ch in range(nch):
                o = local_attn(qv[ch], ch * CM, i)
                x2 = xres[pl.ds(rs[ch], CM), :] + jnp.dot(o, _unpack(woa[...]),
                                                          preferred_element_type=F32)
                xres[pl.ds(rs[ch], CM), :] = x2
                xsave[pl.ds(rs[ch], CM), :] = x2
                xs.append(x2)
            rn = pl.multiple_of(jnp.minimum(i + 1, nblk - 1) * BM, BM)
            for ch in range(nch):
                h2 = _layernorm(xs[ch]).astype(BF16)
                if ch == nch - 1:
                    hnext[...] = _pack(_layernorm(xres[pl.ds(rn, CM), :]))
                full_qkv(h2, rs[ch])
            return c

        with jax.named_scope("row_phase"):
            lax.fori_loop(0, nblk, body, 0)

    nt_dims = (((1,), (1,)), ((), ()))

    def masked_q(q32, hp):
        head = lax.broadcasted_iota(jnp.int32, q32.shape, 1) // DH
        return _unpack(jnp.where(head == hp, q32, jnp.uint32(0)))

    def add_oproj(ot, g, q0, nq):
        g64 = pl.multiple_of(g * 64, 64)
        for j in range(nq // OS):
            y = jnp.dot(ot[:, j * OS:(j + 1) * OS].T.astype(BF16), _unpack(wob[pl.ds(g64, 64), :]),
                        preferred_element_type=F32)
            r = pl.multiple_of(q0 + j * OS, OS)
            xres[pl.ds(r, OS), :] = xres[pl.ds(r, OS), :] + y

    def full_attn():
        nqb = S // QB

        def body(it, bad):
            g = it // nqb
            q0 = pl.multiple_of((it % nqb) * QB, QB)
            q32 = qs[g, pl.ds(pl.multiple_of(q0 // 2, QB // 2), QB // 2), :]
            outs = []
            for hp in range(HPT):
                w = masked_q(q32, hp)
                r0 = pl.multiple_of(g * 64 + hp * (DH // 2), DH // 2)
                acc = jnp.zeros((DH, QB), F32)
                l8 = jnp.zeros((8, QB), F32)
                for t in range(S // KC):
                    kc = _unpack(ks[g, t * KC // 2:(t + 1) * KC // 2, :])
                    s = lax.dot_general(kc, w, nt_dims, preferred_element_type=F32)
                    p = jnp.exp2(s)
                    l8 = l8 + jnp.sum(p.reshape(KC // 8, 8, QB), axis=0)
                    vc = _unpack(vt[pl.ds(r0, DH // 2), t * KC:(t + 1) * KC])
                    acc = acc + jnp.dot(vc, p.astype(BF16), preferred_element_type=F32)
                l = jnp.sum(l8, axis=0, keepdims=True)
                o = acc * (1.0 / l)
                outs.append(o)
                ok = (jnp.abs(o) < O_HI) & (l > L_LO) & (l < L_HI)
                nbad = jnp.where(ok, 0.0, 1.0)
                bad = jnp.maximum(bad, jnp.max(nbad.reshape(DH // 8, 8, QB), axis=0))
            add_oproj(jnp.concatenate(outs, axis=0), g, q0, QB)
            return bad

        with jax.named_scope("full_attn"):
            bad = lax.fori_loop(0, NT * nqb, body, jnp.zeros((8, QB), F32))

        @pl.when(jnp.max(bad) > 0.0)
        def _():
            nq = S // FQ

            def restore(i, c):
                r = pl.multiple_of(i * 32, 32)
                xres[pl.ds(r, 32), :] = xsave[pl.ds(r, 32), :]
                return c

            lax.fori_loop(0, S // 32, restore, 0)

            def fb_body(it, c):
                g = it // nq
                q0 = pl.multiple_of((it % nq) * FQ, FQ)
                q32 = qs[g, pl.ds(pl.multiple_of(q0 // 2, FQ // 2), FQ // 2), :]

                def head_body(hp, c2):
                    r0 = pl.multiple_of(g * 64 + hp * (DH // 2), DH // 2)
                    s = lax.dot_general(_unpack(ks[g]), masked_q(q32, hp), nt_dims,
                                        preferred_element_type=F32)
                    p = jnp.exp2(s - jnp.max(s, axis=0, keepdims=True))
                    l = jnp.sum(p, axis=0, keepdims=True)
                    acc = jnp.dot(_unpack(vt[pl.ds(r0, DH // 2), :]), p.astype(BF16),
                                  preferred_element_type=F32)
                    ots[pl.ds(pl.multiple_of(hp * DH, DH), DH), :] = acc * (1.0 / l)
                    return c2

                lax.fori_loop(0, HPT, head_body, 0)
                add_oproj(ots[...], g, q0, FQ)
                return c

            lax.fori_loop(0, NT * nq, fb_body, 0)

    def pair_body(pair, c):
        row_phase()
        full_attn()
        return c

    with jax.named_scope("pairs"):
        lax.fori_loop(0, 2, pair_body, 0)

    def out_copy(i):
        r0 = pl.multiple_of(i * BM, BM)
        return pltpu.make_async_copy(xio.at[pl.ds(r0, BM), :], out_hbm.at[pl.ds(r0, BM), :],
                                     osems.at[i])

    def out_body(i, c):
        r0 = pl.multiple_of(i * BM, BM)
        xio[pl.ds(r0, BM), :] = xres[pl.ds(r0, BM), :].astype(BF16)
        out_copy(i).start()
        return c

    with jax.named_scope("out_phase"):
        lax.fori_loop(0, nblk, out_body, 0)
        for i in range(nblk):
            out_copy(i).wait()


@jax.jit
def pallas_interleave_layers__sliding_local_dilated__softmax_full_mha__prompt_kernel(
    A_x: jax.Array,
    A_wqkv: jax.Array,
    A_wo: jax.Array,
    B_x: jax.Array,
    B_wqkv: jax.Array,
    B_wo: jax.Array,
):
    del B_x
    x = A_x.reshape(S, D)
    hbm = pl.BlockSpec(memory_space=pl.ANY)
    out = pl.pallas_call(
        _kernel,
        out_shape=jax.ShapeDtypeStruct((S, D), BF16),
        in_specs=[hbm] * 5,
        out_specs=hbm,
        scratch_shapes=[
            pltpu.VMEM((S, D), BF16),
            pltpu.VMEM((S, D), F32),
            pltpu.VMEM((S, D), F32),
            pltpu.VMEM((D, 3 * D), BF16),
            pltpu.VMEM((D, D), BF16),
            pltpu.VMEM((D, 3 * D), BF16),
            pltpu.VMEM((D, D), BF16),
            pltpu.VMEM((D // 2, 3 * D), U32),
            pltpu.VMEM((D // 2, D), U32),
            pltpu.VMEM((D // 2, 3 * D), U32),
            pltpu.VMEM((D // 2, D), U32),
            pltpu.VMEM((CM // 2, D), U32),
            pltpu.VMEM((NT, HALO + BM, 128), F32),
            pltpu.VMEM((NT, HALO + BM, 128), F32),
            pltpu.VMEM((NT, S // 2, 128), U32),
            pltpu.VMEM((NT, S // 2, 128), U32),
            pltpu.VMEM((D // 2, S), U32),
            pltpu.VMEM((128, FQ), F32),
            pltpu.SemaphoreType.DMA((11,)),
            pltpu.SemaphoreType.DMA((S // BM,)),
        ],
        compiler_params=pltpu.CompilerParams(vmem_limit_bytes=110 * 1024 * 1024),
        name="interleaved_attention_stack",
    )(x, A_wqkv, A_wo, B_wqkv, B_wo)
    return out.reshape(1, S, D)
```

```python
import functools
import math

import jax
import jax.numpy as jnp
from jax import lax
import jax.experimental.pallas as pl
import jax.experimental.pallas.tpu as pltpu

S = 2048
D = 1024
H = 32
DH = D // H
NT = D // 128
HPT = 128 // DH
WIN = 8
DIL = 2
HALO = 16
EPS = 1e-5
LOG2E = math.log2(math.e)
QSCALE = (DH ** -0.5) * LOG2E
MASKED = -1e9 * LOG2E

BM = 256
CM = 128
NC = 128
SPLIT1 = 16
SPLIT2 = 16
RG = 16
KC = 512
QB = 1024
OS = 128
OB = 128
FQ = 128

L_LO = 2.0 ** -40
L_HI = 2.0 ** 90
O_HI = 3.0e38

F32 = jnp.float32
BF16 = jnp.bfloat16
U32 = jnp.uint32


def _layernorm(x):
    mu = jnp.mean(x, axis=-1, keepdims=True)
    xc = x - mu
    var = jnp.mean(xc * xc, axis=-1, keepdims=True)
    return xc * lax.rsqrt(var + EPS)


def _permute_cols(w32):
    rows = w32.shape[0]
    lane = lax.broadcasted_iota(jnp.int32, (rows, 128), 1)
    tiles = [w32[:, t * 128:(t + 1) * 128] for t in range(NT)]
    for b in range(3):
        sh = 4 << b
        low = (lane & sh) == 0
        for a in range(NT):
            if a & (1 << b):
                continue
            c = a | (1 << b)
            ta, tc = tiles[a], tiles[c]
            tiles[a] = jnp.where(low, ta, pltpu.roll(tc, sh, 1))
            tiles[c] = jnp.where(low, pltpu.roll(ta, 128 - sh, 1), tc)
    return jnp.concatenate(tiles, axis=1)


def _permute_rows(w32):
    ncols = w32.shape[1]
    nv = D // 16
    v = [w32[i * 8:(i + 1) * 8, :] for i in range(nv)]
    sub = lax.broadcasted_iota(jnp.int32, (8, ncols), 0)
    for vb, sh in ((8, 2), (16, 4)):
        low = (sub & sh) == 0
        for a in range(nv):
            if a & vb:
                continue
            c = a | vb
            ta, tc = v[a], v[c]
            v[a] = jnp.where(low, ta, pltpu.roll(tc, sh, 0))
            v[c] = jnp.where(low, pltpu.roll(ta, 8 - sh, 0), tc)
    def src(i):
        b0, b5 = i & 1, (i >> 5) & 1
        return (i & ~33) | (b0 << 5) | b5
    return jnp.concatenate([v[src(i)] for i in range(nv)], axis=0)


def _group_sum4(x, lane):
    b0 = (lane & 1) == 0
    x = x + jnp.where(b0, pltpu.roll(x, 127, 1), pltpu.roll(x, 1, 1))
    b1 = (lane & 2) == 0
    return x + jnp.where(b1, pltpu.roll(x, 126, 1), pltpu.roll(x, 2, 1))


def _pack(x):
    return pltpu.bitcast(x.astype(BF16), U32)


def _unpack(x):
    return pltpu.bitcast(x, BF16)


def _kernel(x_hbm, wa_hbm, woa_hbm, wb_hbm, wob_hbm, out_hbm,
            xio, xres, xsave, wst, wost, wst2, wost2, wa, woa, wb, wob, hb, h2b, ob, qbuf0, qbuf1, zref, kbuf, vbuf,
            qs, ks, vt, ots, wsems, sems, osems):
    nblk = S // BM
    qbuf = (qbuf0, qbuf1)
    zref[0] = 0
    nch = BM // CM
    pr = 128
    nwc = D // pr

    def wa_copy(c):
        r = pl.multiple_of(c * pr, pr)
        return pltpu.make_async_copy(wa_hbm.at[pl.ds(r, pr), :], wst.at[pl.ds(r, pr), :],
                                     wsems.at[c])

    def x_copy(r0, n, k):
        return pltpu.make_async_copy(x_hbm.at[pl.ds(r0, n), :], xio.at[pl.ds(r0, n), :], sems.at[k])

    cp_woa = pltpu.make_async_copy(woa_hbm, wost, sems.at[0])
    cp_x0 = x_copy(0, BM, 1)
    cp_wb = pltpu.make_async_copy(wb_hbm, wst2, sems.at[2])
    cp_x1 = x_copy(BM, BM, 3)
    cp_x2 = x_copy(2 * BM, S - 2 * BM, 4)
    cp_wob = pltpu.make_async_copy(wob_hbm, wost2, sems.at[5])
    ahead = 3
    for c in range(ahead):
        wa_copy(c).start()

    for t in range(NT):
        kbuf[t, BM:BM + HALO, :] = jnp.zeros((HALO, 128), F32)
        vbuf[t, BM:BM + HALO, :] = jnp.zeros((HALO, 128), F32)

    def perm_body(c, carry):
        wa_copy(c).wait()

        @pl.when(c + ahead < nwc)
        def _():
            wa_copy(jnp.minimum(c + ahead, nwc - 1)).start()

        @pl.when(c + ahead == nwc)
        def _():
            cp_woa.start()

        @pl.when(c + ahead == nwc + 1)
        def _():
            cp_x0.start()

        r = pl.multiple_of(c * pr, pr)
        r2 = pl.multiple_of(c * (pr // 2), pr // 2)
        for sec in range(3):
            w32 = _pack(wst[pl.ds(r, pr), sec * D:(sec + 1) * D])
            wa[pl.ds(r2, pr // 2), sec * D:(sec + 1) * D] = _permute_cols(w32)
        return carry

    with jax.named_scope("perm_cols"):
        lax.fori_loop(0, nwc, perm_body, 0)

    with jax.named_scope("perm_rows"):
        cp_woa.wait()
        cp_wb.start()
        cp_x1.start()

        def permo_body(i, carry):
            c0 = pl.multiple_of(i * 128, 128)
            woa[:, pl.ds(c0, 128)] = _permute_rows(_pack(wost[:, pl.ds(c0, 128)]))
            return carry

        lax.fori_loop(0, NT, permo_body, 0)

    def widen_x(r0, nrows):
        step = 64

        def body(i, carry):
            r = pl.multiple_of(r0 + i * step, step)
            xres[pl.ds(r, step), :] = xio[pl.ds(r, step), :].astype(F32)
            return carry

        lax.fori_loop(0, nrows // step, body, 0)

    def repack(src, dst):
        step = 64

        def body(i, carry):
            r = pl.multiple_of(i * step, step)
            r2 = pl.multiple_of(i * (step // 2), step // 2)
            dst[pl.ds(r2, step // 2), :] = _pack(src[pl.ds(r, step), :])
            return carry

        lax.fori_loop(0, D // step, body, 0)

    with jax.named_scope("x_in"):
        cp_x0.wait()
        widen_x(0, BM)

    lane = lax.broadcasted_iota(jnp.int32, (RG, 128), 1)
    rowi = lax.broadcasted_iota(jnp.int32, (RG, 128), 0)

    def tile_dot(lhs_ref, w_ref, n):
        return jnp.dot(_unpack(lhs_ref[...]), _unpack(w_ref[:, n * NC:(n + 1) * NC]),
                       preferred_element_type=F32)

    tpc = NC // 128

    def local_qkv(h_ref, off, i, lo=0, hi=3 * D // NC):
        for n in (list(range(D // NC, 3 * D // NC)) + list(range(D // NC)))[lo:hi]:
            res = tile_dot(h_ref, wa, n)
            for u in range(tpc):
                sec, t = divmod(n * tpc + u, NT)
                val = res[:, u * 128:(u + 1) * 128]
                if sec == 0:
                    qbuf[off // CM][t, 0:CM, :] = val
                elif sec == 1:
                    kbuf[t, HALO + off:HALO + off + CM, :] = val
                else:
                    vbuf[t, HALO + off:HALO + off + CM, :] = val
                    if off == 0:
                        first = jnp.broadcast_to(val[0:1, :], (HALO, 128))
                        vbuf[t, 0:HALO, :] = jnp.where(i == 0, first, vbuf[t, 0:HALO, :])

    def local_attn(o_ref, off, i):
        zero = zref[0]
        for g in range(CM // RG):
            base = HALO + off + g * RG
            qg = [qbuf[off // CM][t, pl.ds(pl.multiple_of(zero + g * RG, RG), RG), :] for t in range(NT)]
            logit = []
            for w in range(WIN):
                a = base - DIL * w
                part = qg[0] * kbuf[0, a:a + RG, :]
                for t in range(1, NT):
                    part = part + qg[t] * kbuf[t, a:a + RG, :]
                lg = _group_sum4(part, lane) * QSCALE
                if off == 0 and g == 0 and w > 0:
                    lg = jnp.where(rowi + i * BM >= DIL * w, lg, MASKED)
                logit.append(lg)
            m = functools.reduce(jnp.maximum, logit)
            p = [jnp.exp2(lg - m) for lg in logit]
            inv = 1.0 / functools.reduce(lambda u, v: u + v, p)
            for t in range(NT):
                acc = p[0] * vbuf[t, base:base + RG, :]
                for w in range(1, WIN):
                    a = base - DIL * w
                    acc = acc + p[w] * vbuf[t, a:a + RG, :]
                o_ref[g * RG // 2:(g + 1) * RG // 2, t * 128:(t + 1) * 128] = _pack(acc * inv)

    def full_qkv(h_ref, r, lo=0, hi=3 * D // NC):
        r2 = pl.multiple_of(r // 2, CM // 2)
        order = list(range(2 * D // NC, 3 * D // NC)) + list(range(2 * D // NC))
        for n in order[lo:hi]:
            res = tile_dot(h_ref, wb, n)
            for u in range(tpc):
                sec, t = divmod(n * tpc + u, NT)
                val = res[:, u * 128:(u + 1) * 128]
                if sec == 0:
                    qs[t, pl.ds(r2, CM // 2), :] = _pack(val * QSCALE)
                elif sec == 1:
                    ks[t, pl.ds(r2, CM // 2), :] = _pack(val)
                else:
                    vt[t * 64:(t + 1) * 64, pl.ds(r, CM)] = _pack(val.T)

    def row_phase(pair):
        hb[0] = _pack(_layernorm(xres[0:CM, :]))

        def body(i, c):
            @pl.when(jnp.logical_and(pair == 0, i == 1))
            def _():
                cp_x2.wait()
                widen_x(2 * BM, S - 2 * BM)
                cp_wob.wait()
                repack(wost2, wob)

            r0 = pl.multiple_of(i * BM, BM)
            rs = [pl.multiple_of(r0 + ch * CM, CM) for ch in range(nch)]
            for t in range(NT):
                kbuf[t, 0:HALO, :] = kbuf[t, BM:BM + HALO, :]
                vbuf[t, 0:HALO, :] = vbuf[t, BM:BM + HALO, :]
            rn = pl.multiple_of(jnp.minimum(i + 1, nblk - 1) * BM, BM)

            def local_out(ch):
                local_attn(ob.at[ch], ch * CM, i)
                y = jnp.concatenate([tile_dot(ob.at[ch], woa, n) for n in range(D // NC)], axis=1)
                x2 = xres[pl.ds(rs[ch], CM), :] + y
                xres[pl.ds(rs[ch], CM), :] = x2
                xsave[pl.ds(rs[ch], CM), :] = x2
                h2b[ch] = _pack(_layernorm(x2))

            hb[1] = _pack(_layernorm(xres[pl.ds(rs[1], CM), :]))
            local_qkv(hb.at[0], 0, i)
            local_qkv(hb.at[1], CM, i, 0, SPLIT1)
            local_out(0)
            local_qkv(hb.at[1], CM, i, SPLIT1)

            @pl.when(jnp.logical_and(pair == 0, i == 0))
            def _():
                cp_wb.wait()
                cp_x2.start()
                cp_wob.start()
                repack(wst2, wb)
                cp_x1.wait()
                widen_x(BM, BM)

            full_qkv(h2b.at[0], rs[0], 0, SPLIT2)
            local_out(1)
            full_qkv(h2b.at[0], rs[0], SPLIT2)
            full_qkv(h2b.at[1], rs[1], 0, 10)
            hb[0] = _pack(_layernorm(xres[pl.ds(rn, CM), :]))
            full_qkv(h2b.at[1], rs[1], 10)
            return c

        with jax.named_scope("row_phase"):
            lax.fori_loop(0, nblk, body, 0)

    early = QB // OB

    def out_copy(i):
        r0 = pl.multiple_of(i * OB, OB)
        return pltpu.make_async_copy(xio.at[pl.ds(r0, OB), :], out_hbm.at[pl.ds(r0, OB), :],
                                     osems.at[i])

    def write_out(lo, hi):
        def body(i, c):
            r0 = pl.multiple_of(i * OB, OB)
            xio[pl.ds(r0, OB), :] = xres[pl.ds(r0, OB), :].astype(BF16)
            out_copy(i).start()
            return c

        lax.fori_loop(lo, hi, body, 0)

    nt_dims = (((1,), (1,)), ((), ()))

    def masked_q(q32, hp):
        head = lax.broadcasted_iota(jnp.int32, q32.shape, 1) // DH
        return _unpack(jnp.where(head == hp, q32, jnp.uint32(0)))

    def add_oproj(ot, g, q0, nq):
        g64 = pl.multiple_of(g * 64, 64)
        for j in range(nq // OS):
            y = jnp.dot(ot[:, j * OS:(j + 1) * OS].T.astype(BF16), _unpack(wob[pl.ds(g64, 64), :]),
                        preferred_element_type=F32)
            r = pl.multiple_of(q0 + j * OS, OS)
            xres[pl.ds(r, OS), :] = xres[pl.ds(r, OS), :] + y

    def full_attn(pair):
        nqb = S // QB

        def body(it, bad):
            @pl.when(jnp.logical_and(pair == 1, it == NT))
            def _():
                write_out(0, early)

            g = it % NT
            q0 = pl.multiple_of((it // NT) * QB, QB)
            q32 = qs[g, pl.ds(pl.multiple_of(q0 // 2, QB // 2), QB // 2), :]
            outs = []
            for hp in range(HPT):
                w = masked_q(q32, hp)
                r0 = pl.multiple_of(g * 64 + hp * (DH // 2), DH // 2)
                acc = jnp.zeros((DH, QB), F32)
                l8 = jnp.zeros((8, QB), F32)
                for t in range(S // KC):
                    kc = _unpack(ks[g, t * KC // 2:(t + 1) * KC // 2, :])
                    s = lax.dot_general(kc, w, nt_dims, preferred_element_type=F32)
                    p = jnp.exp2(s)
                    l8 = l8 + jnp.sum(p.reshape(KC // 8, 8, QB), axis=0)
                    vc = _unpack(vt[pl.ds(r0, DH // 2), t * KC:(t + 1) * KC])
                    acc = acc + jnp.dot(vc, p.astype(BF16), preferred_element_type=F32)
                l = jnp.sum(l8, axis=0, keepdims=True)
                o = acc * (1.0 / l)
                outs.append(o)
                ok = (jnp.abs(o) < O_HI) & (l > L_LO) & (l < L_HI)
                nbad = jnp.where(ok, 0.0, 1.0)
                bad = jnp.maximum(bad, jnp.max(nbad.reshape(DH // 8, 8, QB), axis=0))
            add_oproj(jnp.concatenate(outs, axis=0), g, q0, QB)
            return bad

        with jax.named_scope("full_attn"):
            bad = lax.fori_loop(0, NT * nqb, body, jnp.zeros((8, QB), F32))

        @pl.when(jnp.max(bad) > 0.0)
        def _():
            nq = S // FQ

            def restore(i, c):
                r = pl.multiple_of(i * 32, 32)
                xres[pl.ds(r, 32), :] = xsave[pl.ds(r, 32), :]
                return c

            lax.fori_loop(0, S // 32, restore, 0)

            def fb_body(it, c):
                g = it // nq
                q0 = pl.multiple_of((it % nq) * FQ, FQ)
                q32 = qs[g, pl.ds(pl.multiple_of(q0 // 2, FQ // 2), FQ // 2), :]

                def head_body(hp, c2):
                    r0 = pl.multiple_of(g * 64 + hp * (DH // 2), DH // 2)
                    s = lax.dot_general(_unpack(ks[g]), masked_q(q32, hp), nt_dims,
                                        preferred_element_type=F32)
                    p = jnp.exp2(s - jnp.max(s, axis=0, keepdims=True))
                    l = jnp.sum(p, axis=0, keepdims=True)
                    acc = jnp.dot(_unpack(vt[pl.ds(r0, DH // 2), :]), p.astype(BF16),
                                  preferred_element_type=F32)
                    ots[pl.ds(pl.multiple_of(hp * DH, DH), DH), :] = acc * (1.0 / l)
                    return c2

                lax.fori_loop(0, HPT, head_body, 0)
                add_oproj(ots[...], g, q0, FQ)
                return c

            lax.fori_loop(0, NT * nq, fb_body, 0)

            @pl.when(pair == 1)
            def _():
                for i in range(early):
                    out_copy(i).wait()
                write_out(0, early)

    def pair_body(pair, c):
        row_phase(pair)
        full_attn(pair)
        return c

    with jax.named_scope("pairs"):
        lax.fori_loop(0, 2, pair_body, 0)

    with jax.named_scope("out_phase"):
        write_out(early, S // OB)
        for i in range(S // OB):
            out_copy(i).wait()


@jax.jit
def pallas_interleave_layers__sliding_local_dilated__softmax_full_mha__prompt_kernel(
    A_x: jax.Array,
    A_wqkv: jax.Array,
    A_wo: jax.Array,
    B_x: jax.Array,
    B_wqkv: jax.Array,
    B_wo: jax.Array,
):
    del B_x
    x = A_x.reshape(S, D)
    hbm = pl.BlockSpec(memory_space=pl.ANY)
    out = pl.pallas_call(
        _kernel,
        out_shape=jax.ShapeDtypeStruct((S, D), BF16),
        in_specs=[hbm] * 5,
        out_specs=hbm,
        scratch_shapes=[
            pltpu.VMEM((S, D), BF16),
            pltpu.VMEM((S, D), F32),
            pltpu.VMEM((S, D), F32),
            pltpu.VMEM((D, 3 * D), BF16),
            pltpu.VMEM((D, D), BF16),
            pltpu.VMEM((D, 3 * D), BF16),
            pltpu.VMEM((D, D), BF16),
            pltpu.VMEM((D // 2, 3 * D), U32),
            pltpu.VMEM((D // 2, D), U32),
            pltpu.VMEM((D // 2, 3 * D), U32),
            pltpu.VMEM((D // 2, D), U32),
            pltpu.VMEM((BM // CM, CM // 2, D), U32),
            pltpu.VMEM((BM // CM, CM // 2, D), U32),
            pltpu.VMEM((BM // CM, CM // 2, D), U32),
            pltpu.VMEM((NT, CM + 8, 128), F32),
            pltpu.VMEM((NT, CM + 8, 128), F32),
            pltpu.SMEM((1,), jnp.int32),
            pltpu.VMEM((NT, HALO + BM, 128), F32),
            pltpu.VMEM((NT, HALO + BM, 128), F32),
            pltpu.VMEM((NT, S // 2, 128), U32),
            pltpu.VMEM((NT, S // 2, 128), U32),
            pltpu.VMEM((D // 2, S), U32),
            pltpu.VMEM((128, FQ), F32),
            pltpu.SemaphoreType.DMA((D // 128,)),
            pltpu.SemaphoreType.DMA((6,)),
            pltpu.SemaphoreType.DMA((S // OB,)),
        ],
        compiler_params=pltpu.CompilerParams(vmem_limit_bytes=110 * 1024 * 1024),
        name="interleaved_attention_stack",
    )(x, A_wqkv, A_wo, B_wqkv, B_wo)
    return out.reshape(1, S, D)
```

```python
import functools
import math

import jax
import jax.numpy as jnp
from jax import lax
import jax.experimental.pallas as pl
import jax.experimental.pallas.tpu as pltpu

S = 2048
D = 1024
H = 32
DH = D // H
NT = D // 128
HPT = 128 // DH
WIN = 8
DIL = 2
HALO = 16
EPS = 1e-5
LOG2E = math.log2(math.e)
QSCALE = (DH ** -0.5) * LOG2E
MASKED = -1e9 * LOG2E

BM = 256
CM = 128
NC = 128
SPLIT1 = 16
SPLIT2 = 16
RG = 16
KC = 512
QB = 1024
OS = 128
OB = 128
FQ = 128

L_LO = 2.0 ** -40
L_HI = 2.0 ** 90
O_HI = 3.0e38

F32 = jnp.float32
BF16 = jnp.bfloat16
U32 = jnp.uint32


def _layernorm(x):
    mu = jnp.mean(x, axis=-1, keepdims=True)
    xc = x - mu
    var = jnp.mean(xc * xc, axis=-1, keepdims=True)
    return xc * lax.rsqrt(var + EPS)


def _permute_cols(w32):
    rows = w32.shape[0]
    lane = lax.broadcasted_iota(jnp.int32, (rows, 128), 1)
    tiles = [w32[:, t * 128:(t + 1) * 128] for t in range(NT)]
    for b in range(3):
        sh = 4 << b
        low = (lane & sh) == 0
        for a in range(NT):
            if a & (1 << b):
                continue
            c = a | (1 << b)
            ta, tc = tiles[a], tiles[c]
            tiles[a] = jnp.where(low, ta, pltpu.roll(tc, sh, 1))
            tiles[c] = jnp.where(low, pltpu.roll(ta, 128 - sh, 1), tc)
    return jnp.concatenate(tiles, axis=1)


def _permute_rows(w32):
    ncols = w32.shape[1]
    nv = D // 16
    v = [w32[i * 8:(i + 1) * 8, :] for i in range(nv)]
    sub = lax.broadcasted_iota(jnp.int32, (8, ncols), 0)
    for vb, sh in ((8, 2), (16, 4)):
        low = (sub & sh) == 0
        for a in range(nv):
            if a & vb:
                continue
            c = a | vb
            ta, tc = v[a], v[c]
            v[a] = jnp.where(low, ta, pltpu.roll(tc, sh, 0))
            v[c] = jnp.where(low, pltpu.roll(ta, 8 - sh, 0), tc)
    def src(i):
        b0, b5 = i & 1, (i >> 5) & 1
        return (i & ~33) | (b0 << 5) | b5
    return jnp.concatenate([v[src(i)] for i in range(nv)], axis=0)


def _group_sum4(x, lane):
    b0 = (lane & 1) == 0
    x = x + jnp.where(b0, pltpu.roll(x, 127, 1), pltpu.roll(x, 1, 1))
    b1 = (lane & 2) == 0
    return x + jnp.where(b1, pltpu.roll(x, 126, 1), pltpu.roll(x, 2, 1))


def _pack(x):
    return pltpu.bitcast(x.astype(BF16), U32)


def _unpack(x):
    return pltpu.bitcast(x, BF16)


def _ipack(x):
    r, c = x.shape
    x4 = x.reshape(r // 16, 2, 8, c)
    lo = x4[:, 0].reshape(r // 2, c)
    hi = x4[:, 1].reshape(r // 2, c)
    return pltpu.bitcast(pltpu.pack_elementwise([lo, hi], packed_dtype=BF16), U32)


def _kernel(x_hbm, wa_hbm, woa_hbm, wb_hbm, wob_hbm, out_hbm,
            xio, xres, xsave, wst, wost, wst2, wost2, wa, woa, wb, wob, hb, h2b, ob, qbuf0, qbuf1, zref, kbuf, vbuf,
            qs, ks, vt, ots, pb0, pb1, pb2, pb3, wsems, sems, osems):
    nblk = S // BM
    qbuf = (qbuf0, qbuf1)
    pbufs = (pb0, pb1, pb2, pb3)
    zref[0] = 0
    nch = BM // CM
    pr = 128
    nwc = D // pr

    def wa_copy(c):
        r = pl.multiple_of(c * pr, pr)
        return pltpu.make_async_copy(wa_hbm.at[pl.ds(r, pr), :], wst.at[pl.ds(r, pr), :],
                                     wsems.at[c])

    def x_copy(r0, n, k):
        return pltpu.make_async_copy(x_hbm.at[pl.ds(r0, n), :], xio.at[pl.ds(r0, n), :], sems.at[k])

    cp_woa = pltpu.make_async_copy(woa_hbm, wost, sems.at[0])
    cp_x0 = x_copy(0, BM, 1)
    cp_wb = pltpu.make_async_copy(wb_hbm, wst2, sems.at[2])
    cp_x1 = x_copy(BM, BM, 3)
    cp_x2 = x_copy(2 * BM, S - 2 * BM, 4)
    cp_wob = pltpu.make_async_copy(wob_hbm, wost2, sems.at[5])
    ahead = 3
    for c in range(ahead):
        wa_copy(c).start()

    for t in range(NT):
        kbuf[t, BM:BM + HALO, :] = jnp.zeros((HALO, 128), F32)
        vbuf[t, BM:BM + HALO, :] = jnp.zeros((HALO, 128), F32)

    def perm_body(c, carry):
        wa_copy(c).wait()

        @pl.when(c + ahead < nwc)
        def _():
            wa_copy(jnp.minimum(c + ahead, nwc - 1)).start()

        @pl.when(c + ahead == nwc)
        def _():
            cp_woa.start()

        @pl.when(c + ahead == nwc + 1)
        def _():
            cp_x0.start()

        r = pl.multiple_of(c * pr, pr)
        r2 = pl.multiple_of(c * (pr // 2), pr // 2)
        for sec in range(3):
            w32 = _pack(wst[pl.ds(r, pr), sec * D:(sec + 1) * D])
            wa[pl.ds(r2, pr // 2), sec * D:(sec + 1) * D] = _permute_cols(w32)
        return carry

    with jax.named_scope("perm_cols"):
        lax.fori_loop(0, nwc, perm_body, 0)

    with jax.named_scope("perm_rows"):
        cp_woa.wait()
        cp_wb.start()
        cp_x1.start()

        def permo_body(i, carry):
            c0 = pl.multiple_of(i * 128, 128)
            woa[:, pl.ds(c0, 128)] = _permute_rows(_pack(wost[:, pl.ds(c0, 128)]))
            return carry

        lax.fori_loop(0, NT, permo_body, 0)

    def widen_x(r0, nrows):
        step = 64

        def body(i, carry):
            r = pl.multiple_of(r0 + i * step, step)
            xres[pl.ds(r, step), :] = xio[pl.ds(r, step), :].astype(F32)
            return carry

        lax.fori_loop(0, nrows // step, body, 0)

    def repack(src, dst):
        step = 64

        def body(i, carry):
            r = pl.multiple_of(i * step, step)
            r2 = pl.multiple_of(i * (step // 2), step // 2)
            dst[pl.ds(r2, step // 2), :] = _pack(src[pl.ds(r, step), :])
            return carry

        lax.fori_loop(0, D // step, body, 0)

    with jax.named_scope("x_in"):
        cp_x0.wait()
        widen_x(0, BM)

    lane = lax.broadcasted_iota(jnp.int32, (RG, 128), 1)
    rowi = lax.broadcasted_iota(jnp.int32, (RG, 128), 0)

    def tile_dot(lhs_ref, w_ref, n):
        return jnp.dot(_unpack(lhs_ref[...]), _unpack(w_ref[:, n * NC:(n + 1) * NC]),
                       preferred_element_type=F32)

    tpc = NC // 128

    def local_qkv(h_ref, off, i, lo=0, hi=3 * D // NC):
        for n in (list(range(D // NC, 3 * D // NC)) + list(range(D // NC)))[lo:hi]:
            res = tile_dot(h_ref, wa, n)
            for u in range(tpc):
                sec, t = divmod(n * tpc + u, NT)
                val = res[:, u * 128:(u + 1) * 128]
                if sec == 0:
                    qbuf[off // CM][t, 0:CM, :] = val
                elif sec == 1:
                    kbuf[t, HALO + off:HALO + off + CM, :] = val
                else:
                    vbuf[t, HALO + off:HALO + off + CM, :] = val
                    if off == 0:
                        first = jnp.broadcast_to(val[0:1, :], (HALO, 128))
                        vbuf[t, 0:HALO, :] = jnp.where(i == 0, first, vbuf[t, 0:HALO, :])

    def local_attn(o_ref, off, i):
        zero = zref[0]
        for g in range(CM // RG):
            base = HALO + off + g * RG
            qg = [qbuf[off // CM][t, pl.ds(pl.multiple_of(zero + g * RG, RG), RG), :] for t in range(NT)]
            logit = []
            for w in range(WIN):
                a = base - DIL * w
                part = qg[0] * kbuf[0, a:a + RG, :]
                for t in range(1, NT):
                    part = part + qg[t] * kbuf[t, a:a + RG, :]
                lg = _group_sum4(part, lane) * QSCALE
                if off == 0 and g == 0 and w > 0:
                    lg = jnp.where(rowi + i * BM >= DIL * w, lg, MASKED)
                logit.append(lg)
            m = functools.reduce(jnp.maximum, logit)
            p = [jnp.exp2(lg - m) for lg in logit]
            inv = 1.0 / functools.reduce(lambda u, v: u + v, p)
            for t in range(NT):
                acc = p[0] * vbuf[t, base:base + RG, :]
                for w in range(1, WIN):
                    a = base - DIL * w
                    acc = acc + p[w] * vbuf[t, a:a + RG, :]
                o_ref[g * RG // 2:(g + 1) * RG // 2, t * 128:(t + 1) * 128] = _pack(acc * inv)

    def full_qkv(h_ref, r, lo=0, hi=3 * D // NC):
        r2 = pl.multiple_of(r // 2, CM // 2)
        order = list(range(2 * D // NC, 3 * D // NC)) + list(range(2 * D // NC))
        for n in order[lo:hi]:
            res = tile_dot(h_ref, wb, n)
            for u in range(tpc):
                sec, t = divmod(n * tpc + u, NT)
                val = res[:, u * 128:(u + 1) * 128]
                if sec == 0:
                    qs[t, pl.ds(r2, CM // 2), :] = _pack(val * QSCALE)
                elif sec == 1:
                    ks[t, pl.ds(r2, CM // 2), :] = _pack(val)
                else:
                    vt[t * 64:(t + 1) * 64, pl.ds(r, CM)] = pltpu.bitcast(_unpack(_ipack(val)).T, U32)

    def row_phase(pair):
        hb[0] = _pack(_layernorm(xres[0:CM, :]))

        def body(i, c):
            @pl.when(jnp.logical_and(pair == 0, i == 1))
            def _():
                cp_x2.wait()
                widen_x(2 * BM, S - 2 * BM)
                cp_wob.wait()
                repack(wost2, wob)

            r0 = pl.multiple_of(i * BM, BM)
            rs = [pl.multiple_of(r0 + ch * CM, CM) for ch in range(nch)]
            for t in range(NT):
                kbuf[t, 0:HALO, :] = kbuf[t, BM:BM + HALO, :]
                vbuf[t, 0:HALO, :] = vbuf[t, BM:BM + HALO, :]
            rn = pl.multiple_of(jnp.minimum(i + 1, nblk - 1) * BM, BM)

            def local_out(ch):
                local_attn(ob.at[ch], ch * CM, i)
                y = jnp.concatenate([tile_dot(ob.at[ch], woa, n) for n in range(D // NC)], axis=1)
                x2 = xres[pl.ds(rs[ch], CM), :] + y
                xres[pl.ds(rs[ch], CM), :] = x2
                xsave[pl.ds(rs[ch], CM), :] = x2
                h2b[ch] = _pack(_layernorm(x2))

            hb[1] = _pack(_layernorm(xres[pl.ds(rs[1], CM), :]))
            local_qkv(hb.at[0], 0, i)
            local_qkv(hb.at[1], CM, i, 0, SPLIT1)
            local_out(0)
            local_qkv(hb.at[1], CM, i, SPLIT1)

            @pl.when(jnp.logical_and(pair == 0, i == 0))
            def _():
                cp_wb.wait()
                cp_x2.start()
                cp_wob.start()
                repack(wst2, wb)
                cp_x1.wait()
                widen_x(BM, BM)

            full_qkv(h2b.at[0], rs[0], 0, SPLIT2)
            local_out(1)
            full_qkv(h2b.at[0], rs[0], SPLIT2)
            full_qkv(h2b.at[1], rs[1], 0, 10)
            hb[0] = _pack(_layernorm(xres[pl.ds(rn, CM), :]))
            full_qkv(h2b.at[1], rs[1], 10)
            return c

        with jax.named_scope("row_phase"):
            lax.fori_loop(0, nblk, body, 0)

    early = QB // OB

    def out_copy(i):
        r0 = pl.multiple_of(i * OB, OB)
        return pltpu.make_async_copy(xio.at[pl.ds(r0, OB), :], out_hbm.at[pl.ds(r0, OB), :],
                                     osems.at[i])

    def write_out(lo, hi):
        def body(i, c):
            r0 = pl.multiple_of(i * OB, OB)
            xio[pl.ds(r0, OB), :] = xres[pl.ds(r0, OB), :].astype(BF16)
            out_copy(i).start()
            return c

        lax.fori_loop(lo, hi, body, 0)

    nt_dims = (((1,), (1,)), ((), ()))

    def masked_q(q32, hp):
        head = lax.broadcasted_iota(jnp.int32, q32.shape, 1) // DH
        return _unpack(jnp.where(head == hp, q32, jnp.uint32(0)))

    def add_oproj(ot, g, q0, nq):
        g64 = pl.multiple_of(g * 64, 64)
        for j in range(nq // OS):
            y = jnp.dot(ot[:, j * OS:(j + 1) * OS].T.astype(BF16), _unpack(wob[pl.ds(g64, 64), :]),
                        preferred_element_type=F32)
            r = pl.multiple_of(q0 + j * OS, OS)
            xres[pl.ds(r, OS), :] = xres[pl.ds(r, OS), :] + y

    def full_attn(pair):
        nqb = S // QB

        def body(it, bad):
            @pl.when(jnp.logical_and(pair == 1, it == NT))
            def _():
                write_out(0, early)

            g = it % NT
            q0 = pl.multiple_of((it // NT) * QB, QB)
            q32 = qs[g, pl.ds(pl.multiple_of(q0 // 2, QB // 2), QB // 2), :]
            zero = zref[0]
            acc = [None] * HPT
            l8 = [None] * HPT

            def pv(hp, t, buf):
                r0 = pl.multiple_of(g * 64 + hp * (DH // 2), DH // 2)
                vc = _unpack(vt[pl.ds(r0, DH // 2), t * KC:(t + 1) * KC])
                a = jnp.dot(vc, _unpack(buf[zero]), preferred_element_type=F32)
                acc[hp] = a if acc[hp] is None else acc[hp] + a

            pending = None
            for hp in range(HPT):
                w = masked_q(q32, hp)
                for t in range(S // KC):
                    kc = _unpack(ks[g, t * KC // 2:(t + 1) * KC // 2, :])
                    p = jnp.exp2(lax.dot_general(kc, w, nt_dims, preferred_element_type=F32))
                    part = jnp.sum(p.reshape(KC // 8, 8, QB), axis=0)
                    l8[hp] = part if l8[hp] is None else l8[hp] + part
                    buf = pbufs[(hp * (S // KC) + t) % len(pbufs)]
                    buf[0] = _ipack(p)
                    if pending is not None:
                        pv(*pending)
                    pending = (hp, t, buf)
            pv(*pending)
            outs = []
            for hp in range(HPT):
                l = jnp.sum(l8[hp], axis=0, keepdims=True)
                o = acc[hp] * (1.0 / l)
                outs.append(o)
                ok = (jnp.abs(o) < O_HI) & (l > L_LO) & (l < L_HI)
                nbad = jnp.where(ok, 0.0, 1.0)
                bad = jnp.maximum(bad, jnp.max(nbad.reshape(DH // 8, 8, QB), axis=0))
            add_oproj(jnp.concatenate(outs, axis=0), g, q0, QB)
            return bad

        with jax.named_scope("full_attn"):
            bad = lax.fori_loop(0, NT * nqb, body, jnp.zeros((8, QB), F32))

        @pl.when(jnp.max(bad) > 0.0)
        def _():
            nq = S // FQ

            def restore(i, c):
                r = pl.multiple_of(i * 32, 32)
                xres[pl.ds(r, 32), :] = xsave[pl.ds(r, 32), :]
                return c

            lax.fori_loop(0, S // 32, restore, 0)

            def fb_body(it, c):
                g = it // nq
                q0 = pl.multiple_of((it % nq) * FQ, FQ)
                q32 = qs[g, pl.ds(pl.multiple_of(q0 // 2, FQ // 2), FQ // 2), :]

                def head_body(hp, c2):
                    r0 = pl.multiple_of(g * 64 + hp * (DH // 2), DH // 2)
                    s = lax.dot_general(_unpack(ks[g]), masked_q(q32, hp), nt_dims,
                                        preferred_element_type=F32)
                    p = jnp.exp2(s - jnp.max(s, axis=0, keepdims=True))
                    l = jnp.sum(p, axis=0, keepdims=True)
                    acc = jnp.dot(_unpack(vt[pl.ds(r0, DH // 2), :]), _unpack(_ipack(p)),
                                  preferred_element_type=F32)
                    ots[pl.ds(pl.multiple_of(hp * DH, DH), DH), :] = acc * (1.0 / l)
                    return c2

                lax.fori_loop(0, HPT, head_body, 0)
                add_oproj(ots[...], g, q0, FQ)
                return c

            lax.fori_loop(0, NT * nq, fb_body, 0)

            @pl.when(pair == 1)
            def _():
                for i in range(early):
                    out_copy(i).wait()
                write_out(0, early)

    def pair_body(pair, c):
        row_phase(pair)
        full_attn(pair)
        return c

    with jax.named_scope("pairs"):
        lax.fori_loop(0, 2, pair_body, 0)

    with jax.named_scope("out_phase"):
        write_out(early, S // OB)
        for i in range(S // OB):
            out_copy(i).wait()


@jax.jit
def pallas_interleave_layers__sliding_local_dilated__softmax_full_mha__prompt_kernel(
    A_x: jax.Array,
    A_wqkv: jax.Array,
    A_wo: jax.Array,
    B_x: jax.Array,
    B_wqkv: jax.Array,
    B_wo: jax.Array,
):
    del B_x
    x = A_x.reshape(S, D)
    hbm = pl.BlockSpec(memory_space=pl.ANY)
    out = pl.pallas_call(
        _kernel,
        out_shape=jax.ShapeDtypeStruct((S, D), BF16),
        in_specs=[hbm] * 5,
        out_specs=hbm,
        scratch_shapes=[
            pltpu.VMEM((S, D), BF16),
            pltpu.VMEM((S, D), F32),
            pltpu.VMEM((S, D), F32),
            pltpu.VMEM((D, 3 * D), BF16),
            pltpu.VMEM((D, D), BF16),
            pltpu.VMEM((D, 3 * D), BF16),
            pltpu.VMEM((D, D), BF16),
            pltpu.VMEM((D // 2, 3 * D), U32),
            pltpu.VMEM((D // 2, D), U32),
            pltpu.VMEM((D // 2, 3 * D), U32),
            pltpu.VMEM((D // 2, D), U32),
            pltpu.VMEM((BM // CM, CM // 2, D), U32),
            pltpu.VMEM((BM // CM, CM // 2, D), U32),
            pltpu.VMEM((BM // CM, CM // 2, D), U32),
            pltpu.VMEM((NT, CM + 8, 128), F32),
            pltpu.VMEM((NT, CM + 8, 128), F32),
            pltpu.SMEM((1,), jnp.int32),
            pltpu.VMEM((NT, HALO + BM, 128), F32),
            pltpu.VMEM((NT, HALO + BM, 128), F32),
            pltpu.VMEM((NT, S // 2, 128), U32),
            pltpu.VMEM((NT, S // 2, 128), U32),
            pltpu.VMEM((D // 2, S), U32),
            pltpu.VMEM((128, FQ), F32),
            pltpu.VMEM((1, KC // 2, QB), U32),
            pltpu.VMEM((1, KC // 2, QB), U32),
            pltpu.VMEM((1, KC // 2, QB), U32),
            pltpu.VMEM((1, KC // 2, QB), U32),
            pltpu.SemaphoreType.DMA((D // 128,)),
            pltpu.SemaphoreType.DMA((6,)),
            pltpu.SemaphoreType.DMA((S // OB,)),
        ],
        compiler_params=pltpu.CompilerParams(vmem_limit_bytes=110 * 1024 * 1024),
        name="interleaved_attention_stack",
    )(x, A_wqkv, A_wo, B_wqkv, B_wo)
    return out.reshape(1, S, D)
```

```python
import functools
import math

import jax
import jax.numpy as jnp
from jax import lax
import jax.experimental.pallas as pl
import jax.experimental.pallas.tpu as pltpu

S = 2048
D = 1024
H = 32
DH = D // H
NT = D // 128
HPT = 128 // DH
WIN = 8
DIL = 2
HALO = 16
EPS = 1e-5
LOG2E = math.log2(math.e)
QSCALE = (DH ** -0.5) * LOG2E
MASKED = -1e9 * LOG2E

BM = 256
CM = 128
NC = 128
SPLIT1 = 16
SPLIT2 = 16
RG = 16
KC = 512
QB = 1024
OS = 128
OB = 128
FQ = 128

L_LO = 2.0 ** -40
L_HI = 2.0 ** 90
O_HI = 3.0e38

F32 = jnp.float32
BF16 = jnp.bfloat16
U32 = jnp.uint32


def _layernorm(x):
    mu = jnp.mean(x, axis=-1, keepdims=True)
    xc = x - mu
    var = jnp.mean(xc * xc, axis=-1, keepdims=True)
    return xc * lax.rsqrt(var + EPS)


def _permute_cols(w32):
    rows = w32.shape[0]
    lane = lax.broadcasted_iota(jnp.int32, (rows, 128), 1)
    tiles = [w32[:, t * 128:(t + 1) * 128] for t in range(NT)]
    for b in range(3):
        sh = 4 << b
        low = (lane & sh) == 0
        for a in range(NT):
            if a & (1 << b):
                continue
            c = a | (1 << b)
            ta, tc = tiles[a], tiles[c]
            tiles[a] = jnp.where(low, ta, pltpu.roll(tc, sh, 1))
            tiles[c] = jnp.where(low, pltpu.roll(ta, 128 - sh, 1), tc)
    return jnp.concatenate(tiles, axis=1)


def _permute_rows(w32):
    ncols = w32.shape[1]
    nv = D // 16
    v = [w32[i * 8:(i + 1) * 8, :] for i in range(nv)]
    sub = lax.broadcasted_iota(jnp.int32, (8, ncols), 0)
    for vb, sh in ((8, 2), (16, 4)):
        low = (sub & sh) == 0
        for a in range(nv):
            if a & vb:
                continue
            c = a | vb
            ta, tc = v[a], v[c]
            v[a] = jnp.where(low, ta, pltpu.roll(tc, sh, 0))
            v[c] = jnp.where(low, pltpu.roll(ta, 8 - sh, 0), tc)
    def src(i):
        b0, b5 = i & 1, (i >> 5) & 1
        return (i & ~33) | (b0 << 5) | b5
    return jnp.concatenate([v[src(i)] for i in range(nv)], axis=0)


def _group_sum4(x, lane):
    b0 = (lane & 1) == 0
    x = x + jnp.where(b0, pltpu.roll(x, 127, 1), pltpu.roll(x, 1, 1))
    b1 = (lane & 2) == 0
    return x + jnp.where(b1, pltpu.roll(x, 126, 1), pltpu.roll(x, 2, 1))


def _pack(x):
    return pltpu.bitcast(x.astype(BF16), U32)


def _unpack(x):
    return pltpu.bitcast(x, BF16)


def _ipack(x):
    r, c = x.shape
    x4 = x.reshape(r // 16, 2, 8, c)
    lo = x4[:, 0].reshape(r // 2, c)
    hi = x4[:, 1].reshape(r // 2, c)
    return pltpu.bitcast(pltpu.pack_elementwise([lo, hi], packed_dtype=BF16), U32)


def _kernel(x_hbm, wa_hbm, woa_hbm, wb_hbm, wob_hbm, out_hbm,
            xio, xres, xsave, wst, wost, wst2, wost2, wa, woa, wb, wob, hb, h2b, ob, qbuf0, qbuf1, zref, kbuf, vbuf,
            qs, ks, vt, ots, pb0, pb1, pb2, pb3, wsems, sems, osems):
    nblk = S // BM
    qbuf = (qbuf0, qbuf1)
    pbufs = (pb0, pb1, pb2, pb3)
    zref[0] = 0
    nch = BM // CM
    pr = 128
    nwc = D // pr

    def wa_copy(c):
        r = pl.multiple_of(c * pr, pr)
        return pltpu.make_async_copy(wa_hbm.at[pl.ds(r, pr), :], wst.at[pl.ds(r, pr), :],
                                     wsems.at[c])

    def x_copy(r0, n, k):
        return pltpu.make_async_copy(x_hbm.at[pl.ds(r0, n), :], xio.at[pl.ds(r0, n), :], sems.at[k])

    cp_woa = pltpu.make_async_copy(woa_hbm, wost, sems.at[0])
    cp_x0 = x_copy(0, BM, 1)
    cp_wb = pltpu.make_async_copy(wb_hbm, wst2, sems.at[2])
    cp_x1 = x_copy(BM, BM, 3)
    cp_x2 = x_copy(2 * BM, S - 2 * BM, 4)
    cp_wob = pltpu.make_async_copy(wob_hbm, wost2, sems.at[5])
    ahead = 3
    for c in range(ahead):
        wa_copy(c).start()

    for t in range(NT):
        kbuf[t, BM:BM + HALO, :] = jnp.zeros((HALO, 128), F32)
        vbuf[t, BM:BM + HALO, :] = jnp.zeros((HALO, 128), F32)

    def perm_body(c, carry):
        wa_copy(c).wait()

        @pl.when(c + ahead < nwc)
        def _():
            wa_copy(jnp.minimum(c + ahead, nwc - 1)).start()

        @pl.when(c + ahead == nwc)
        def _():
            cp_woa.start()

        @pl.when(c + ahead == nwc + 1)
        def _():
            cp_x0.start()

        r = pl.multiple_of(c * pr, pr)
        r2 = pl.multiple_of(c * (pr // 2), pr // 2)
        for sec in range(3):
            w32 = _pack(wst[pl.ds(r, pr), sec * D:(sec + 1) * D])
            wa[pl.ds(r2, pr // 2), sec * D:(sec + 1) * D] = _permute_cols(w32)
        return carry

    with jax.named_scope("perm_cols"):
        lax.fori_loop(0, nwc, perm_body, 0)

    with jax.named_scope("perm_rows"):
        cp_woa.wait()
        cp_wb.start()
        cp_x1.start()

        def permo_body(i, carry):
            c0 = pl.multiple_of(i * 128, 128)
            woa[:, pl.ds(c0, 128)] = _permute_rows(_pack(wost[:, pl.ds(c0, 128)]))
            return carry

        lax.fori_loop(0, NT, permo_body, 0)

    def widen_x(r0, nrows):
        step = 64

        def body(i, carry):
            r = pl.multiple_of(r0 + i * step, step)
            xres[pl.ds(r, step), :] = xio[pl.ds(r, step), :].astype(F32)
            return carry

        lax.fori_loop(0, nrows // step, body, 0)

    def repack(src, dst):
        step = 64

        def body(i, carry):
            r = pl.multiple_of(i * step, step)
            r2 = pl.multiple_of(i * (step // 2), step // 2)
            dst[pl.ds(r2, step // 2), :] = _pack(src[pl.ds(r, step), :])
            return carry

        lax.fori_loop(0, D // step, body, 0)

    with jax.named_scope("x_in"):
        cp_x0.wait()
        widen_x(0, BM)

    lane = lax.broadcasted_iota(jnp.int32, (RG, 128), 1)
    rowi = lax.broadcasted_iota(jnp.int32, (RG, 128), 0)

    def tile_dot(lhs_ref, w_ref, n):
        return jnp.dot(_unpack(lhs_ref[...]), _unpack(w_ref[:, n * NC:(n + 1) * NC]),
                       preferred_element_type=F32)

    tpc = NC // 128

    def local_qkv(h_ref, off, i, lo=0, hi=3 * D // NC):
        for n in (list(range(D // NC, 3 * D // NC)) + list(range(D // NC)))[lo:hi]:
            res = tile_dot(h_ref, wa, n)
            for u in range(tpc):
                sec, t = divmod(n * tpc + u, NT)
                val = res[:, u * 128:(u + 1) * 128]
                if sec == 0:
                    qbuf[off // CM][t, 0:CM, :] = val
                elif sec == 1:
                    kbuf[t, HALO + off:HALO + off + CM, :] = val
                else:
                    vbuf[t, HALO + off:HALO + off + CM, :] = val
                    if off == 0:
                        first = jnp.broadcast_to(val[0:1, :], (HALO, 128))
                        vbuf[t, 0:HALO, :] = jnp.where(i == 0, first, vbuf[t, 0:HALO, :])

    def local_attn(o_ref, off, i):
        zero = zref[0]
        for g in range(CM // RG):
            base = HALO + off + g * RG
            qg = [qbuf[off // CM][t, pl.ds(pl.multiple_of(zero + g * RG, RG), RG), :] for t in range(NT)]
            logit = []
            for w in range(WIN):
                a = base - DIL * w
                part = qg[0] * kbuf[0, a:a + RG, :]
                for t in range(1, NT):
                    part = part + qg[t] * kbuf[t, a:a + RG, :]
                lg = _group_sum4(part, lane) * QSCALE
                if off == 0 and g == 0 and w > 0:
                    lg = jnp.where(rowi + i * BM >= DIL * w, lg, MASKED)
                logit.append(lg)
            m = functools.reduce(jnp.maximum, logit)
            p = [jnp.exp2(lg - m) for lg in logit]
            inv = 1.0 / functools.reduce(lambda u, v: u + v, p)
            for t in range(NT):
                acc = p[0] * vbuf[t, base:base + RG, :]
                for w in range(1, WIN):
                    a = base - DIL * w
                    acc = acc + p[w] * vbuf[t, a:a + RG, :]
                o_ref[g * RG // 2:(g + 1) * RG // 2, t * 128:(t + 1) * 128] = _pack(acc * inv)

    def full_qkv(h_ref, r, lo=0, hi=3 * D // NC):
        r2 = pl.multiple_of(r // 2, CM // 2)
        order = list(range(2 * D // NC, 3 * D // NC)) + list(range(2 * D // NC))
        for n in order[lo:hi]:
            res = tile_dot(h_ref, wb, n)
            for u in range(tpc):
                sec, t = divmod(n * tpc + u, NT)
                val = res[:, u * 128:(u + 1) * 128]
                if sec == 0:
                    qs[t, pl.ds(r2, CM // 2), :] = _pack(val * QSCALE)
                elif sec == 1:
                    ks[t, pl.ds(r2, CM // 2), :] = _pack(val)
                else:
                    vt[t * 64:(t + 1) * 64, pl.ds(r, CM)] = pltpu.bitcast(_unpack(_ipack(val)).T, U32)

    def row_phase(pair):
        hb[0] = _pack(_layernorm(xres[0:CM, :]))

        def body(i, c):
            @pl.when(jnp.logical_and(pair == 0, i == 1))
            def _():
                cp_x2.wait()
                cp_wob.wait()
                repack(wost2, wob)

            r0 = pl.multiple_of(i * BM, BM)
            rs = [pl.multiple_of(r0 + ch * CM, CM) for ch in range(nch)]
            for t in range(NT):
                kbuf[t, 0:HALO, :] = kbuf[t, BM:BM + HALO, :]
                vbuf[t, 0:HALO, :] = vbuf[t, BM:BM + HALO, :]
            rn = pl.multiple_of(jnp.minimum(i + 1, nblk - 1) * BM, BM)

            def local_out(ch):
                local_attn(ob.at[ch], ch * CM, i)
                y = jnp.concatenate([tile_dot(ob.at[ch], woa, n) for n in range(D // NC)], axis=1)
                x2 = xres[pl.ds(rs[ch], CM), :] + y
                xres[pl.ds(rs[ch], CM), :] = x2
                xsave[pl.ds(rs[ch], CM), :] = x2
                h2b[ch] = _pack(_layernorm(x2))

            hb[1] = _pack(_layernorm(xres[pl.ds(rs[1], CM), :]))
            local_qkv(hb.at[0], 0, i)
            local_qkv(hb.at[1], CM, i, 0, SPLIT1)
            local_out(0)
            local_qkv(hb.at[1], CM, i, SPLIT1)

            @pl.when(jnp.logical_and(pair == 0, i == 0))
            def _():
                cp_wb.wait()
                cp_x2.start()
                cp_wob.start()
                repack(wst2, wb)
                cp_x1.wait()

            full_qkv(h2b.at[0], rs[0], 0, SPLIT2)
            local_out(1)
            full_qkv(h2b.at[0], rs[0], SPLIT2)
            full_qkv(h2b.at[1], rs[1], 0, 10)
            fresh = jnp.logical_and(pair == 0, i + 1 < nblk)
            xn = jnp.where(fresh, xio[pl.ds(rn, BM), :].astype(F32), xres[pl.ds(rn, BM), :])
            xres[pl.ds(rn, BM), :] = xn
            hb[0] = _pack(_layernorm(xn[0:CM, :]))
            full_qkv(h2b.at[1], rs[1], 10)
            return c

        with jax.named_scope("row_phase"):
            lax.fori_loop(0, nblk, body, 0)

    early = QB // OB

    def out_copy(i):
        r0 = pl.multiple_of(i * OB, OB)
        return pltpu.make_async_copy(xio.at[pl.ds(r0, OB), :], out_hbm.at[pl.ds(r0, OB), :],
                                     osems.at[i])

    def write_out(lo, hi):
        def body(i, c):
            r0 = pl.multiple_of(i * OB, OB)
            xio[pl.ds(r0, OB), :] = xres[pl.ds(r0, OB), :].astype(BF16)
            out_copy(i).start()
            return c

        lax.fori_loop(lo, hi, body, 0)

    nt_dims = (((1,), (1,)), ((), ()))

    def masked_q(q32, hp):
        head = lax.broadcasted_iota(jnp.int32, q32.shape, 1) // DH
        return _unpack(jnp.where(head == hp, q32, jnp.uint32(0)))

    def add_oproj(ot, g, q0, nq):
        g64 = pl.multiple_of(g * 64, 64)
        for j in range(nq // OS):
            y = jnp.dot(ot[:, j * OS:(j + 1) * OS].T.astype(BF16), _unpack(wob[pl.ds(g64, 64), :]),
                        preferred_element_type=F32)
            r = pl.multiple_of(q0 + j * OS, OS)
            xres[pl.ds(r, OS), :] = xres[pl.ds(r, OS), :] + y

    def full_attn(pair):
        nqb = S // QB

        def body(it, bad):
            @pl.when(jnp.logical_and(pair == 1, it == NT))
            def _():
                write_out(0, early)

            g = it % NT
            q0 = pl.multiple_of((it // NT) * QB, QB)
            q32 = qs[g, pl.ds(pl.multiple_of(q0 // 2, QB // 2), QB // 2), :]
            zero = zref[0]
            acc = [None] * HPT
            l8 = [None] * HPT

            def pv(hp, t, buf):
                r0 = pl.multiple_of(g * 64 + hp * (DH // 2), DH // 2)
                vc = _unpack(vt[pl.ds(r0, DH // 2), t * KC:(t + 1) * KC])
                a = jnp.dot(vc, _unpack(buf[zero]), preferred_element_type=F32)
                acc[hp] = a if acc[hp] is None else acc[hp] + a

            pending = None
            for hp in range(HPT):
                w = masked_q(q32, hp)
                for t in range(S // KC):
                    kc = _unpack(ks[g, t * KC // 2:(t + 1) * KC // 2, :])
                    p = jnp.exp2(lax.dot_general(kc, w, nt_dims, preferred_element_type=F32))
                    part = jnp.sum(p.reshape(KC // 8, 8, QB), axis=0)
                    l8[hp] = part if l8[hp] is None else l8[hp] + part
                    buf = pbufs[(hp * (S // KC) + t) % len(pbufs)]
                    buf[0] = _ipack(p)
                    if pending is not None:
                        pv(*pending)
                    pending = (hp, t, buf)
            pv(*pending)
            outs = []
            for hp in range(HPT):
                l = jnp.sum(l8[hp], axis=0, keepdims=True)
                o = acc[hp] * (1.0 / l)
                outs.append(o)
                ok = (jnp.abs(o) < O_HI) & (l > L_LO) & (l < L_HI)
                nbad = jnp.where(ok, 0.0, 1.0)
                bad = jnp.maximum(bad, jnp.max(nbad.reshape(DH // 8, 8, QB), axis=0))
            add_oproj(jnp.concatenate(outs, axis=0), g, q0, QB)
            return bad

        with jax.named_scope("full_attn"):
            bad = lax.fori_loop(0, NT * nqb, body, jnp.zeros((8, QB), F32))

        @pl.when(jnp.max(bad) > 0.0)
        def _():
            nq = S // FQ

            def restore(i, c):
                r = pl.multiple_of(i * 32, 32)
                xres[pl.ds(r, 32), :] = xsave[pl.ds(r, 32), :]
                return c

            lax.fori_loop(0, S // 32, restore, 0)

            def fb_body(it, c):
                g = it // nq
                q0 = pl.multiple_of((it % nq) * FQ, FQ)
                q32 = qs[g, pl.ds(pl.multiple_of(q0 // 2, FQ // 2), FQ // 2), :]

                def head_body(hp, c2):
                    r0 = pl.multiple_of(g * 64 + hp * (DH // 2), DH // 2)
                    s = lax.dot_general(_unpack(ks[g]), masked_q(q32, hp), nt_dims,
                                        preferred_element_type=F32)
                    p = jnp.exp2(s - jnp.max(s, axis=0, keepdims=True))
                    l = jnp.sum(p, axis=0, keepdims=True)
                    acc = jnp.dot(_unpack(vt[pl.ds(r0, DH // 2), :]), _unpack(_ipack(p)),
                                  preferred_element_type=F32)
                    ots[pl.ds(pl.multiple_of(hp * DH, DH), DH), :] = acc * (1.0 / l)
                    return c2

                lax.fori_loop(0, HPT, head_body, 0)
                add_oproj(ots[...], g, q0, FQ)
                return c

            lax.fori_loop(0, NT * nq, fb_body, 0)

            @pl.when(pair == 1)
            def _():
                for i in range(early):
                    out_copy(i).wait()
                write_out(0, early)

    def pair_body(pair, c):
        row_phase(pair)
        full_attn(pair)
        return c

    with jax.named_scope("pairs"):
        lax.fori_loop(0, 2, pair_body, 0)

    with jax.named_scope("out_phase"):
        write_out(early, S // OB)
        for i in range(S // OB):
            out_copy(i).wait()


@jax.jit
def pallas_interleave_layers__sliding_local_dilated__softmax_full_mha__prompt_kernel(
    A_x: jax.Array,
    A_wqkv: jax.Array,
    A_wo: jax.Array,
    B_x: jax.Array,
    B_wqkv: jax.Array,
    B_wo: jax.Array,
):
    del B_x
    x = A_x.reshape(S, D)
    hbm = pl.BlockSpec(memory_space=pl.ANY)
    out = pl.pallas_call(
        _kernel,
        out_shape=jax.ShapeDtypeStruct((S, D), BF16),
        in_specs=[hbm] * 5,
        out_specs=hbm,
        scratch_shapes=[
            pltpu.VMEM((S, D), BF16),
            pltpu.VMEM((S, D), F32),
            pltpu.VMEM((S, D), F32),
            pltpu.VMEM((D, 3 * D), BF16),
            pltpu.VMEM((D, D), BF16),
            pltpu.VMEM((D, 3 * D), BF16),
            pltpu.VMEM((D, D), BF16),
            pltpu.VMEM((D // 2, 3 * D), U32),
            pltpu.VMEM((D // 2, D), U32),
            pltpu.VMEM((D // 2, 3 * D), U32),
            pltpu.VMEM((D // 2, D), U32),
            pltpu.VMEM((BM // CM, CM // 2, D), U32),
            pltpu.VMEM((BM // CM, CM // 2, D), U32),
            pltpu.VMEM((BM // CM, CM // 2, D), U32),
            pltpu.VMEM((NT, CM + 8, 128), F32),
            pltpu.VMEM((NT, CM + 8, 128), F32),
            pltpu.SMEM((1,), jnp.int32),
            pltpu.VMEM((NT, HALO + BM, 128), F32),
            pltpu.VMEM((NT, HALO + BM, 128), F32),
            pltpu.VMEM((NT, S // 2, 128), U32),
            pltpu.VMEM((NT, S // 2, 128), U32),
            pltpu.VMEM((D // 2, S), U32),
            pltpu.VMEM((128, FQ), F32),
            pltpu.VMEM((1, KC // 2, QB), U32),
            pltpu.VMEM((1, KC // 2, QB), U32),
            pltpu.VMEM((1, KC // 2, QB), U32),
            pltpu.VMEM((1, KC // 2, QB), U32),
            pltpu.SemaphoreType.DMA((D // 128,)),
            pltpu.SemaphoreType.DMA((6,)),
            pltpu.SemaphoreType.DMA((S // OB,)),
        ],
        compiler_params=pltpu.CompilerParams(vmem_limit_bytes=110 * 1024 * 1024),
        name="interleaved_attention_stack",
    )(x, A_wqkv, A_wo, B_wqkv, B_wo)
    return out.reshape(1, S, D)
```

```python
import functools
import math

import jax
import jax.numpy as jnp
from jax import lax
import jax.experimental.pallas as pl
import jax.experimental.pallas.tpu as pltpu

S = 2048
D = 1024
H = 32
DH = D // H
NT = D // 128
HPT = 128 // DH
WIN = 8
DIL = 2
HALO = 16
EPS = 1e-5
LOG2E = math.log2(math.e)
QSCALE = (DH ** -0.5) * LOG2E
MASKED = -1e9 * LOG2E

BM = 256
CM = 128
NC = 128
SPLIT1 = 16
SPLIT2 = 16
RG = 16
KC = 512
QB = 1024
OS = 128
OB = 128
FQ = 128

L_LO = 2.0 ** -40
L_HI = 2.0 ** 90
O_HI = 3.0e38

F32 = jnp.float32
BF16 = jnp.bfloat16
U32 = jnp.uint32


def _layernorm(x):
    mu = jnp.mean(x, axis=-1, keepdims=True)
    xc = x - mu
    var = jnp.mean(xc * xc, axis=-1, keepdims=True)
    return xc * lax.rsqrt(var + EPS)


def _permute_cols(w32):
    rows = w32.shape[0]
    lane = lax.broadcasted_iota(jnp.int32, (rows, 128), 1)
    tiles = [w32[:, t * 128:(t + 1) * 128] for t in range(NT)]
    for b in range(3):
        sh = 4 << b
        low = (lane & sh) == 0
        for a in range(NT):
            if a & (1 << b):
                continue
            c = a | (1 << b)
            ta, tc = tiles[a], tiles[c]
            tiles[a] = jnp.where(low, ta, pltpu.roll(tc, sh, 1))
            tiles[c] = jnp.where(low, pltpu.roll(ta, 128 - sh, 1), tc)
    return jnp.concatenate(tiles, axis=1)


def _permute_rows(w32):
    ncols = w32.shape[1]
    nv = D // 16
    v = [w32[i * 8:(i + 1) * 8, :] for i in range(nv)]
    sub = lax.broadcasted_iota(jnp.int32, (8, ncols), 0)
    for vb, sh in ((8, 2), (16, 4)):
        low = (sub & sh) == 0
        for a in range(nv):
            if a & vb:
                continue
            c = a | vb
            ta, tc = v[a], v[c]
            v[a] = jnp.where(low, ta, pltpu.roll(tc, sh, 0))
            v[c] = jnp.where(low, pltpu.roll(ta, 8 - sh, 0), tc)
    def src(i):
        b0, b5 = i & 1, (i >> 5) & 1
        return (i & ~33) | (b0 << 5) | b5
    return jnp.concatenate([v[src(i)] for i in range(nv)], axis=0)


def _group_sum4(x, lane):
    b0 = (lane & 1) == 0
    x = x + jnp.where(b0, pltpu.roll(x, 127, 1), pltpu.roll(x, 1, 1))
    b1 = (lane & 2) == 0
    return x + jnp.where(b1, pltpu.roll(x, 126, 1), pltpu.roll(x, 2, 1))


def _pack(x):
    return pltpu.bitcast(x.astype(BF16), U32)


def _unpack(x):
    return pltpu.bitcast(x, BF16)


def _kernel(x_hbm, wa_hbm, woa_hbm, wb_hbm, wob_hbm, out_hbm,
            xio, xres, xsave, wst, wost, wst2, wost2, wa, woa, wb, wob, hb, h2b, ob, qbuf0, qbuf1, zref, kbuf, vbuf,
            qs, ks, vt, ots, pb0, pb1, pb2, pb3, wsems, sems, osems):
    nblk = S // BM
    qbuf = (qbuf0, qbuf1)
    pbufs = (pb0, pb1, pb2, pb3)
    zref[0] = 0
    nch = BM // CM
    pr = 128
    nwc = D // pr

    def wa_copy(c):
        r = pl.multiple_of(c * pr, pr)
        return pltpu.make_async_copy(wa_hbm.at[pl.ds(r, pr), :], wst.at[pl.ds(r, pr), :],
                                     wsems.at[c])

    def x_copy(r0, n, k):
        return pltpu.make_async_copy(x_hbm.at[pl.ds(r0, n), :], xio.at[pl.ds(r0, n), :], sems.at[k])

    cp_woa = pltpu.make_async_copy(woa_hbm, wost, sems.at[0])
    cp_x0 = x_copy(0, BM, 1)
    cp_wb = pltpu.make_async_copy(wb_hbm, wst2, sems.at[2])
    cp_x1 = x_copy(BM, BM, 3)
    cp_x2 = x_copy(2 * BM, S - 2 * BM, 4)
    cp_wob = pltpu.make_async_copy(wob_hbm, wost2, sems.at[5])
    ahead = 3
    for c in range(ahead):
        wa_copy(c).start()

    for t in range(NT):
        kbuf[t, BM:BM + HALO, :] = jnp.zeros((HALO, 128), F32)
        vbuf[t, BM:BM + HALO, :] = jnp.zeros((HALO, 128), F32)

    def perm_body(c, carry):
        wa_copy(c).wait()

        @pl.when(c + ahead < nwc)
        def _():
            wa_copy(jnp.minimum(c + ahead, nwc - 1)).start()

        @pl.when(c + ahead == nwc)
        def _():
            cp_woa.start()

        @pl.when(c + ahead == nwc + 1)
        def _():
            cp_x0.start()

        r = pl.multiple_of(c * pr, pr)
        r2 = pl.multiple_of(c * (pr // 2), pr // 2)
        for sec in range(3):
            w32 = _pack(wst[pl.ds(r, pr), sec * D:(sec + 1) * D])
            wa[pl.ds(r2, pr // 2), sec * D:(sec + 1) * D] = _permute_cols(w32)
        return carry

    with jax.named_scope("perm_cols"):
        lax.fori_loop(0, nwc, perm_body, 0)

    with jax.named_scope("perm_rows"):
        cp_woa.wait()
        cp_wb.start()
        cp_x1.start()

        def permo_body(i, carry):
            c0 = pl.multiple_of(i * 128, 128)
            woa[:, pl.ds(c0, 128)] = _permute_rows(_pack(wost[:, pl.ds(c0, 128)]))
            return carry

        lax.fori_loop(0, NT, permo_body, 0)

    def widen_x(r0, nrows):
        step = 64

        def body(i, carry):
            r = pl.multiple_of(r0 + i * step, step)
            xres[pl.ds(r, step), :] = xio[pl.ds(r, step), :].astype(F32)
            return carry

        lax.fori_loop(0, nrows // step, body, 0)

    def repack(src, dst):
        step = 64

        def body(i, carry):
            r = pl.multiple_of(i * step, step)
            r2 = pl.multiple_of(i * (step // 2), step // 2)
            dst[pl.ds(r2, step // 2), :] = _pack(src[pl.ds(r, step), :])
            return carry

        lax.fori_loop(0, D // step, body, 0)

    with jax.named_scope("x_in"):
        cp_x0.wait()
        widen_x(0, BM)

    lane = lax.broadcasted_iota(jnp.int32, (RG, 128), 1)
    rowi = lax.broadcasted_iota(jnp.int32, (RG, 128), 0)

    def tile_dot(lhs_ref, w_ref, n):
        return jnp.dot(_unpack(lhs_ref[...]), _unpack(w_ref[:, n * NC:(n + 1) * NC]),
                       preferred_element_type=F32)

    tpc = NC // 128

    def local_qkv(h_ref, off, i, lo=0, hi=3 * D // NC):
        for n in (list(range(D // NC, 3 * D // NC)) + list(range(D // NC)))[lo:hi]:
            res = tile_dot(h_ref, wa, n)
            for u in range(tpc):
                sec, t = divmod(n * tpc + u, NT)
                val = res[:, u * 128:(u + 1) * 128]
                if sec == 0:
                    qbuf[off // CM][t, 0:CM, :] = val
                elif sec == 1:
                    kbuf[t, HALO + off:HALO + off + CM, :] = val
                else:
                    vbuf[t, HALO + off:HALO + off + CM, :] = val
                    if off == 0:
                        first = jnp.broadcast_to(val[0:1, :], (HALO, 128))
                        vbuf[t, 0:HALO, :] = jnp.where(i == 0, first, vbuf[t, 0:HALO, :])

    def local_attn(o_ref, off, i):
        zero = zref[0]
        for g in range(CM // RG):
            base = HALO + off + g * RG
            qg = [qbuf[off // CM][t, pl.ds(pl.multiple_of(zero + g * RG, RG), RG), :] for t in range(NT)]
            logit = []
            for w in range(WIN):
                a = base - DIL * w
                part = qg[0] * kbuf[0, a:a + RG, :]
                for t in range(1, NT):
                    part = part + qg[t] * kbuf[t, a:a + RG, :]
                lg = _group_sum4(part, lane) * QSCALE
                if off == 0 and g == 0 and w > 0:
                    lg = jnp.where(rowi + i * BM >= DIL * w, lg, MASKED)
                logit.append(lg)
            m = functools.reduce(jnp.maximum, logit)
            p = [jnp.exp2(lg - m) for lg in logit]
            inv = 1.0 / functools.reduce(lambda u, v: u + v, p)
            for t in range(NT):
                acc = p[0] * vbuf[t, base:base + RG, :]
                for w in range(1, WIN):
                    a = base - DIL * w
                    acc = acc + p[w] * vbuf[t, a:a + RG, :]
                o_ref[g * RG // 2:(g + 1) * RG // 2, t * 128:(t + 1) * 128] = _pack(acc * inv)

    def full_qkv(h_ref, r, lo=0, hi=3 * D // NC):
        r2 = pl.multiple_of(r // 2, CM // 2)
        order = list(range(2 * D // NC, 3 * D // NC)) + list(range(2 * D // NC))
        for n in order[lo:hi]:
            res = tile_dot(h_ref, wb, n)
            for u in range(tpc):
                sec, t = divmod(n * tpc + u, NT)
                val = res[:, u * 128:(u + 1) * 128]
                if sec == 0:
                    qs[t, pl.ds(r2, CM // 2), :] = _pack(val * QSCALE)
                elif sec == 1:
                    ks[t, pl.ds(r2, CM // 2), :] = _pack(val)
                else:
                    vt[t * 64:(t + 1) * 64, pl.ds(r, CM)] = _pack(val.T)

    def row_phase(pair):
        hb[0] = _pack(_layernorm(xres[0:CM, :]))

        def body(i, c):
            @pl.when(jnp.logical_and(pair == 0, i == 1))
            def _():
                cp_x2.wait()
                cp_wob.wait()
                repack(wost2, wob)

            r0 = pl.multiple_of(i * BM, BM)
            rs = [pl.multiple_of(r0 + ch * CM, CM) for ch in range(nch)]
            for t in range(NT):
                kbuf[t, 0:HALO, :] = kbuf[t, BM:BM + HALO, :]
                vbuf[t, 0:HALO, :] = vbuf[t, BM:BM + HALO, :]
            rn = pl.multiple_of(jnp.minimum(i + 1, nblk - 1) * BM, BM)

            def local_out(ch):
                local_attn(ob.at[ch], ch * CM, i)
                y = jnp.concatenate([tile_dot(ob.at[ch], woa, n) for n in range(D // NC)], axis=1)
                x2 = xres[pl.ds(rs[ch], CM), :] + y
                xres[pl.ds(rs[ch], CM), :] = x2
                xsave[pl.ds(rs[ch], CM), :] = x2
                h2b[ch] = _pack(_layernorm(x2))

            hb[1] = _pack(_layernorm(xres[pl.ds(rs[1], CM), :]))
            local_qkv(hb.at[0], 0, i)
            local_qkv(hb.at[1], CM, i, 0, SPLIT1)
            local_out(0)
            local_qkv(hb.at[1], CM, i, SPLIT1)

            @pl.when(jnp.logical_and(pair == 0, i == 0))
            def _():
                cp_wb.wait()
                cp_x2.start()
                cp_wob.start()
                repack(wst2, wb)
                cp_x1.wait()

            full_qkv(h2b.at[0], rs[0], 0, SPLIT2)
            local_out(1)
            full_qkv(h2b.at[0], rs[0], SPLIT2)
            full_qkv(h2b.at[1], rs[1], 0, 10)
            fresh = jnp.logical_and(pair == 0, i + 1 < nblk)
            xn = jnp.where(fresh, xio[pl.ds(rn, BM), :].astype(F32), xres[pl.ds(rn, BM), :])
            xres[pl.ds(rn, BM), :] = xn
            hb[0] = _pack(_layernorm(xn[0:CM, :]))
            full_qkv(h2b.at[1], rs[1], 10)
            return c

        with jax.named_scope("row_phase"):
            lax.fori_loop(0, nblk, body, 0)

    early = QB // OB

    def out_copy(i):
        r0 = pl.multiple_of(i * OB, OB)
        return pltpu.make_async_copy(xio.at[pl.ds(r0, OB), :], out_hbm.at[pl.ds(r0, OB), :],
                                     osems.at[i])

    def write_out(lo, hi):
        def body(i, c):
            r0 = pl.multiple_of(i * OB, OB)
            xio[pl.ds(r0, OB), :] = xres[pl.ds(r0, OB), :].astype(BF16)
            out_copy(i).start()
            return c

        lax.fori_loop(lo, hi, body, 0)

    nt_dims = (((1,), (1,)), ((), ()))

    def masked_q(q32, hp):
        head = lax.broadcasted_iota(jnp.int32, q32.shape, 1) // DH
        return _unpack(jnp.where(head == hp, q32, jnp.uint32(0)))

    def add_oproj(ot, g, q0, nq):
        g64 = pl.multiple_of(g * 64, 64)
        for j in range(nq // OS):
            y = jnp.dot(ot[:, j * OS:(j + 1) * OS].T.astype(BF16), _unpack(wob[pl.ds(g64, 64), :]),
                        preferred_element_type=F32)
            r = pl.multiple_of(q0 + j * OS, OS)
            xres[pl.ds(r, OS), :] = xres[pl.ds(r, OS), :] + y

    def full_attn(pair):
        nqb = S // QB

        def body(it, bad):
            @pl.when(jnp.logical_and(pair == 1, it == NT))
            def _():
                write_out(0, early)

            g = it % NT
            q0 = pl.multiple_of((it // NT) * QB, QB)
            q32 = qs[g, pl.ds(pl.multiple_of(q0 // 2, QB // 2), QB // 2), :]
            zero = zref[0]
            acc = [None] * HPT
            l8 = [None] * HPT

            def pv(hp, t, buf):
                r0 = pl.multiple_of(g * 64 + hp * (DH // 2), DH // 2)
                vc = _unpack(vt[pl.ds(r0, DH // 2), t * KC:(t + 1) * KC])
                a = jnp.dot(vc, _unpack(buf[zero]), preferred_element_type=F32)
                acc[hp] = a if acc[hp] is None else acc[hp] + a

            pending = None
            for hp in range(HPT):
                w = masked_q(q32, hp)
                for t in range(S // KC):
                    kc = _unpack(ks[g, t * KC // 2:(t + 1) * KC // 2, :])
                    p = jnp.exp2(lax.dot_general(kc, w, nt_dims, preferred_element_type=F32))
                    part = jnp.sum(p.reshape(KC // 8, 8, QB), axis=0)
                    l8[hp] = part if l8[hp] is None else l8[hp] + part
                    buf = pbufs[(hp * (S // KC) + t) % len(pbufs)]
                    buf[0] = _pack(p)
                    if pending is not None:
                        pv(*pending)
                    pending = (hp, t, buf)
            pv(*pending)
            outs = []
            for hp in range(HPT):
                l = jnp.sum(l8[hp], axis=0, keepdims=True)
                o = acc[hp] * (1.0 / l)
                outs.append(o)
                ok = (jnp.abs(o) < O_HI) & (l > L_LO) & (l < L_HI)
                nbad = jnp.where(ok, 0.0, 1.0)
                bad = jnp.maximum(bad, jnp.max(nbad.reshape(DH // 8, 8, QB), axis=0))
            add_oproj(jnp.concatenate(outs, axis=0), g, q0, QB)
            return bad

        with jax.named_scope("full_attn"):
            bad = lax.fori_loop(0, NT * nqb, body, jnp.zeros((8, QB), F32))

        @pl.when(jnp.max(bad) > 0.0)
        def _():
            nq = S // FQ

            def restore(i, c):
                r = pl.multiple_of(i * 32, 32)
                xres[pl.ds(r, 32), :] = xsave[pl.ds(r, 32), :]
                return c

            lax.fori_loop(0, S // 32, restore, 0)

            def fb_body(it, c):
                g = it // nq
                q0 = pl.multiple_of((it % nq) * FQ, FQ)
                q32 = qs[g, pl.ds(pl.multiple_of(q0 // 2, FQ // 2), FQ // 2), :]

                def head_body(hp, c2):
                    r0 = pl.multiple_of(g * 64 + hp * (DH // 2), DH // 2)
                    s = lax.dot_general(_unpack(ks[g]), masked_q(q32, hp), nt_dims,
                                        preferred_element_type=F32)
                    p = jnp.exp2(s - jnp.max(s, axis=0, keepdims=True))
                    l = jnp.sum(p, axis=0, keepdims=True)
                    acc = jnp.dot(_unpack(vt[pl.ds(r0, DH // 2), :]), p.astype(BF16),
                                  preferred_element_type=F32)
                    ots[pl.ds(pl.multiple_of(hp * DH, DH), DH), :] = acc * (1.0 / l)
                    return c2

                lax.fori_loop(0, HPT, head_body, 0)
                add_oproj(ots[...], g, q0, FQ)
                return c

            lax.fori_loop(0, NT * nq, fb_body, 0)

            @pl.when(pair == 1)
            def _():
                for i in range(early):
                    out_copy(i).wait()
                write_out(0, early)

    def pair_body(pair, c):
        row_phase(pair)
        full_attn(pair)
        return c

    with jax.named_scope("pairs"):
        lax.fori_loop(0, 2, pair_body, 0)

    with jax.named_scope("out_phase"):
        write_out(early, S // OB)
        for i in range(S // OB):
            out_copy(i).wait()


@jax.jit
def pallas_interleave_layers__sliding_local_dilated__softmax_full_mha__prompt_kernel(
    A_x: jax.Array,
    A_wqkv: jax.Array,
    A_wo: jax.Array,
    B_x: jax.Array,
    B_wqkv: jax.Array,
    B_wo: jax.Array,
):
    del B_x
    x = A_x.reshape(S, D)
    hbm = pl.BlockSpec(memory_space=pl.ANY)
    out = pl.pallas_call(
        _kernel,
        out_shape=jax.ShapeDtypeStruct((S, D), BF16),
        in_specs=[hbm] * 5,
        out_specs=hbm,
        scratch_shapes=[
            pltpu.VMEM((S, D), BF16),
            pltpu.VMEM((S, D), F32),
            pltpu.VMEM((S, D), F32),
            pltpu.VMEM((D, 3 * D), BF16),
            pltpu.VMEM((D, D), BF16),
            pltpu.VMEM((D, 3 * D), BF16),
            pltpu.VMEM((D, D), BF16),
            pltpu.VMEM((D // 2, 3 * D), U32),
            pltpu.VMEM((D // 2, D), U32),
            pltpu.VMEM((D // 2, 3 * D), U32),
            pltpu.VMEM((D // 2, D), U32),
            pltpu.VMEM((BM // CM, CM // 2, D), U32),
            pltpu.VMEM((BM // CM, CM // 2, D), U32),
            pltpu.VMEM((BM // CM, CM // 2, D), U32),
            pltpu.VMEM((NT, CM + 8, 128), F32),
            pltpu.VMEM((NT, CM + 8, 128), F32),
            pltpu.SMEM((1,), jnp.int32),
            pltpu.VMEM((NT, HALO + BM, 128), F32),
            pltpu.VMEM((NT, HALO + BM, 128), F32),
            pltpu.VMEM((NT, S // 2, 128), U32),
            pltpu.VMEM((NT, S // 2, 128), U32),
            pltpu.VMEM((D // 2, S), U32),
            pltpu.VMEM((128, FQ), F32),
            pltpu.VMEM((1, KC // 2, QB), U32),
            pltpu.VMEM((1, KC // 2, QB), U32),
            pltpu.VMEM((1, KC // 2, QB), U32),
            pltpu.VMEM((1, KC // 2, QB), U32),
            pltpu.SemaphoreType.DMA((D // 128,)),
            pltpu.SemaphoreType.DMA((6,)),
            pltpu.SemaphoreType.DMA((S // OB,)),
        ],
        compiler_params=pltpu.CompilerParams(vmem_limit_bytes=110 * 1024 * 1024),
        name="interleaved_attention_stack",
    )(x, A_wqkv, A_wo, B_wqkv, B_wo)
    return out.reshape(1, S, D)
```

```python
import functools
import math

import jax
import jax.numpy as jnp
from jax import lax
import jax.experimental.pallas as pl
import jax.experimental.pallas.tpu as pltpu

S = 2048
D = 1024
H = 32
DH = D // H
NT = D // 128
HPT = 128 // DH
WIN = 8
DIL = 2
HALO = 16
EPS = 1e-5
LOG2E = math.log2(math.e)
QSCALE = (DH ** -0.5) * LOG2E
MASKED = -1e9 * LOG2E

BM = 256
CM = 128
NC = 128
SPLIT1 = 16
SPLIT2 = 16
RG = 16
KC = 512
QB = 1024
OS = 128
WOC = 256
OB = 128
FQ = 128

L_LO = 2.0 ** -40
L_HI = 2.0 ** 90
O_HI = 3.0e38

F32 = jnp.float32
BF16 = jnp.bfloat16
U32 = jnp.uint32


def _layernorm(x):
    mu = jnp.mean(x, axis=-1, keepdims=True)
    xc = x - mu
    var = jnp.mean(xc * xc, axis=-1, keepdims=True)
    return xc * lax.rsqrt(var + EPS)


def _permute_cols(w32):
    rows = w32.shape[0]
    lane = lax.broadcasted_iota(jnp.int32, (rows, 128), 1)
    tiles = [w32[:, t * 128:(t + 1) * 128] for t in range(NT)]
    for b in range(3):
        sh = 4 << b
        low = (lane & sh) == 0
        for a in range(NT):
            if a & (1 << b):
                continue
            c = a | (1 << b)
            ta, tc = tiles[a], tiles[c]
            tiles[a] = jnp.where(low, ta, pltpu.roll(tc, sh, 1))
            tiles[c] = jnp.where(low, pltpu.roll(ta, 128 - sh, 1), tc)
    return jnp.concatenate(tiles, axis=1)


def _permute_rows(w32):
    ncols = w32.shape[1]
    nv = D // 16
    v = [w32[i * 8:(i + 1) * 8, :] for i in range(nv)]
    sub = lax.broadcasted_iota(jnp.int32, (8, ncols), 0)
    for vb, sh in ((8, 2), (16, 4)):
        low = (sub & sh) == 0
        for a in range(nv):
            if a & vb:
                continue
            c = a | vb
            ta, tc = v[a], v[c]
            v[a] = jnp.where(low, ta, pltpu.roll(tc, sh, 0))
            v[c] = jnp.where(low, pltpu.roll(ta, 8 - sh, 0), tc)
    def src(i):
        b0, b5 = i & 1, (i >> 5) & 1
        return (i & ~33) | (b0 << 5) | b5
    return jnp.concatenate([v[src(i)] for i in range(nv)], axis=0)


def _group_sum4(x, lane):
    b0 = (lane & 1) == 0
    x = x + jnp.where(b0, pltpu.roll(x, 127, 1), pltpu.roll(x, 1, 1))
    b1 = (lane & 2) == 0
    return x + jnp.where(b1, pltpu.roll(x, 126, 1), pltpu.roll(x, 2, 1))


def _pack(x):
    return pltpu.bitcast(x.astype(BF16), U32)


def _unpack(x):
    return pltpu.bitcast(x, BF16)


def _kernel(x_hbm, wa_hbm, woa_hbm, wb_hbm, wob_hbm, out_hbm,
            xio, xres, xsave, wst, wost, wst2, wost2, wa, woa, wb, wob, hb, h2b, ob, qbuf0, qbuf1, zref, kbuf, vbuf,
            qs, ks, vt, ots, pb0, pb1, pb2, pb3, wsems, sems, osems):
    nblk = S // BM
    qbuf = (qbuf0, qbuf1)
    pbufs = (pb0, pb1, pb2, pb3)
    zref[0] = 0
    nch = BM // CM
    pr = 128
    nwc = D // pr

    def wa_copy(c):
        r = pl.multiple_of(c * pr, pr)
        return pltpu.make_async_copy(wa_hbm.at[pl.ds(r, pr), :], wst.at[pl.ds(r, pr), :],
                                     wsems.at[c])

    def x_copy(r0, n, k):
        return pltpu.make_async_copy(x_hbm.at[pl.ds(r0, n), :], xio.at[pl.ds(r0, n), :], sems.at[k])

    def woa_copy(t):
        c0 = pl.multiple_of(t * WOC, WOC)
        return pltpu.make_async_copy(woa_hbm.at[:, pl.ds(c0, WOC)], wost.at[:, pl.ds(c0, WOC)],
                                     wsems.at[nwc + t])

    cp_x0 = x_copy(0, BM, 1)
    cp_wb = pltpu.make_async_copy(wb_hbm, wst2, sems.at[2])
    cp_x1 = x_copy(BM, BM, 3)
    cp_x2 = x_copy(2 * BM, S - 2 * BM, 4)
    cp_wob = pltpu.make_async_copy(wob_hbm, wost2, sems.at[5])
    ahead = 3
    for c in range(ahead):
        wa_copy(c).start()

    for t in range(NT):
        kbuf[t, BM:BM + HALO, :] = jnp.zeros((HALO, 128), F32)
        vbuf[t, BM:BM + HALO, :] = jnp.zeros((HALO, 128), F32)

    def perm_body(c, carry):
        wa_copy(c).wait()

        @pl.when(c + ahead < nwc)
        def _():
            wa_copy(jnp.minimum(c + ahead, nwc - 1)).start()

        @pl.when(c + ahead == nwc)
        def _():
            cp_x0.start()

        @pl.when(c + ahead == nwc + 1)
        def _():
            for t in range(D // WOC):
                woa_copy(t).start()

        r = pl.multiple_of(c * pr, pr)
        r2 = pl.multiple_of(c * (pr // 2), pr // 2)
        for sec in range(3):
            w32 = _pack(wst[pl.ds(r, pr), sec * D:(sec + 1) * D])
            wa[pl.ds(r2, pr // 2), sec * D:(sec + 1) * D] = _permute_cols(w32)
        return carry

    with jax.named_scope("perm_cols"):
        lax.fori_loop(0, nwc, perm_body, 0)

    def widen_x(r0, nrows):
        step = 64

        def body(i, carry):
            r = pl.multiple_of(r0 + i * step, step)
            xres[pl.ds(r, step), :] = xio[pl.ds(r, step), :].astype(F32)
            return carry

        lax.fori_loop(0, nrows // step, body, 0)

    def repack(src, dst):
        step = 64

        def body(i, carry):
            r = pl.multiple_of(i * step, step)
            r2 = pl.multiple_of(i * (step // 2), step // 2)
            dst[pl.ds(r2, step // 2), :] = _pack(src[pl.ds(r, step), :])
            return carry

        lax.fori_loop(0, D // step, body, 0)

    with jax.named_scope("x_in"):
        cp_x0.wait()
        widen_x(0, BM)
        hb[0] = _pack(_layernorm(xres[0:CM, :]))

    def permo_body(t, carry):
        woa_copy(t).wait()

        @pl.when(t == 0)
        def _():
            cp_wb.start()
            cp_x1.start()

        for u in range(WOC // 128):
            c0 = pl.multiple_of(t * WOC + u * 128, 128)
            woa[:, pl.ds(c0, 128)] = _permute_rows(_pack(wost[:, pl.ds(c0, 128)]))
        return carry

    with jax.named_scope("perm_rows"):
        lax.fori_loop(0, D // WOC, permo_body, 0)

    lane = lax.broadcasted_iota(jnp.int32, (RG, 128), 1)
    rowi = lax.broadcasted_iota(jnp.int32, (RG, 128), 0)

    def tile_dot(lhs_ref, w_ref, n):
        return jnp.dot(_unpack(lhs_ref[...]), _unpack(w_ref[:, n * NC:(n + 1) * NC]),
                       preferred_element_type=F32)

    tpc = NC // 128

    def local_qkv(h_ref, off, i, lo=0, hi=3 * D // NC):
        for n in (list(range(D // NC, 3 * D // NC)) + list(range(D // NC)))[lo:hi]:
            res = tile_dot(h_ref, wa, n)
            for u in range(tpc):
                sec, t = divmod(n * tpc + u, NT)
                val = res[:, u * 128:(u + 1) * 128]
                if sec == 0:
                    qbuf[off // CM][t, 0:CM, :] = val
                elif sec == 1:
                    kbuf[t, HALO + off:HALO + off + CM, :] = val
                else:
                    vbuf[t, HALO + off:HALO + off + CM, :] = val
                    if off == 0:
                        first = jnp.broadcast_to(val[0:1, :], (HALO, 128))
                        vbuf[t, 0:HALO, :] = jnp.where(i == 0, first, vbuf[t, 0:HALO, :])

    def local_attn(o_ref, off, i):
        zero = zref[0]
        for g in range(CM // RG):
            base = HALO + off + g * RG
            qg = [qbuf[off // CM][t, pl.ds(pl.multiple_of(zero + g * RG, RG), RG), :] for t in range(NT)]
            logit = []
            for w in range(WIN):
                a = base - DIL * w
                part = qg[0] * kbuf[0, a:a + RG, :]
                for t in range(1, NT):
                    part = part + qg[t] * kbuf[t, a:a + RG, :]
                lg = _group_sum4(part, lane) * QSCALE
                if off == 0 and g == 0 and w > 0:
                    lg = jnp.where(rowi + i * BM >= DIL * w, lg, MASKED)
                logit.append(lg)
            m = functools.reduce(jnp.maximum, logit)
            p = [jnp.exp2(lg - m) for lg in logit]
            inv = 1.0 / functools.reduce(lambda u, v: u + v, p)
            for t in range(NT):
                acc = p[0] * vbuf[t, base:base + RG, :]
                for w in range(1, WIN):
                    a = base - DIL * w
                    acc = acc + p[w] * vbuf[t, a:a + RG, :]
                o_ref[g * RG // 2:(g + 1) * RG // 2, t * 128:(t + 1) * 128] = _pack(acc * inv)

    def full_qkv(h_ref, r, lo=0, hi=3 * D // NC):
        r2 = pl.multiple_of(r // 2, CM // 2)
        order = list(range(2 * D // NC, 3 * D // NC)) + list(range(2 * D // NC))
        for n in order[lo:hi]:
            res = tile_dot(h_ref, wb, n)
            for u in range(tpc):
                sec, t = divmod(n * tpc + u, NT)
                val = res[:, u * 128:(u + 1) * 128]
                if sec == 0:
                    qs[t, pl.ds(r2, CM // 2), :] = _pack(val * QSCALE)
                elif sec == 1:
                    ks[t, pl.ds(r2, CM // 2), :] = _pack(val)
                else:
                    vt[t * 64:(t + 1) * 64, pl.ds(r, CM)] = _pack(val.T)

    def row_phase(pair):
        @pl.when(pair == 1)
        def _():
            hb[0] = _pack(_layernorm(xres[0:CM, :]))

        def body(i, c):
            @pl.when(jnp.logical_and(pair == 0, i == 1))
            def _():
                cp_x2.wait()
                cp_wob.wait()
                repack(wost2, wob)

            r0 = pl.multiple_of(i * BM, BM)
            rs = [pl.multiple_of(r0 + ch * CM, CM) for ch in range(nch)]
            for t in range(NT):
                kbuf[t, 0:HALO, :] = kbuf[t, BM:BM + HALO, :]
                vbuf[t, 0:HALO, :] = vbuf[t, BM:BM + HALO, :]
            rn = pl.multiple_of(jnp.minimum(i + 1, nblk - 1) * BM, BM)

            def local_out(ch):
                local_attn(ob.at[ch], ch * CM, i)
                y = jnp.concatenate([tile_dot(ob.at[ch], woa, n) for n in range(D // NC)], axis=1)
                x2 = xres[pl.ds(rs[ch], CM), :] + y
                xres[pl.ds(rs[ch], CM), :] = x2
                xsave[pl.ds(rs[ch], CM), :] = x2
                h2b[ch] = _pack(_layernorm(x2))

            hb[1] = _pack(_layernorm(xres[pl.ds(rs[1], CM), :]))
            local_qkv(hb.at[0], 0, i)
            local_qkv(hb.at[1], CM, i, 0, SPLIT1)
            local_out(0)
            local_qkv(hb.at[1], CM, i, SPLIT1)

            @pl.when(jnp.logical_and(pair == 0, i == 0))
            def _():
                cp_wb.wait()
                cp_x2.start()
                cp_wob.start()
                repack(wst2, wb)
                cp_x1.wait()

            full_qkv(h2b.at[0], rs[0], 0, SPLIT2)
            local_out(1)
            full_qkv(h2b.at[0], rs[0], SPLIT2)
            full_qkv(h2b.at[1], rs[1], 0, 10)
            fresh = jnp.logical_and(pair == 0, i + 1 < nblk)
            xn = jnp.where(fresh, xio[pl.ds(rn, BM), :].astype(F32), xres[pl.ds(rn, BM), :])
            xres[pl.ds(rn, BM), :] = xn
            hb[0] = _pack(_layernorm(xn[0:CM, :]))
            full_qkv(h2b.at[1], rs[1], 10)
            return c

        with jax.named_scope("row_phase"):
            lax.fori_loop(0, nblk, body, 0)

    early = QB // OB

    def out_copy(i):
        r0 = pl.multiple_of(i * OB, OB)
        return pltpu.make_async_copy(xio.at[pl.ds(r0, OB), :], out_hbm.at[pl.ds(r0, OB), :],
                                     osems.at[i])

    def write_out(lo, hi):
        def body(i, c):
            r0 = pl.multiple_of(i * OB, OB)
            xio[pl.ds(r0, OB), :] = xres[pl.ds(r0, OB), :].astype(BF16)
            out_copy(i).start()
            return c

        lax.fori_loop(lo, hi, body, 0)

    nt_dims = (((1,), (1,)), ((), ()))

    def masked_q(q32, hp):
        head = lax.broadcasted_iota(jnp.int32, q32.shape, 1) // DH
        return _unpack(jnp.where(head == hp, q32, jnp.uint32(0)))

    def add_oproj(ot, g, q0, nq):
        g64 = pl.multiple_of(g * 64, 64)
        for j in range(nq // OS):
            y = jnp.dot(ot[:, j * OS:(j + 1) * OS].T.astype(BF16), _unpack(wob[pl.ds(g64, 64), :]),
                        preferred_element_type=F32)
            r = pl.multiple_of(q0 + j * OS, OS)
            xres[pl.ds(r, OS), :] = xres[pl.ds(r, OS), :] + y

    def full_attn(pair):
        nqb = S // QB

        def body(it, bad):
            @pl.when(jnp.logical_and(pair == 1, it == NT))
            def _():
                write_out(0, early)

            g = it % NT
            q0 = pl.multiple_of((it // NT) * QB, QB)
            q32 = qs[g, pl.ds(pl.multiple_of(q0 // 2, QB // 2), QB // 2), :]
            zero = zref[0]
            acc = [None] * HPT
            l8 = [None] * HPT

            def pv(hp, t, buf):
                r0 = pl.multiple_of(g * 64 + hp * (DH // 2), DH // 2)
                vc = _unpack(vt[pl.ds(r0, DH // 2), t * KC:(t + 1) * KC])
                a = jnp.dot(vc, _unpack(buf[zero]), preferred_element_type=F32)
                acc[hp] = a if acc[hp] is None else acc[hp] + a

            pending = None
            for hp in range(HPT):
                w = masked_q(q32, hp)
                for t in range(S // KC):
                    kc = _unpack(ks[g, t * KC // 2:(t + 1) * KC // 2, :])
                    p = jnp.exp2(lax.dot_general(kc, w, nt_dims, preferred_element_type=F32))
                    part = jnp.sum(p.reshape(KC // 8, 8, QB), axis=0)
                    l8[hp] = part if l8[hp] is None else l8[hp] + part
                    buf = pbufs[(hp * (S // KC) + t) % len(pbufs)]
                    buf[0] = _pack(p)
                    if pending is not None:
                        pv(*pending)
                    pending = (hp, t, buf)
            pv(*pending)
            outs = []
            for hp in range(HPT):
                l = jnp.sum(l8[hp], axis=0, keepdims=True)
                o = acc[hp] * (1.0 / l)
                outs.append(o)
                ok = (jnp.abs(o) < O_HI) & (l > L_LO) & (l < L_HI)
                nbad = jnp.where(ok, 0.0, 1.0)
                bad = jnp.maximum(bad, jnp.max(nbad.reshape(DH // 8, 8, QB), axis=0))
            add_oproj(jnp.concatenate(outs, axis=0), g, q0, QB)
            return bad

        with jax.named_scope("full_attn"):
            bad = lax.fori_loop(0, NT * nqb, body, jnp.zeros((8, QB), F32))

        @pl.when(jnp.max(bad) > 0.0)
        def _():
            nq = S // FQ

            def restore(i, c):
                r = pl.multiple_of(i * 32, 32)
                xres[pl.ds(r, 32), :] = xsave[pl.ds(r, 32), :]
                return c

            lax.fori_loop(0, S // 32, restore, 0)

            def fb_body(it, c):
                g = it // nq
                q0 = pl.multiple_of((it % nq) * FQ, FQ)
                q32 = qs[g, pl.ds(pl.multiple_of(q0 // 2, FQ // 2), FQ // 2), :]

                def head_body(hp, c2):
                    r0 = pl.multiple_of(g * 64 + hp * (DH // 2), DH // 2)
                    s = lax.dot_general(_unpack(ks[g]), masked_q(q32, hp), nt_dims,
                                        preferred_element_type=F32)
                    p = jnp.exp2(s - jnp.max(s, axis=0, keepdims=True))
                    l = jnp.sum(p, axis=0, keepdims=True)
                    acc = jnp.dot(_unpack(vt[pl.ds(r0, DH // 2), :]), p.astype(BF16),
                                  preferred_element_type=F32)
                    ots[pl.ds(pl.multiple_of(hp * DH, DH), DH), :] = acc * (1.0 / l)
                    return c2

                lax.fori_loop(0, HPT, head_body, 0)
                add_oproj(ots[...], g, q0, FQ)
                return c

            lax.fori_loop(0, NT * nq, fb_body, 0)

            @pl.when(pair == 1)
            def _():
                for i in range(early):
                    out_copy(i).wait()
                write_out(0, early)

    def pair_body(pair, c):
        row_phase(pair)
        full_attn(pair)
        return c

    with jax.named_scope("pairs"):
        lax.fori_loop(0, 2, pair_body, 0)

    with jax.named_scope("out_phase"):
        write_out(early, S // OB)
        for i in range(S // OB):
            out_copy(i).wait()


@jax.jit
def pallas_interleave_layers__sliding_local_dilated__softmax_full_mha__prompt_kernel(
    A_x: jax.Array,
    A_wqkv: jax.Array,
    A_wo: jax.Array,
    B_x: jax.Array,
    B_wqkv: jax.Array,
    B_wo: jax.Array,
):
    del B_x
    x = A_x.reshape(S, D)
    hbm = pl.BlockSpec(memory_space=pl.ANY)
    out = pl.pallas_call(
        _kernel,
        out_shape=jax.ShapeDtypeStruct((S, D), BF16),
        in_specs=[hbm] * 5,
        out_specs=hbm,
        scratch_shapes=[
            pltpu.VMEM((S, D), BF16),
            pltpu.VMEM((S, D), F32),
            pltpu.VMEM((S, D), F32),
            pltpu.VMEM((D, 3 * D), BF16),
            pltpu.VMEM((D, D), BF16),
            pltpu.VMEM((D, 3 * D), BF16),
            pltpu.VMEM((D, D), BF16),
            pltpu.VMEM((D // 2, 3 * D), U32),
            pltpu.VMEM((D // 2, D), U32),
            pltpu.VMEM((D // 2, 3 * D), U32),
            pltpu.VMEM((D // 2, D), U32),
            pltpu.VMEM((BM // CM, CM // 2, D), U32),
            pltpu.VMEM((BM // CM, CM // 2, D), U32),
            pltpu.VMEM((BM // CM, CM // 2, D), U32),
            pltpu.VMEM((NT, CM + 8, 128), F32),
            pltpu.VMEM((NT, CM + 8, 128), F32),
            pltpu.SMEM((1,), jnp.int32),
            pltpu.VMEM((NT, HALO + BM, 128), F32),
            pltpu.VMEM((NT, HALO + BM, 128), F32),
            pltpu.VMEM((NT, S // 2, 128), U32),
            pltpu.VMEM((NT, S // 2, 128), U32),
            pltpu.VMEM((D // 2, S), U32),
            pltpu.VMEM((128, FQ), F32),
            pltpu.VMEM((1, KC // 2, QB), U32),
            pltpu.VMEM((1, KC // 2, QB), U32),
            pltpu.VMEM((1, KC // 2, QB), U32),
            pltpu.VMEM((1, KC // 2, QB), U32),
            pltpu.SemaphoreType.DMA((D // 128 + D // WOC,)),
            pltpu.SemaphoreType.DMA((6,)),
            pltpu.SemaphoreType.DMA((S // OB,)),
        ],
        compiler_params=pltpu.CompilerParams(vmem_limit_bytes=110 * 1024 * 1024),
        name="interleaved_attention_stack",
    )(x, A_wqkv, A_wo, B_wqkv, B_wo)
    return out.reshape(1, S, D)
```

```python
import functools
import math

import jax
import jax.numpy as jnp
from jax import lax
import jax.experimental.pallas as pl
import jax.experimental.pallas.tpu as pltpu

S = 2048
D = 1024
H = 32
DH = D // H
NT = D // 128
HPT = 128 // DH
WIN = 8
DIL = 2
HALO = 16
EPS = 1e-5
LOG2E = math.log2(math.e)
QSCALE = (DH ** -0.5) * LOG2E
MASKED = -1e9 * LOG2E

BM = 256
CM = 128
NC = 128
SPLIT1 = 16
SPLIT2 = 16
LAG = 6
RG = 16
KC = 512
QB = 1024
OS = 128
WOC = 256
OB = 128
FQ = 128

L_LO = 2.0 ** -40
L_HI = 2.0 ** 90
O_HI = 3.0e38

F32 = jnp.float32
BF16 = jnp.bfloat16
U32 = jnp.uint32


def _layernorm(x):
    mu = jnp.mean(x, axis=-1, keepdims=True)
    xc = x - mu
    var = jnp.mean(xc * xc, axis=-1, keepdims=True)
    return xc * lax.rsqrt(var + EPS)


def _permute_cols(w32):
    rows = w32.shape[0]
    lane = lax.broadcasted_iota(jnp.int32, (rows, 128), 1)
    tiles = [w32[:, t * 128:(t + 1) * 128] for t in range(NT)]
    for b in range(3):
        sh = 4 << b
        low = (lane & sh) == 0
        for a in range(NT):
            if a & (1 << b):
                continue
            c = a | (1 << b)
            ta, tc = tiles[a], tiles[c]
            tiles[a] = jnp.where(low, ta, pltpu.roll(tc, sh, 1))
            tiles[c] = jnp.where(low, pltpu.roll(ta, 128 - sh, 1), tc)
    return jnp.concatenate(tiles, axis=1)


def _permute_rows(w32):
    ncols = w32.shape[1]
    nv = D // 16
    v = [w32[i * 8:(i + 1) * 8, :] for i in range(nv)]
    sub = lax.broadcasted_iota(jnp.int32, (8, ncols), 0)
    for vb, sh in ((8, 2), (16, 4)):
        low = (sub & sh) == 0
        for a in range(nv):
            if a & vb:
                continue
            c = a | vb
            ta, tc = v[a], v[c]
            v[a] = jnp.where(low, ta, pltpu.roll(tc, sh, 0))
            v[c] = jnp.where(low, pltpu.roll(ta, 8 - sh, 0), tc)
    def src(i):
        b0, b5 = i & 1, (i >> 5) & 1
        return (i & ~33) | (b0 << 5) | b5
    return jnp.concatenate([v[src(i)] for i in range(nv)], axis=0)


def _group_sum4(x, lane):
    b0 = (lane & 1) == 0
    x = x + jnp.where(b0, pltpu.roll(x, 127, 1), pltpu.roll(x, 1, 1))
    b1 = (lane & 2) == 0
    return x + jnp.where(b1, pltpu.roll(x, 126, 1), pltpu.roll(x, 2, 1))


def _pack(x):
    return pltpu.bitcast(x.astype(BF16), U32)


def _unpack(x):
    return pltpu.bitcast(x, BF16)


def _kernel(x_hbm, wa_hbm, woa_hbm, wb_hbm, wob_hbm, out_hbm,
            xio, xres, xsave, wst, wost, wst2, wost2, wa, woa, wb, wob, hb, h2b, ob, qbuf0, qbuf1, zref, zvec, kbuf, vbuf,
            qs, ks, vt, ots, pb0, pb1, pb2, pb3, wsems, sems, osems):
    nblk = S // BM
    qbuf = (qbuf0, qbuf1)
    pbufs = (pb0, pb1, pb2, pb3)
    zref[0] = 0
    zvec[...] = jnp.zeros(zvec.shape, U32)
    nch = BM // CM
    pr = 128
    nwc = D // pr

    def wa_copy(c):
        r = pl.multiple_of(c * pr, pr)
        return pltpu.make_async_copy(wa_hbm.at[pl.ds(r, pr), :], wst.at[pl.ds(r, pr), :],
                                     wsems.at[c])

    def x_copy(r0, n, k):
        return pltpu.make_async_copy(x_hbm.at[pl.ds(r0, n), :], xio.at[pl.ds(r0, n), :], sems.at[k])

    def woa_copy(t):
        c0 = pl.multiple_of(t * WOC, WOC)
        return pltpu.make_async_copy(woa_hbm.at[:, pl.ds(c0, WOC)], wost.at[:, pl.ds(c0, WOC)],
                                     wsems.at[nwc + t])

    cp_x0 = x_copy(0, BM, 1)
    cp_wb = pltpu.make_async_copy(wb_hbm, wst2, sems.at[2])
    cp_x1 = x_copy(BM, BM, 3)
    cp_x2 = x_copy(2 * BM, S - 2 * BM, 4)
    cp_wob = pltpu.make_async_copy(wob_hbm, wost2, sems.at[5])
    ahead = 3
    for c in range(ahead):
        wa_copy(c).start()

    for t in range(NT):
        kbuf[t, BM:BM + HALO, :] = jnp.zeros((HALO, 128), F32)
        vbuf[t, BM:BM + HALO, :] = jnp.zeros((HALO, 128), F32)

    def perm_body(c, carry):
        wa_copy(c).wait()

        @pl.when(c + ahead < nwc)
        def _():
            wa_copy(jnp.minimum(c + ahead, nwc - 1)).start()

        @pl.when(c + ahead == nwc)
        def _():
            cp_x0.start()

        @pl.when(c + ahead == nwc + 1)
        def _():
            for t in range(D // WOC):
                woa_copy(t).start()

        r = pl.multiple_of(c * pr, pr)
        r2 = pl.multiple_of(c * (pr // 2), pr // 2)
        for sec in range(3):
            w32 = _pack(wst[pl.ds(r, pr), sec * D:(sec + 1) * D])
            wa[pl.ds(r2, pr // 2), sec * D:(sec + 1) * D] = _permute_cols(w32)
        return carry

    with jax.named_scope("perm_cols"):
        lax.fori_loop(0, nwc, perm_body, 0)

    def widen_x(r0, nrows):
        step = 64

        def body(i, carry):
            r = pl.multiple_of(r0 + i * step, step)
            xres[pl.ds(r, step), :] = xio[pl.ds(r, step), :].astype(F32)
            return carry

        lax.fori_loop(0, nrows // step, body, 0)

    def repack(src, dst):
        step = 64

        def body(i, carry):
            r = pl.multiple_of(i * step, step)
            r2 = pl.multiple_of(i * (step // 2), step // 2)
            dst[pl.ds(r2, step // 2), :] = _pack(src[pl.ds(r, step), :])
            return carry

        lax.fori_loop(0, D // step, body, 0)

    with jax.named_scope("x_in"):
        cp_x0.wait()
        widen_x(0, BM)
        hb[0] = _pack(_layernorm(xres[0:CM, :]))

    def permo_body(t, carry):
        woa_copy(t).wait()

        @pl.when(t == 0)
        def _():
            cp_wb.start()
            cp_x1.start()

        for u in range(WOC // 128):
            c0 = pl.multiple_of(t * WOC + u * 128, 128)
            woa[:, pl.ds(c0, 128)] = _permute_rows(_pack(wost[:, pl.ds(c0, 128)]))
        return carry

    with jax.named_scope("perm_rows"):
        lax.fori_loop(0, D // WOC, permo_body, 0)

    lane = lax.broadcasted_iota(jnp.int32, (RG, 128), 1)
    rowi = lax.broadcasted_iota(jnp.int32, (RG, 128), 0)

    ties = []

    def tile_dot(lhs_ref, w_ref, n):
        lhs = lhs_ref[...]
        for e in ties:
            e[0] -= 1
        due = [e[1] for e in ties if e[0] <= 0]
        ties[:] = [e for e in ties if e[0] > 0]
        if due:
            first = functools.reduce(lambda u, v: u | v, due, lhs[0:8, 0:128])
            top = jnp.concatenate([first, lhs[0:8, 128:]], axis=1)
            lhs = jnp.concatenate([top, lhs[8:, :]], axis=0)
        return jnp.dot(_unpack(lhs), _unpack(w_ref[:, n * NC:(n + 1) * NC]),
                       preferred_element_type=F32)

    def pack_t(val):
        pt = _pack(val.T)
        bits = functools.reduce(lambda u, v: u | v, [pt[j * 8:(j + 1) * 8, :] for j in range(8)])
        ties.append([LAG, bits & zvec[...]])
        return pt

    tpc = NC // 128

    def local_qkv(h_ref, off, i, lo=0, hi=3 * D // NC):
        for n in (list(range(D // NC, 3 * D // NC)) + list(range(D // NC)))[lo:hi]:
            res = tile_dot(h_ref, wa, n)
            for u in range(tpc):
                sec, t = divmod(n * tpc + u, NT)
                val = res[:, u * 128:(u + 1) * 128]
                if sec == 0:
                    qbuf[off // CM][t, 0:CM, :] = val
                elif sec == 1:
                    kbuf[t, HALO + off:HALO + off + CM, :] = val
                else:
                    vbuf[t, HALO + off:HALO + off + CM, :] = val
                    if off == 0:
                        first = jnp.broadcast_to(val[0:1, :], (HALO, 128))
                        vbuf[t, 0:HALO, :] = jnp.where(i == 0, first, vbuf[t, 0:HALO, :])

    def local_attn(o_ref, off, i):
        zero = zref[0]
        for g in range(CM // RG):
            base = HALO + off + g * RG
            qg = [qbuf[off // CM][t, pl.ds(pl.multiple_of(zero + g * RG, RG), RG), :] for t in range(NT)]
            logit = []
            for w in range(WIN):
                a = base - DIL * w
                part = qg[0] * kbuf[0, a:a + RG, :]
                for t in range(1, NT):
                    part = part + qg[t] * kbuf[t, a:a + RG, :]
                lg = _group_sum4(part, lane) * QSCALE
                if off == 0 and g == 0 and w > 0:
                    lg = jnp.where(rowi + i * BM >= DIL * w, lg, MASKED)
                logit.append(lg)
            m = functools.reduce(jnp.maximum, logit)
            p = [jnp.exp2(lg - m) for lg in logit]
            inv = 1.0 / functools.reduce(lambda u, v: u + v, p)
            for t in range(NT):
                acc = p[0] * vbuf[t, base:base + RG, :]
                for w in range(1, WIN):
                    a = base - DIL * w
                    acc = acc + p[w] * vbuf[t, a:a + RG, :]
                o_ref[g * RG // 2:(g + 1) * RG // 2, t * 128:(t + 1) * 128] = _pack(acc * inv)

    def full_qkv(h_ref, r, lo=0, hi=3 * D // NC):
        r2 = pl.multiple_of(r >> 1, CM // 2)
        order = list(range(2 * D // NC, 3 * D // NC)) + list(range(2 * D // NC))
        for n in order[lo:hi]:
            res = tile_dot(h_ref, wb, n)
            for u in range(tpc):
                sec, t = divmod(n * tpc + u, NT)
                val = res[:, u * 128:(u + 1) * 128]
                if sec == 0:
                    qs[t * 64:(t + 1) * 64, pl.ds(r, CM)] = pack_t(val * QSCALE)
                elif sec == 1:
                    ks[t, pl.ds(r2, CM // 2), :] = _pack(val)
                else:
                    vt[t * 64:(t + 1) * 64, pl.ds(r, CM)] = pack_t(val)

    def row_phase(pair):
        @pl.when(pair == 1)
        def _():
            hb[0] = _pack(_layernorm(xres[0:CM, :]))

        def body(i, c):
            @pl.when(jnp.logical_and(pair == 0, i == 1))
            def _():
                cp_x2.wait()
                cp_wob.wait()
                repack(wost2, wob)

            r0 = pl.multiple_of(i * BM, BM)
            rs = [pl.multiple_of(r0 + ch * CM, CM) for ch in range(nch)]
            for t in range(NT):
                kbuf[t, 0:HALO, :] = kbuf[t, BM:BM + HALO, :]
                vbuf[t, 0:HALO, :] = vbuf[t, BM:BM + HALO, :]
            rn = pl.multiple_of(jnp.minimum(i + 1, nblk - 1) * BM, BM)

            def local_out(ch):
                local_attn(ob.at[ch], ch * CM, i)
                y = jnp.concatenate([tile_dot(ob.at[ch], woa, n) for n in range(D // NC)], axis=1)
                x2 = xres[pl.ds(rs[ch], CM), :] + y
                xres[pl.ds(rs[ch], CM), :] = x2
                xsave[pl.ds(rs[ch], CM), :] = x2
                h2b[ch] = _pack(_layernorm(x2))

            hb[1] = _pack(_layernorm(xres[pl.ds(rs[1], CM), :]))
            local_qkv(hb.at[0], 0, i)
            local_qkv(hb.at[1], CM, i, 0, SPLIT1)
            local_out(0)
            local_qkv(hb.at[1], CM, i, SPLIT1)

            @pl.when(jnp.logical_and(pair == 0, i == 0))
            def _():
                cp_wb.wait()
                cp_x2.start()
                cp_wob.start()
                repack(wst2, wb)
                cp_x1.wait()

            full_qkv(h2b.at[0], rs[0], 0, SPLIT2)
            local_out(1)
            full_qkv(h2b.at[0], rs[0], SPLIT2)
            full_qkv(h2b.at[1], rs[1], 0, 10)
            fresh = jnp.logical_and(pair == 0, i + 1 < nblk)
            xn = jnp.where(fresh, xio[pl.ds(rn, BM), :].astype(F32), xres[pl.ds(rn, BM), :])
            xres[pl.ds(rn, BM), :] = xn
            hb[0] = _pack(_layernorm(xn[0:CM, :]))
            full_qkv(h2b.at[1], rs[1], 10)
            assert not ties
            return c

        with jax.named_scope("row_phase"):
            lax.fori_loop(0, nblk, body, 0)

    early = QB // OB

    def out_copy(i):
        r0 = pl.multiple_of(i * OB, OB)
        return pltpu.make_async_copy(xio.at[pl.ds(r0, OB), :], out_hbm.at[pl.ds(r0, OB), :],
                                     osems.at[i])

    def write_out(lo, hi):
        def body(i, c):
            r0 = pl.multiple_of(i * OB, OB)
            xio[pl.ds(r0, OB), :] = xres[pl.ds(r0, OB), :].astype(BF16)
            out_copy(i).start()
            return c

        lax.fori_loop(lo, hi, body, 0)

    nt_dims = (((1,), (1,)), ((), ()))

    def masked_q(q32, hp):
        head = lax.broadcasted_iota(jnp.int32, q32.shape, 0) >> (DH.bit_length() - 2)
        return _unpack(jnp.where(head == hp, q32, jnp.uint32(0)))

    def padded_qt(g, hp, q0, nq):
        hr = DH // 2
        qt = qs[pl.ds(pl.multiple_of(g * 64 + hp * hr, hr), hr), pl.ds(q0, nq)]
        parts = [jnp.zeros((hp * hr, nq), U32), qt, jnp.zeros(((HPT - 1 - hp) * hr, nq), U32)]
        return _unpack(jnp.concatenate([x for x in parts if x.shape[0]], axis=0))

    def add_oproj(ot, g, q0, nq):
        g64 = pl.multiple_of(g * 64, 64)
        for j in range(nq // OS):
            y = jnp.dot(ot[:, j * OS:(j + 1) * OS].T.astype(BF16), _unpack(wob[pl.ds(g64, 64), :]),
                        preferred_element_type=F32)
            r = pl.multiple_of(q0 + j * OS, OS)
            xres[pl.ds(r, OS), :] = xres[pl.ds(r, OS), :] + y

    def full_attn(pair):
        nqb = S // QB

        def body(it, bad):
            @pl.when(jnp.logical_and(pair == 1, it == NT))
            def _():
                write_out(0, early)

            g = it & (NT - 1)
            qh = it >> (NT.bit_length() - 1)
            q0 = pl.multiple_of(qh * QB, QB)
            zero = zref[0]
            acc = [None] * HPT
            l8 = [None] * HPT

            def pv(hp, t, buf):
                r0 = pl.multiple_of(g * 64 + hp * (DH // 2), DH // 2)
                vc = _unpack(vt[pl.ds(r0, DH // 2), t * KC:(t + 1) * KC])
                a = jnp.dot(vc, _unpack(buf[zero]), preferred_element_type=F32)
                acc[hp] = a if acc[hp] is None else acc[hp] + a

            pending = None
            for hp in range(HPT):
                w = padded_qt(g, hp, q0, QB)
                for t in range(S // KC):
                    kc = _unpack(ks[g, t * KC // 2:(t + 1) * KC // 2, :])
                    p = jnp.exp2(jnp.dot(kc, w, preferred_element_type=F32))
                    part = jnp.sum(p.reshape(KC // 8, 8, QB), axis=0)
                    l8[hp] = part if l8[hp] is None else l8[hp] + part
                    buf = pbufs[(hp * (S // KC) + t) % len(pbufs)]
                    buf[0] = _pack(p)
                    if pending is not None:
                        pv(*pending)
                    pending = (hp, t, buf)
            pv(*pending)
            outs = []
            for hp in range(HPT):
                l = jnp.sum(l8[hp], axis=0, keepdims=True)
                o = acc[hp] * (1.0 / l)
                outs.append(o)
                ok = (jnp.abs(o) < O_HI) & (l > L_LO) & (l < L_HI)
                nbad = jnp.where(ok, 0.0, 1.0)
                nbad = jnp.max(nbad.reshape(DH // 8, 8, QB), axis=0)
                for j in range(QB // 128):
                    bad = jnp.maximum(bad, nbad[:, j * 128:(j + 1) * 128])
            add_oproj(jnp.concatenate(outs, axis=0), g, q0, QB)
            return bad

        with jax.named_scope("full_attn"):
            bad = lax.fori_loop(0, NT * nqb, body, jnp.zeros((8, 128), F32))

        @pl.when(jnp.max(bad) > 0.0)
        def _():
            nq = S // FQ

            def restore(i, c):
                r = pl.multiple_of(i * 32, 32)
                xres[pl.ds(r, 32), :] = xsave[pl.ds(r, 32), :]
                return c

            lax.fori_loop(0, S // 32, restore, 0)

            def fb_body(it, c):
                g = it // nq
                q0 = pl.multiple_of((it % nq) * FQ, FQ)
                q32 = qs[pl.ds(pl.multiple_of(g * 64, 64), 64), pl.ds(q0, FQ)]

                def head_body(hp, c2):
                    r0 = pl.multiple_of(g * 64 + hp * (DH // 2), DH // 2)
                    s = jnp.dot(_unpack(ks[g]), masked_q(q32, hp), preferred_element_type=F32)
                    p = jnp.exp2(s - jnp.max(s, axis=0, keepdims=True))
                    l = jnp.sum(p, axis=0, keepdims=True)
                    acc = jnp.dot(_unpack(vt[pl.ds(r0, DH // 2), :]), p.astype(BF16),
                                  preferred_element_type=F32)
                    ots[pl.ds(pl.multiple_of(hp * DH, DH), DH), :] = acc * (1.0 / l)
                    return c2

                lax.fori_loop(0, HPT, head_body, 0)
                add_oproj(ots[...], g, q0, FQ)
                return c

            lax.fori_loop(0, NT * nq, fb_body, 0)

            @pl.when(pair == 1)
            def _():
                for i in range(early):
                    out_copy(i).wait()
                write_out(0, early)

    def pair_body(pair, c):
        row_phase(pair)
        full_attn(pair)
        return c

    with jax.named_scope("pairs"):
        lax.fori_loop(0, 2, pair_body, 0)

    with jax.named_scope("out_phase"):
        write_out(early, S // OB)
        for i in range(S // OB):
            out_copy(i).wait()


@jax.jit
def pallas_interleave_layers__sliding_local_dilated__softmax_full_mha__prompt_kernel(
    A_x: jax.Array,
    A_wqkv: jax.Array,
    A_wo: jax.Array,
    B_x: jax.Array,
    B_wqkv: jax.Array,
    B_wo: jax.Array,
):
    del B_x
    x = A_x.reshape(S, D)
    hbm = pl.BlockSpec(memory_space=pl.ANY)
    out = pl.pallas_call(
        _kernel,
        out_shape=jax.ShapeDtypeStruct((S, D), BF16),
        in_specs=[hbm] * 5,
        out_specs=hbm,
        scratch_shapes=[
            pltpu.VMEM((S, D), BF16),
            pltpu.VMEM((S, D), F32),
            pltpu.VMEM((S, D), F32),
            pltpu.VMEM((D, 3 * D), BF16),
            pltpu.VMEM((D, D), BF16),
            pltpu.VMEM((D, 3 * D), BF16),
            pltpu.VMEM((D, D), BF16),
            pltpu.VMEM((D // 2, 3 * D), U32),
            pltpu.VMEM((D // 2, D), U32),
            pltpu.VMEM((D // 2, 3 * D), U32),
            pltpu.VMEM((D // 2, D), U32),
            pltpu.VMEM((BM // CM, CM // 2, D), U32),
            pltpu.VMEM((BM // CM, CM // 2, D), U32),
            pltpu.VMEM((BM // CM, CM // 2, D), U32),
            pltpu.VMEM((NT, CM + 8, 128), F32),
            pltpu.VMEM((NT, CM + 8, 128), F32),
            pltpu.SMEM((1,), jnp.int32),
            pltpu.VMEM((8, 128), U32),
            pltpu.VMEM((NT, HALO + BM, 128), F32),
            pltpu.VMEM((NT, HALO + BM, 128), F32),
            pltpu.VMEM((D // 2, S), U32),
            pltpu.VMEM((NT, S // 2, 128), U32),
            pltpu.VMEM((D // 2, S), U32),
            pltpu.VMEM((128, FQ), F32),
            pltpu.VMEM((1, KC // 2, QB), U32),
            pltpu.VMEM((1, KC // 2, QB), U32),
            pltpu.VMEM((1, KC // 2, QB), U32),
            pltpu.VMEM((1, KC // 2, QB), U32),
            pltpu.SemaphoreType.DMA((D // 128 + D // WOC,)),
            pltpu.SemaphoreType.DMA((6,)),
            pltpu.SemaphoreType.DMA((S // OB,)),
        ],
        compiler_params=pltpu.CompilerParams(vmem_limit_bytes=110 * 1024 * 1024),
        name="interleaved_attention_stack",
    )(x, A_wqkv, A_wo, B_wqkv, B_wo)
    return out.reshape(1, S, D)
```

```python
import functools
import math

import jax
import jax.numpy as jnp
from jax import lax
import jax.experimental.pallas as pl
import jax.experimental.pallas.tpu as pltpu

S = 2048
D = 1024
H = 32
DH = D // H
NT = D // 128
HPT = 128 // DH
WIN = 8
DIL = 2
HALO = 16
EPS = 1e-5
LOG2E = math.log2(math.e)
QSCALE = (DH ** -0.5) * LOG2E
MASKED = -1e9 * LOG2E

BM = 256
CM = 128
NC = 128
SPLIT1 = 12
KS1 = 0
KS2 = 1
KL0 = 4
KLS = 0.6
NL0 = None
NLS = 0.3
NLT = 0.7
CL0 = 2
AEARLY = 0
AL0 = None
ALS = 1
BL0 = 6
BLS = 1
SPLIT2 = 16
LAG = 6
RG = 16
KC = 512
QB = 1024
OS = 128
OB = 128
FQ = 128

L_LO = 2.0 ** -40
L_HI = 2.0 ** 90
O_HI = 3.0e38

F32 = jnp.float32
BF16 = jnp.bfloat16
U32 = jnp.uint32


def _layernorm(x):
    mu = jnp.mean(x, axis=-1, keepdims=True)
    xc = x - mu
    var = jnp.mean(xc * xc, axis=-1, keepdims=True)
    return xc * lax.rsqrt(var + EPS)


def _permute_cols(w32):
    rows = w32.shape[0]
    lane = lax.broadcasted_iota(jnp.int32, (rows, 128), 1)
    tiles = [w32[:, t * 128:(t + 1) * 128] for t in range(NT)]
    for b in range(3):
        sh = 4 << b
        low = (lane & sh) == 0
        for a in range(NT):
            if a & (1 << b):
                continue
            c = a | (1 << b)
            ta, tc = tiles[a], tiles[c]
            tiles[a] = jnp.where(low, ta, pltpu.roll(tc, sh, 1))
            tiles[c] = jnp.where(low, pltpu.roll(ta, 128 - sh, 1), tc)
    return jnp.concatenate(tiles, axis=1)


def _permute_rows(w32):
    ncols = w32.shape[1]
    nv = D // 16
    v = [w32[i * 8:(i + 1) * 8, :] for i in range(nv)]
    sub = lax.broadcasted_iota(jnp.int32, (8, ncols), 0)
    for vb, sh in ((8, 2), (16, 4)):
        low = (sub & sh) == 0
        for a in range(nv):
            if a & vb:
                continue
            c = a | vb
            ta, tc = v[a], v[c]
            v[a] = jnp.where(low, ta, pltpu.roll(tc, sh, 0))
            v[c] = jnp.where(low, pltpu.roll(ta, 8 - sh, 0), tc)
    def src(i):
        b0, b5 = i & 1, (i >> 5) & 1
        return (i & ~33) | (b0 << 5) | b5
    return jnp.concatenate([v[src(i)] for i in range(nv)], axis=0)


def _group_sum4(x, lane):
    b0 = (lane & 1) == 0
    x = x + jnp.where(b0, pltpu.roll(x, 127, 1), pltpu.roll(x, 1, 1))
    b1 = (lane & 2) == 0
    return x + jnp.where(b1, pltpu.roll(x, 126, 1), pltpu.roll(x, 2, 1))


def _pack(x):
    return pltpu.bitcast(x.astype(BF16), U32)


def _unpack(x):
    return pltpu.bitcast(x, BF16)


def _kernel(x_hbm, wa_hbm, woa_hbm, wb_hbm, wob_hbm, out_hbm,
            xio, xres, xsave, wst, wost, wst2, wost2, wak, wvq, woa, wb, wob, hb, hall, h2b, ob,
            qbuf0, qbuf1, zref, zvec, kall, kbuf, vbuf, qs, ks, vt, ots, pb0, pb1, pb2, pb3,
            wsems, xsems, sems, osems):
    nblk = S // BM
    qbuf = (qbuf0, qbuf1)
    pbufs = (pb0, pb1, pb2, pb3)
    zref[0] = 0
    zvec[...] = jnp.zeros(zvec.shape, U32)
    pr = 128
    nwc = D // pr
    sec_q, sec_k, sec_v = 0, 1, 2

    def wak_copy(c):
        r = pl.multiple_of(c * pr, pr)
        return pltpu.make_async_copy(wa_hbm.at[pl.ds(r, pr), pl.ds(sec_k * D, D)],
                                     wst.at[pl.ds(r, pr), pl.ds(sec_k * D, D)], wsems.at[c])

    def x_copy(j):
        r = pl.multiple_of(j * BM, BM)
        return pltpu.make_async_copy(x_hbm.at[pl.ds(r, BM), :], xio.at[pl.ds(r, BM), :],
                                     xsems.at[j])

    def sec_copy(sec, k):
        return pltpu.make_async_copy(wa_hbm.at[:, pl.ds(sec * D, D)], wst.at[:, pl.ds(sec * D, D)],
                                     sems.at[k])

    cp_wav = sec_copy(sec_v, 0)
    cp_waq = sec_copy(sec_q, 1)
    cp_woa = pltpu.make_async_copy(woa_hbm, wost, sems.at[2])
    cp_wb = pltpu.make_async_copy(wb_hbm, wst2, sems.at[3])
    cp_wob = pltpu.make_async_copy(wob_hbm, wost2, sems.at[4])
    ahead = 3
    for c in range(ahead):
        wak_copy(c).start()

    for t in range(NT):
        kall[t, 0:HALO, :] = jnp.zeros((HALO, 128), F32)
        vbuf[t, BM:BM + HALO, :] = jnp.zeros((HALO, 128), F32)

    def perm_body(c, carry):
        wak_copy(c).wait()

        @pl.when(c + ahead < nwc)
        def _():
            wak_copy(jnp.minimum(c + ahead, nwc - 1)).start()

        @pl.when(c + ahead >= nwc)
        def _():
            x_copy(jnp.maximum(c + ahead - nwc, 0)).start()

        r = pl.multiple_of(c * pr, pr)
        r2 = pl.multiple_of(c * (pr // 2), pr // 2)
        w32 = _pack(wst[pl.ds(r, pr), sec_k * D:(sec_k + 1) * D])
        wak[pl.ds(r2, pr // 2), :] = _permute_cols(w32)
        return carry

    with jax.named_scope("perm_cols"):
        lax.fori_loop(0, nwc, perm_body, 0)

    for prio, group in ((0, (cp_wav,)), (0, (x_copy(3), x_copy(4))), (0, (cp_waq,)),
                        (0, (x_copy(5), x_copy(6), x_copy(7))), (1, (cp_woa,)), (1, (cp_wb,)),
                        (1, (cp_wob,))):
        @pl.when(zref[0] == 0)
        def _(prio=prio, group=group):
            for cp in group:
                cp.start(priority=prio)

    def repack(src, dst):
        step = 64

        def body(i, carry):
            r = pl.multiple_of(i * step, step)
            r2 = pl.multiple_of(i * (step // 2), step // 2)
            dst[pl.ds(r2, step // 2), :] = _pack(src[pl.ds(r, step), :])
            return carry

        lax.fori_loop(0, D // step, body, 0)

    def permo_body(t, carry):
        c0 = pl.multiple_of(t * 128, 128)
        woa[:, pl.ds(c0, 128)] = _permute_rows(_pack(wost[:, pl.ds(c0, 128)]))
        return carry

    lane = lax.broadcasted_iota(jnp.int32, (RG, 128), 1)
    rowi = lax.broadcasted_iota(jnp.int32, (RG, 128), 0)

    ties = []

    def tile_dot(lhs_ref, w_ref, n):
        lhs = lhs_ref[...]
        for e in ties:
            e[0] -= 1
        due = [e[1] for e in ties if e[0] <= 0]
        ties[:] = [e for e in ties if e[0] > 0]
        if due:
            first = functools.reduce(lambda u, v: u | v, due, lhs[0:8, 0:128])
            top = jnp.concatenate([first, lhs[0:8, 128:]], axis=1)
            lhs = jnp.concatenate([top, lhs[8:, :]], axis=0)
        return jnp.dot(_unpack(lhs), _unpack(w_ref[:, n * NC:(n + 1) * NC]),
                       preferred_element_type=F32)

    def add_tie(lag, x32):
        vregs = [x32[j * 8:(j + 1) * 8, c * 128:(c + 1) * 128]
                 for j in range(x32.shape[0] // 8) for c in range(x32.shape[1] // 128)]
        ties.append([lag, functools.reduce(lambda u, v: u | v, vregs) & zvec[...]])

    def pack_t(val):
        pt = _pack(val.T)
        add_tie(LAG, pt)
        return pt

    def paced_layernorm(x, lag0, step):
        if lag0 is None:
            return _pack(_layernorm(x))
        hs = []
        for j in range(CM // RG):
            hs.append(_pack(_layernorm(x[j * RG:(j + 1) * RG, :])))
            add_tie(int(lag0 + j * step), hs[-1])
        return jnp.concatenate(hs, axis=0)

    tpc = NC // 128

    def local_vq(h_ref, off, i, lo=0, hi=2 * NT):
        for n in range(lo, hi):
            slot, t = divmod(n, NT)
            val = tile_dot(h_ref, wvq.at[slot], t)
            if slot == 1:
                qbuf[off // CM][t, 0:CM, :] = val
            else:
                vbuf[t, HALO + off:HALO + off + CM, :] = val
                if off == 0:
                    first = jnp.broadcast_to(val[0:1, :], (HALO, 128))
                    vbuf[t, 0:HALO, :] = jnp.where(i == 0, first, vbuf[t, 0:HALO, :])

    def local_attn(o_ref, off, i, lag0, step):
        zero = zref[0]
        for g in range(CM // RG):
            base = HALO + off + g * RG
            qg = [qbuf[off // CM][t, pl.ds(pl.multiple_of(zero + g * RG, RG), RG), :] for t in range(NT)]
            logit = []
            for w in range(WIN):
                a = base - DIL * w
                part = qg[0] * kbuf[0, a:a + RG, :]
                for t in range(1, NT):
                    part = part + qg[t] * kbuf[t, a:a + RG, :]
                lg = _group_sum4(part, lane) * QSCALE
                if off == 0 and g == 0 and w > 0:
                    lg = jnp.where(rowi + i * BM >= DIL * w, lg, MASKED)
                logit.append(lg)
            m = functools.reduce(jnp.maximum, logit)
            p = [jnp.exp2(lg - m) for lg in logit]
            inv = 1.0 / functools.reduce(lambda u, v: u + v, p)
            if lag0 is not None:
                add_tie(int(lag0 + g * step), pltpu.bitcast(inv, U32))
            og = []
            for t in range(NT):
                acc = p[0] * vbuf[t, base:base + RG, :]
                for w in range(1, WIN):
                    a = base - DIL * w
                    acc = acc + p[w] * vbuf[t, a:a + RG, :]
                og.append(_pack(acc * inv))
                o_ref[g * RG // 2:(g + 1) * RG // 2, t * 128:(t + 1) * 128] = og[-1]

    def full_qkv(h_ref, r, lo=0, hi=3 * D // NC, kfirst=False):
        r2 = pl.multiple_of(r >> 1, CM // 2)
        order = list(range(2 * D // NC, 3 * D // NC)) + list(range(2 * D // NC))
        if kfirst:
            order = list(range(NT, 3 * NT)) + list(range(NT))
        for n in order[lo:hi]:
            res = tile_dot(h_ref, wb, n)
            for u in range(tpc):
                sec, t = divmod(n * tpc + u, NT)
                val = res[:, u * 128:(u + 1) * 128]
                if sec == 0:
                    qs[t * 64:(t + 1) * 64, pl.ds(r, CM)] = pack_t(val * QSCALE)
                elif sec == 1:
                    ks[t, pl.ds(r2, CM // 2), :] = _pack(val)
                else:
                    vt[t * 64:(t + 1) * 64, pl.ds(r, CM)] = pack_t(val)

    def normalize(pair, r, ch, lag0=None, step=None, gated=False):
        x = jnp.where(pair == 0, xio[pl.ds(r, CM), :].astype(F32), xres[pl.ds(r, CM), :])
        xres[pl.ds(r, CM), :] = x
        if gated:
            gate = pltpu.bitcast(pltpu.bitcast(kall[0, 0:8, :], U32) & zvec[...], F32)
            head = x[:, 0:128] + jnp.concatenate([gate] * (CM // 8), axis=0)
            x = jnp.concatenate([head, x[:, 128:]], axis=1)
        h = paced_layernorm(x, lag0, step)
        hb[ch] = h
        hall[pl.ds(pl.multiple_of(r >> 1, CM // 2), CM // 2), :] = h

    def key_phase(pair):
        @pl.when(pair == 0)
        def _():
            x_copy(0).wait()

        normalize(pair, 0, 0)

        def body(j, c):
            @pl.when(pair == 0)
            def _():
                x_copy(2 * j + 1).wait()

                @pl.when(j + 1 < nblk // 2)
                def _():
                    x_copy(jnp.minimum(2 * j + 2, nblk - 1)).wait()

                @pl.when(j == 1)
                def _():
                    cp_wav.wait()

                @pl.when(j == 2)
                def _():
                    cp_waq.wait()

            r0 = pl.multiple_of(j * (2 * BM), 2 * BM)
            nsub = 2 * BM // CM
            rows = [pl.multiple_of(r0 + u * CM, CM) for u in range(nsub)]
            rows.append(pl.multiple_of(jnp.minimum(r0 + 2 * BM, S - BM), BM))

            def keys(u, lo, hi):
                for t in range(lo, hi):
                    kall[t, pl.ds(pl.multiple_of(HALO + rows[u], 8), CM), :] = tile_dot(
                        hb.at[u % 2], wak, t)

            sec = jnp.where(j == 0, sec_k, jnp.where(j == 1, sec_v, sec_q))
            c0 = pl.multiple_of(sec * D, D)
            for u in range(nsub):
                keys(u, 0, KS1)
                normalize(pair, rows[u + 1], (u + 1) % 2, KL0, KLS, True)
                for cc in range(u * nwc // nsub, (u + 1) * nwc // nsub):
                    w32 = _pack(wst[cc * pr:(cc + 1) * pr, pl.ds(c0, D)])
                    wvq[j >> 1, cc * pr // 2:(cc + 1) * pr // 2, :] = _permute_cols(w32)
                keys(u, KS1, NT)
            assert not ties
            return c

        with jax.named_scope("key_phase"):
            lax.fori_loop(0, nblk // 2, body, 0)

        @pl.when(pair == 0)
        def _():
            cp_woa.wait()
            lax.fori_loop(0, NT, permo_body, 0)
            cp_wb.wait()
            repack(wst2, wb)

    def row_phase(pair):
        def body(i, c):
            @pl.when(jnp.logical_and(pair == 0, i == 1))
            def _():
                cp_wob.wait()
                repack(wost2, wob)

            r0 = pl.multiple_of(i * BM, BM)
            rs = [r0, pl.multiple_of(r0 + CM, CM)]
            hs = [hall.at[pl.ds(pl.multiple_of(r >> 1, CM // 2), CM // 2), :] for r in rs]

            def local_out(ch):
                y = jnp.concatenate([tile_dot(ob.at[ch], woa, n) for n in range(D // NC)], axis=1)
                x2 = xres[pl.ds(rs[ch], CM), :] + y
                xres[pl.ds(rs[ch], CM), :] = x2
                xsave[pl.ds(rs[ch], CM), :] = x2
                h2b[ch] = paced_layernorm(x2, NL0, (NLS, NLT)[ch])

            for t in range(NT):
                vbuf[t, 0:HALO, :] = vbuf[t, BM:BM + HALO, :]
            local_vq(hs[0], 0, i, 0, 1)
            for t in range(NT):
                kt = kall[t, pl.ds(r0, HALO + BM), :]
                kbuf[t] = kt
                if CL0 is not None:
                    add_tie(CL0 + t, pltpu.bitcast(kt, U32))
            local_vq(hs[0], 0, i, 1)
            if AEARLY:
                local_attn(ob.at[0], 0, i, AL0, ALS)
            local_vq(hs[1], CM, i, 0, SPLIT1)
            if not AEARLY:
                local_attn(ob.at[0], 0, i, None, None)
            local_out(0)
            local_vq(hs[1], CM, i, SPLIT1)
            local_attn(ob.at[1], CM, i, BL0, BLS)
            full_qkv(h2b.at[0], rs[0], 0, SPLIT2, True)
            local_out(1)
            full_qkv(h2b.at[0], rs[0], SPLIT2, 3 * NT, True)
            full_qkv(h2b.at[1], rs[1])
            assert not ties
            return c

        with jax.named_scope("row_phase"):
            lax.fori_loop(0, nblk, body, 0)

    early = QB // OB

    def out_copy(i):
        r0 = pl.multiple_of(i * OB, OB)
        return pltpu.make_async_copy(xio.at[pl.ds(r0, OB), :], out_hbm.at[pl.ds(r0, OB), :],
                                     osems.at[i])

    def write_out(lo, hi):
        def body(i, c):
            r0 = pl.multiple_of(i * OB, OB)
            xio[pl.ds(r0, OB), :] = xres[pl.ds(r0, OB), :].astype(BF16)
            out_copy(i).start()
            return c

        lax.fori_loop(lo, hi, body, 0)

    nt_dims = (((1,), (1,)), ((), ()))

    def masked_q(q32, hp):
        head = lax.broadcasted_iota(jnp.int32, q32.shape, 0) >> (DH.bit_length() - 2)
        return _unpack(jnp.where(head == hp, q32, jnp.uint32(0)))

    def padded_qt(g, hp, q0, nq):
        hr = DH // 2
        qt = qs[pl.ds(pl.multiple_of(g * 64 + hp * hr, hr), hr), pl.ds(q0, nq)]
        parts = [jnp.zeros((hp * hr, nq), U32), qt, jnp.zeros(((HPT - 1 - hp) * hr, nq), U32)]
        return _unpack(jnp.concatenate([x for x in parts if x.shape[0]], axis=0))

    def add_oproj(ot, g, q0, nq):
        g64 = pl.multiple_of(g * 64, 64)
        for j in range(nq // OS):
            y = jnp.dot(ot[:, j * OS:(j + 1) * OS].T.astype(BF16), _unpack(wob[pl.ds(g64, 64), :]),
                        preferred_element_type=F32)
            r = pl.multiple_of(q0 + j * OS, OS)
            xres[pl.ds(r, OS), :] = xres[pl.ds(r, OS), :] + y

    def full_attn(pair):
        nqb = S // QB

        def body(it, bad):
            @pl.when(jnp.logical_and(pair == 1, it == NT))
            def _():
                write_out(0, early)

            g = it & (NT - 1)
            qh = it >> (NT.bit_length() - 1)
            q0 = pl.multiple_of(qh * QB, QB)
            zero = zref[0]
            acc = [None] * HPT
            l8 = [None] * HPT

            def pv(hp, t, buf):
                r0 = pl.multiple_of(g * 64 + hp * (DH // 2), DH // 2)
                vc = _unpack(vt[pl.ds(r0, DH // 2), t * KC:(t + 1) * KC])
                a = jnp.dot(vc, _unpack(buf[zero]), preferred_element_type=F32)
                acc[hp] = a if acc[hp] is None else acc[hp] + a

            pending = None
            for hp in range(HPT):
                w = padded_qt(g, hp, q0, QB)
                for t in range(S // KC):
                    kc = _unpack(ks[g, t * KC // 2:(t + 1) * KC // 2, :])
                    p = jnp.exp2(jnp.dot(kc, w, preferred_element_type=F32))
                    part = jnp.sum(p.reshape(KC // 8, 8, QB), axis=0)
                    l8[hp] = part if l8[hp] is None else l8[hp] + part
                    buf = pbufs[(hp * (S // KC) + t) % len(pbufs)]
                    buf[0] = _pack(p)
                    if pending is not None:
                        pv(*pending)
                    pending = (hp, t, buf)
            pv(*pending)
            outs = []
            for hp in range(HPT):
                l = jnp.sum(l8[hp], axis=0, keepdims=True)
                o = acc[hp] * (1.0 / l)
                outs.append(o)
                ok = (jnp.abs(o) < O_HI) & (l > L_LO) & (l < L_HI)
                nbad = jnp.where(ok, 0.0, 1.0)
                nbad = jnp.max(nbad.reshape(DH // 8, 8, QB), axis=0)
                for j in range(QB // 128):
                    bad = jnp.maximum(bad, nbad[:, j * 128:(j + 1) * 128])
            add_oproj(jnp.concatenate(outs, axis=0), g, q0, QB)
            return bad

        with jax.named_scope("full_attn"):
            bad = lax.fori_loop(0, NT * nqb, body, jnp.zeros((8, 128), F32))

        @pl.when(jnp.max(bad) > 0.0)
        def _():
            nq = S // FQ

            def restore(i, c):
                r = pl.multiple_of(i * 32, 32)
                xres[pl.ds(r, 32), :] = xsave[pl.ds(r, 32), :]
                return c

            lax.fori_loop(0, S // 32, restore, 0)

            def fb_body(it, c):
                g = it // nq
                q0 = pl.multiple_of((it % nq) * FQ, FQ)
                q32 = qs[pl.ds(pl.multiple_of(g * 64, 64), 64), pl.ds(q0, FQ)]

                def head_body(hp, c2):
                    r0 = pl.multiple_of(g * 64 + hp * (DH // 2), DH // 2)
                    s = jnp.dot(_unpack(ks[g]), masked_q(q32, hp), preferred_element_type=F32)
                    p = jnp.exp2(s - jnp.max(s, axis=0, keepdims=True))
                    l = jnp.sum(p, axis=0, keepdims=True)
                    acc = jnp.dot(_unpack(vt[pl.ds(r0, DH // 2), :]), p.astype(BF16),
                                  preferred_element_type=F32)
                    ots[pl.ds(pl.multiple_of(hp * DH, DH), DH), :] = acc * (1.0 / l)
                    return c2

                lax.fori_loop(0, HPT, head_body, 0)
                add_oproj(ots[...], g, q0, FQ)
                return c

            lax.fori_loop(0, NT * nq, fb_body, 0)

            @pl.when(pair == 1)
            def _():
                for i in range(early):
                    out_copy(i).wait()
                write_out(0, early)

    def pair_body(pair, c):
        key_phase(pair)
        row_phase(pair)
        full_attn(pair)
        return c

    with jax.named_scope("pairs"):
        lax.fori_loop(0, 2, pair_body, 0)

    with jax.named_scope("out_phase"):
        write_out(early, S // OB)
        for i in range(S // OB):
            out_copy(i).wait()


@jax.jit
def pallas_interleave_layers__sliding_local_dilated__softmax_full_mha__prompt_kernel(
    A_x: jax.Array,
    A_wqkv: jax.Array,
    A_wo: jax.Array,
    B_x: jax.Array,
    B_wqkv: jax.Array,
    B_wo: jax.Array,
):
    del B_x
    x = A_x.reshape(S, D)
    hbm = pl.BlockSpec(memory_space=pl.ANY)
    out = pl.pallas_call(
        _kernel,
        out_shape=jax.ShapeDtypeStruct((S, D), BF16),
        in_specs=[hbm] * 5,
        out_specs=hbm,
        scratch_shapes=[
            pltpu.VMEM((S, D), BF16),
            pltpu.VMEM((S, D), F32),
            pltpu.VMEM((S, D), F32),
            pltpu.VMEM((D, 3 * D), BF16),
            pltpu.VMEM((D, D), BF16),
            pltpu.VMEM((D, 3 * D), BF16),
            pltpu.VMEM((D, D), BF16),
            pltpu.VMEM((D // 2, D), U32),
            pltpu.VMEM((2, D // 2, D), U32),
            pltpu.VMEM((D // 2, D), U32),
            pltpu.VMEM((D // 2, 3 * D), U32),
            pltpu.VMEM((D // 2, D), U32),
            pltpu.VMEM((BM // CM, CM // 2, D), U32),
            pltpu.VMEM((S // 2, D), U32),
            pltpu.VMEM((BM // CM, CM // 2, D), U32),
            pltpu.VMEM((BM // CM, CM // 2, D), U32),
            pltpu.VMEM((NT, CM + 8, 128), F32),
            pltpu.VMEM((NT, CM + 8, 128), F32),
            pltpu.SMEM((1,), jnp.int32),
            pltpu.VMEM((8, 128), U32),
            pltpu.VMEM((NT, HALO + S, 128), F32),
            pltpu.VMEM((NT, HALO + BM, 128), F32),
            pltpu.VMEM((NT, HALO + BM, 128), F32),
            pltpu.VMEM((D // 2, S), U32),
            pltpu.VMEM((NT, S // 2, 128), U32),
            pltpu.VMEM((D // 2, S), U32),
            pltpu.VMEM((128, FQ), F32),
            pltpu.VMEM((1, KC // 2, QB), U32),
            pltpu.VMEM((1, KC // 2, QB), U32),
            pltpu.VMEM((1, KC // 2, QB), U32),
            pltpu.VMEM((1, KC // 2, QB), U32),
            pltpu.SemaphoreType.DMA((D // 128,)),
            pltpu.SemaphoreType.DMA((S // BM,)),
            pltpu.SemaphoreType.DMA((5,)),
            pltpu.SemaphoreType.DMA((S // OB,)),
        ],
        compiler_params=pltpu.CompilerParams(vmem_limit_bytes=110 * 1024 * 1024),
        name="interleaved_attention_stack",
    )(x, A_wqkv, A_wo, B_wqkv, B_wo)
    return out.reshape(1, S, D)
```

```python
import functools
import math

import jax
import jax.numpy as jnp
from jax import lax
import jax.experimental.pallas as pl
import jax.experimental.pallas.tpu as pltpu

S = 2048
D = 1024
H = 32
DH = D // H
NT = D // 128
HPT = 128 // DH
WIN = 8
DIL = 2
HALO = 16
EPS = 1e-5
LOG2E = math.log2(math.e)
QSCALE = (DH ** -0.5) * LOG2E
MASKED = -1e9 * LOG2E

BM = 256
KB = 512
CM = 128
NC = 128
SPLIT1 = 12
KS1 = 0
KS2 = 1
KL0 = 4
KLS = 0.6
NL0 = None
NLS = 0.3
NLT = 0.7
CL0 = 2
AEARLY = 0
AL0 = None
ALS = 1
BL0 = 6
BLS = 1
SPLIT2 = 16
LAG = 6
RG = 16
KC = 512
QB = 1024
OS = 128
OB = 128
FQ = 128

L_LO = 2.0 ** -40
L_HI = 2.0 ** 90
O_HI = 3.0e38

F32 = jnp.float32
BF16 = jnp.bfloat16
U32 = jnp.uint32


def _layernorm(x):
    mu = jnp.mean(x, axis=-1, keepdims=True)
    xc = x - mu
    var = jnp.mean(xc * xc, axis=-1, keepdims=True)
    return xc * lax.rsqrt(var + EPS)


def _permute_cols(w32):
    rows = w32.shape[0]
    lane = lax.broadcasted_iota(jnp.int32, (rows, 128), 1)
    tiles = [w32[:, t * 128:(t + 1) * 128] for t in range(NT)]
    for b in range(3):
        sh = 4 << b
        low = (lane & sh) == 0
        for a in range(NT):
            if a & (1 << b):
                continue
            c = a | (1 << b)
            ta, tc = tiles[a], tiles[c]
            tiles[a] = jnp.where(low, ta, pltpu.roll(tc, sh, 1))
            tiles[c] = jnp.where(low, pltpu.roll(ta, 128 - sh, 1), tc)
    return jnp.concatenate(tiles, axis=1)


def _permute_rows(w32):
    ncols = w32.shape[1]
    nv = D // 16
    v = [w32[i * 8:(i + 1) * 8, :] for i in range(nv)]
    sub = lax.broadcasted_iota(jnp.int32, (8, ncols), 0)
    for vb, sh in ((8, 2), (16, 4)):
        low = (sub & sh) == 0
        for a in range(nv):
            if a & vb:
                continue
            c = a | vb
            ta, tc = v[a], v[c]
            v[a] = jnp.where(low, ta, pltpu.roll(tc, sh, 0))
            v[c] = jnp.where(low, pltpu.roll(ta, 8 - sh, 0), tc)
    def src(i):
        b0, b5 = i & 1, (i >> 5) & 1
        return (i & ~33) | (b0 << 5) | b5
    return jnp.concatenate([v[src(i)] for i in range(nv)], axis=0)


def _group_sum4(x, lane):
    b0 = (lane & 1) == 0
    x = x + jnp.where(b0, pltpu.roll(x, 127, 1), pltpu.roll(x, 1, 1))
    b1 = (lane & 2) == 0
    return x + jnp.where(b1, pltpu.roll(x, 126, 1), pltpu.roll(x, 2, 1))


def _pack(x):
    return pltpu.bitcast(x.astype(BF16), U32)


def _unpack(x):
    return pltpu.bitcast(x, BF16)


def _kernel(x_hbm, wa_hbm, woa_hbm, wb_hbm, wob_hbm, out_hbm,
            xio, xres, xsave, wst, wost, wst2, wost2, wak, wvq, woa, wb, wob, hb, hall, h2b, ob,
            qbuf0, qbuf1, zref, zvec, kall, kbuf, vbuf, qs, ks, vt, ots, pb0, pb1, pb2, pb3,
            wsems, xsems, sems, osems):
    nblk = S // BM
    qbuf = (qbuf0, qbuf1)
    pbufs = (pb0, pb1, pb2, pb3)
    zref[0] = 0
    zvec[...] = jnp.zeros(zvec.shape, U32)
    pr = 128
    nwc = D // pr
    sec_q, sec_k, sec_v = 0, 1, 2

    def wak_copy(c):
        r = pl.multiple_of(c * pr, pr)
        return pltpu.make_async_copy(wa_hbm.at[pl.ds(r, pr), pl.ds(sec_k * D, D)],
                                     wst.at[pl.ds(r, pr), pl.ds(sec_k * D, D)], wsems.at[c])

    x_cuts = [0, CM] + [min(CM + (j + 1) * KB, S) for j in range(S // KB)]
    cp_x = [pltpu.make_async_copy(x_hbm.at[pl.ds(lo, hi - lo), :], xio.at[pl.ds(lo, hi - lo), :],
                                  xsems.at[k])
            for k, (lo, hi) in enumerate(zip(x_cuts[:-1], x_cuts[1:]))]

    def sec_copy(sec, k):
        return pltpu.make_async_copy(wa_hbm.at[:, pl.ds(sec * D, D)], wst.at[:, pl.ds(sec * D, D)],
                                     sems.at[k])

    cp_wav = sec_copy(sec_v, 0)
    cp_waq = sec_copy(sec_q, 1)
    cp_woa = pltpu.make_async_copy(woa_hbm, wost, sems.at[2])
    cp_wb = pltpu.make_async_copy(wb_hbm, wst2, sems.at[3])
    cp_wob = pltpu.make_async_copy(wob_hbm, wost2, sems.at[4])
    ahead = 3
    for c in range(ahead):
        wak_copy(c).start()

    for t in range(NT):
        kall[t, 0:HALO, :] = jnp.zeros((HALO, 128), F32)
        vbuf[t, BM:BM + HALO, :] = jnp.zeros((HALO, 128), F32)

    def perm_body(c, carry):
        wak_copy(c).wait()

        @pl.when(c + ahead < nwc)
        def _():
            wak_copy(jnp.minimum(c + ahead, nwc - 1)).start()

        for k, cp in enumerate((cp_x[0], cp_x[1], cp_wav)):
            @pl.when(c + ahead == nwc + k)
            def _(cp=cp):
                cp.start()

        r = pl.multiple_of(c * pr, pr)
        r2 = pl.multiple_of(c * (pr // 2), pr // 2)
        w32 = _pack(wst[pl.ds(r, pr), sec_k * D:(sec_k + 1) * D])
        wak[pl.ds(r2, pr // 2), :] = _permute_cols(w32)
        return carry

    with jax.named_scope("perm_cols"):
        lax.fori_loop(0, nwc, perm_body, 0)

    def repack(src, dst):
        step = 64

        def body(i, carry):
            r = pl.multiple_of(i * step, step)
            r2 = pl.multiple_of(i * (step // 2), step // 2)
            dst[pl.ds(r2, step // 2), :] = _pack(src[pl.ds(r, step), :])
            return carry

        lax.fori_loop(0, D // step, body, 0)

    def permo_body(t, carry):
        c0 = pl.multiple_of(t * 128, 128)
        woa[:, pl.ds(c0, 128)] = _permute_rows(_pack(wost[:, pl.ds(c0, 128)]))
        return carry

    lane = lax.broadcasted_iota(jnp.int32, (RG, 128), 1)
    rowi = lax.broadcasted_iota(jnp.int32, (RG, 128), 0)

    ties = []

    def tile_dot(lhs_ref, w_ref, n):
        lhs = lhs_ref[...]
        for e in ties:
            e[0] -= 1
        due = [e[1] for e in ties if e[0] <= 0]
        ties[:] = [e for e in ties if e[0] > 0]
        if due:
            first = functools.reduce(lambda u, v: u | v, due, lhs[0:8, 0:128])
            top = jnp.concatenate([first, lhs[0:8, 128:]], axis=1)
            lhs = jnp.concatenate([top, lhs[8:, :]], axis=0)
        return jnp.dot(_unpack(lhs), _unpack(w_ref[:, n * NC:(n + 1) * NC]),
                       preferred_element_type=F32)

    def add_tie(lag, x32):
        vregs = [x32[j * 8:(j + 1) * 8, c * 128:(c + 1) * 128]
                 for j in range(x32.shape[0] // 8) for c in range(x32.shape[1] // 128)]
        ties.append([lag, functools.reduce(lambda u, v: u | v, vregs) & zvec[...]])

    def pack_t(val):
        pt = _pack(val.T)
        add_tie(LAG, pt)
        return pt

    def paced_layernorm(x, lag0, step):
        if lag0 is None:
            return _pack(_layernorm(x))
        hs = []
        for j in range(CM // RG):
            hs.append(_pack(_layernorm(x[j * RG:(j + 1) * RG, :])))
            add_tie(int(lag0 + j * step), hs[-1])
        return jnp.concatenate(hs, axis=0)

    tpc = NC // 128

    def local_vq(h_ref, off, i, lo=0, hi=2 * NT):
        for n in range(lo, hi):
            slot, t = divmod(n, NT)
            val = tile_dot(h_ref, wvq.at[slot], t)
            if slot == 1:
                qbuf[off // CM][t, 0:CM, :] = val
            else:
                vbuf[t, HALO + off:HALO + off + CM, :] = val
                if off == 0:
                    first = jnp.broadcast_to(val[0:1, :], (HALO, 128))
                    vbuf[t, 0:HALO, :] = jnp.where(i == 0, first, vbuf[t, 0:HALO, :])

    def local_attn(o_ref, off, i, lag0, step):
        zero = zref[0]
        for g in range(CM // RG):
            base = HALO + off + g * RG
            qg = [qbuf[off // CM][t, pl.ds(pl.multiple_of(zero + g * RG, RG), RG), :] for t in range(NT)]
            logit = []
            for w in range(WIN):
                a = base - DIL * w
                part = qg[0] * kbuf[0, a:a + RG, :]
                for t in range(1, NT):
                    part = part + qg[t] * kbuf[t, a:a + RG, :]
                lg = _group_sum4(part, lane) * QSCALE
                if off == 0 and g == 0 and w > 0:
                    lg = jnp.where(rowi + i * BM >= DIL * w, lg, MASKED)
                logit.append(lg)
            m = functools.reduce(jnp.maximum, logit)
            p = [jnp.exp2(lg - m) for lg in logit]
            inv = 1.0 / functools.reduce(lambda u, v: u + v, p)
            if lag0 is not None:
                add_tie(int(lag0 + g * step), pltpu.bitcast(inv, U32))
            og = []
            for t in range(NT):
                acc = p[0] * vbuf[t, base:base + RG, :]
                for w in range(1, WIN):
                    a = base - DIL * w
                    acc = acc + p[w] * vbuf[t, a:a + RG, :]
                og.append(_pack(acc * inv))
                o_ref[g * RG // 2:(g + 1) * RG // 2, t * 128:(t + 1) * 128] = og[-1]

    def full_qkv(h_ref, r, lo=0, hi=3 * D // NC, kfirst=False):
        r2 = pl.multiple_of(r >> 1, CM // 2)
        order = list(range(2 * D // NC, 3 * D // NC)) + list(range(2 * D // NC))
        if kfirst:
            order = list(range(NT, 3 * NT)) + list(range(NT))
        for n in order[lo:hi]:
            res = tile_dot(h_ref, wb, n)
            for u in range(tpc):
                sec, t = divmod(n * tpc + u, NT)
                val = res[:, u * 128:(u + 1) * 128]
                if sec == 0:
                    qs[t * 64:(t + 1) * 64, pl.ds(r, CM)] = pack_t(val * QSCALE)
                elif sec == 1:
                    ks[t, pl.ds(r2, CM // 2), :] = _pack(val)
                else:
                    vt[t * 64:(t + 1) * 64, pl.ds(r, CM)] = pack_t(val)

    def normalize(pair, r, ch, lag0=None, step=None, gated=False):
        x = jnp.where(pair == 0, xio[pl.ds(r, CM), :].astype(F32), xres[pl.ds(r, CM), :])
        xres[pl.ds(r, CM), :] = x
        if gated:
            gate = pltpu.bitcast(pltpu.bitcast(kall[0, 0:8, :], U32) & zvec[...], F32)
            head = x[:, 0:128] + jnp.concatenate([gate] * (CM // 8), axis=0)
            x = jnp.concatenate([head, x[:, 128:]], axis=1)
        h = paced_layernorm(x, lag0, step)
        hb[ch] = h
        hall[pl.ds(pl.multiple_of(r >> 1, CM // 2), CM // 2), :] = h

    def key_phase(pair):
        @pl.when(pair == 0)
        def _():
            cp_x[0].wait()
            cp_x[2].start()

        normalize(pair, 0, 0)

        def body(j, c):
            @pl.when(pair == 0)
            def _():
                @pl.when(j == 0)
                def _():
                    cp_x[1].wait()
                    cp_waq.start()
                    cp_woa.start(priority=1)
                    cp_wb.start(priority=1)

                @pl.when(j == 1)
                def _():
                    cp_x[3].start()
                    cp_x[4].start()
                    cp_x[2].wait()
                    cp_wav.wait()

                @pl.when(j == 2)
                def _():
                    cp_wob.start(priority=1)
                    cp_x[3].wait()
                    cp_waq.wait()

                @pl.when(j == 3)
                def _():
                    cp_x[4].wait()

            r0 = pl.multiple_of(j * KB, KB)
            nsub = KB // CM
            rows = [pl.multiple_of(r0 + u * CM, CM) for u in range(nsub)]
            rows.append(pl.multiple_of(jnp.minimum(r0 + KB, S - CM), CM))

            def keys(u, lo, hi):
                for t in range(lo, hi):
                    kall[t, pl.ds(pl.multiple_of(HALO + rows[u], 8), CM), :] = tile_dot(
                        hb.at[u % 2], wak, t)

            sec = jnp.where(j == 0, sec_k, jnp.where(j == 1, sec_v, sec_q))
            c0 = pl.multiple_of(sec * D, D)
            for u in range(nsub):
                keys(u, 0, KS1)
                normalize(pair, rows[u + 1], (u + 1) % 2, KL0, KLS, True)
                for cc in range(u * nwc // nsub, (u + 1) * nwc // nsub):
                    w32 = _pack(wst[cc * pr:(cc + 1) * pr, pl.ds(c0, D)])
                    wvq[j >> 1, cc * pr // 2:(cc + 1) * pr // 2, :] = _permute_cols(w32)
                keys(u, KS1, NT)
            assert not ties
            return c

        with jax.named_scope("key_phase"):
            lax.fori_loop(0, S // KB, body, 0)

        @pl.when(pair == 0)
        def _():
            cp_woa.wait()
            lax.fori_loop(0, NT, permo_body, 0)
            cp_wb.wait()
            repack(wst2, wb)

    def row_phase(pair):
        def body(i, c):
            @pl.when(jnp.logical_and(pair == 0, i == 1))
            def _():
                cp_wob.wait()
                repack(wost2, wob)

            r0 = pl.multiple_of(i * BM, BM)
            rs = [r0, pl.multiple_of(r0 + CM, CM)]
            hs = [hall.at[pl.ds(pl.multiple_of(r >> 1, CM // 2), CM // 2), :] for r in rs]

            def local_out(ch):
                y = jnp.concatenate([tile_dot(ob.at[ch], woa, n) for n in range(D // NC)], axis=1)
                x2 = xres[pl.ds(rs[ch], CM), :] + y
                xres[pl.ds(rs[ch], CM), :] = x2
                xsave[pl.ds(rs[ch], CM), :] = x2
                h2b[ch] = paced_layernorm(x2, NL0, (NLS, NLT)[ch])

            for t in range(NT):
                vbuf[t, 0:HALO, :] = vbuf[t, BM:BM + HALO, :]
            local_vq(hs[0], 0, i, 0, 1)
            for t in range(NT):
                kt = kall[t, pl.ds(r0, HALO + BM), :]
                kbuf[t] = kt
                if CL0 is not None:
                    add_tie(CL0 + t, pltpu.bitcast(kt, U32))
            local_vq(hs[0], 0, i, 1)
            if AEARLY:
                local_attn(ob.at[0], 0, i, AL0, ALS)
            local_vq(hs[1], CM, i, 0, SPLIT1)
            if not AEARLY:
                local_attn(ob.at[0], 0, i, None, None)
            local_out(0)
            local_vq(hs[1], CM, i, SPLIT1)
            local_attn(ob.at[1], CM, i, BL0, BLS)
            full_qkv(h2b.at[0], rs[0], 0, SPLIT2, True)
            local_out(1)
            full_qkv(h2b.at[0], rs[0], SPLIT2, 3 * NT, True)
            full_qkv(h2b.at[1], rs[1])
            assert not ties
            return c

        with jax.named_scope("row_phase"):
            lax.fori_loop(0, nblk, body, 0)

    early = QB // OB

    def out_copy(i):
        r0 = pl.multiple_of(i * OB, OB)
        return pltpu.make_async_copy(xio.at[pl.ds(r0, OB), :], out_hbm.at[pl.ds(r0, OB), :],
                                     osems.at[i])

    def write_out(lo, hi):
        def body(i, c):
            r0 = pl.multiple_of(i * OB, OB)
            xio[pl.ds(r0, OB), :] = xres[pl.ds(r0, OB), :].astype(BF16)
            out_copy(i).start()
            return c

        lax.fori_loop(lo, hi, body, 0)

    nt_dims = (((1,), (1,)), ((), ()))

    def masked_q(q32, hp):
        head = lax.broadcasted_iota(jnp.int32, q32.shape, 0) >> (DH.bit_length() - 2)
        return _unpack(jnp.where(head == hp, q32, jnp.uint32(0)))

    def padded_qt(g, hp, q0, nq):
        hr = DH // 2
        qt = qs[pl.ds(pl.multiple_of(g * 64 + hp * hr, hr), hr), pl.ds(q0, nq)]
        parts = [jnp.zeros((hp * hr, nq), U32), qt, jnp.zeros(((HPT - 1 - hp) * hr, nq), U32)]
        return _unpack(jnp.concatenate([x for x in parts if x.shape[0]], axis=0))

    def add_oproj(ot, g, q0, nq):
        g64 = pl.multiple_of(g * 64, 64)
        for j in range(nq // OS):
            y = jnp.dot(ot[:, j * OS:(j + 1) * OS].T.astype(BF16), _unpack(wob[pl.ds(g64, 64), :]),
                        preferred_element_type=F32)
            r = pl.multiple_of(q0 + j * OS, OS)
            xres[pl.ds(r, OS), :] = xres[pl.ds(r, OS), :] + y

    def full_attn(pair):
        nqb = S // QB

        def body(it, bad):
            @pl.when(jnp.logical_and(pair == 1, it == NT))
            def _():
                write_out(0, early)

            g = it & (NT - 1)
            qh = it >> (NT.bit_length() - 1)
            q0 = pl.multiple_of(qh * QB, QB)
            zero = zref[0]
            acc = [None] * HPT
            l8 = [None] * HPT

            def pv(hp, t, buf):
                r0 = pl.multiple_of(g * 64 + hp * (DH // 2), DH // 2)
                vc = _unpack(vt[pl.ds(r0, DH // 2), t * KC:(t + 1) * KC])
                a = jnp.dot(vc, _unpack(buf[zero]), preferred_element_type=F32)
                acc[hp] = a if acc[hp] is None else acc[hp] + a

            pending = None
            for hp in range(HPT):
                w = padded_qt(g, hp, q0, QB)
                for t in range(S // KC):
                    kc = _unpack(ks[g, t * KC // 2:(t + 1) * KC // 2, :])
                    p = jnp.exp2(jnp.dot(kc, w, preferred_element_type=F32))
                    part = jnp.sum(p.reshape(KC // 8, 8, QB), axis=0)
                    l8[hp] = part if l8[hp] is None else l8[hp] + part
                    buf = pbufs[(hp * (S // KC) + t) % len(pbufs)]
                    buf[0] = _pack(p)
                    if pending is not None:
                        pv(*pending)
                    pending = (hp, t, buf)
            pv(*pending)
            outs = []
            for hp in range(HPT):
                l = jnp.sum(l8[hp], axis=0, keepdims=True)
                o = acc[hp] * (1.0 / l)
                outs.append(o)
                ok = (jnp.abs(o) < O_HI) & (l > L_LO) & (l < L_HI)
                nbad = jnp.where(ok, 0.0, 1.0)
                nbad = jnp.max(nbad.reshape(DH // 8, 8, QB), axis=0)
                for j in range(QB // 128):
                    bad = jnp.maximum(bad, nbad[:, j * 128:(j + 1) * 128])
            add_oproj(jnp.concatenate(outs, axis=0), g, q0, QB)
            return bad

        with jax.named_scope("full_attn"):
            bad = lax.fori_loop(0, NT * nqb, body, jnp.zeros((8, 128), F32))

        @pl.when(jnp.max(bad) > 0.0)
        def _():
            nq = S // FQ

            def restore(i, c):
                r = pl.multiple_of(i * 32, 32)
                xres[pl.ds(r, 32), :] = xsave[pl.ds(r, 32), :]
                return c

            lax.fori_loop(0, S // 32, restore, 0)

            def fb_body(it, c):
                g = it // nq
                q0 = pl.multiple_of((it % nq) * FQ, FQ)
                q32 = qs[pl.ds(pl.multiple_of(g * 64, 64), 64), pl.ds(q0, FQ)]

                def head_body(hp, c2):
                    r0 = pl.multiple_of(g * 64 + hp * (DH // 2), DH // 2)
                    s = jnp.dot(_unpack(ks[g]), masked_q(q32, hp), preferred_element_type=F32)
                    p = jnp.exp2(s - jnp.max(s, axis=0, keepdims=True))
                    l = jnp.sum(p, axis=0, keepdims=True)
                    acc = jnp.dot(_unpack(vt[pl.ds(r0, DH // 2), :]), p.astype(BF16),
                                  preferred_element_type=F32)
                    ots[pl.ds(pl.multiple_of(hp * DH, DH), DH), :] = acc * (1.0 / l)
                    return c2

                lax.fori_loop(0, HPT, head_body, 0)
                add_oproj(ots[...], g, q0, FQ)
                return c

            lax.fori_loop(0, NT * nq, fb_body, 0)

            @pl.when(pair == 1)
            def _():
                for i in range(early):
                    out_copy(i).wait()
                write_out(0, early)

    def pair_body(pair, c):
        key_phase(pair)
        row_phase(pair)
        full_attn(pair)
        return c

    with jax.named_scope("pairs"):
        lax.fori_loop(0, 2, pair_body, 0)

    with jax.named_scope("out_phase"):
        write_out(early, S // OB)
        for i in range(S // OB):
            out_copy(i).wait()


@jax.jit
def pallas_interleave_layers__sliding_local_dilated__softmax_full_mha__prompt_kernel(
    A_x: jax.Array,
    A_wqkv: jax.Array,
    A_wo: jax.Array,
    B_x: jax.Array,
    B_wqkv: jax.Array,
    B_wo: jax.Array,
):
    del B_x
    x = A_x.reshape(S, D)
    hbm = pl.BlockSpec(memory_space=pl.ANY)
    out = pl.pallas_call(
        _kernel,
        out_shape=jax.ShapeDtypeStruct((S, D), BF16),
        in_specs=[hbm] * 5,
        out_specs=hbm,
        scratch_shapes=[
            pltpu.VMEM((S, D), BF16),
            pltpu.VMEM((S, D), F32),
            pltpu.VMEM((S, D), F32),
            pltpu.VMEM((D, 3 * D), BF16),
            pltpu.VMEM((D, D), BF16),
            pltpu.VMEM((D, 3 * D), BF16),
            pltpu.VMEM((D, D), BF16),
            pltpu.VMEM((D // 2, D), U32),
            pltpu.VMEM((2, D // 2, D), U32),
            pltpu.VMEM((D // 2, D), U32),
            pltpu.VMEM((D // 2, 3 * D), U32),
            pltpu.VMEM((D // 2, D), U32),
            pltpu.VMEM((BM // CM, CM // 2, D), U32),
            pltpu.VMEM((S // 2, D), U32),
            pltpu.VMEM((BM // CM, CM // 2, D), U32),
            pltpu.VMEM((BM // CM, CM // 2, D), U32),
            pltpu.VMEM((NT, CM + 8, 128), F32),
            pltpu.VMEM((NT, CM + 8, 128), F32),
            pltpu.SMEM((1,), jnp.int32),
            pltpu.VMEM((8, 128), U32),
            pltpu.VMEM((NT, HALO + S, 128), F32),
            pltpu.VMEM((NT, HALO + BM, 128), F32),
            pltpu.VMEM((NT, HALO + BM, 128), F32),
            pltpu.VMEM((D // 2, S), U32),
            pltpu.VMEM((NT, S // 2, 128), U32),
            pltpu.VMEM((D // 2, S), U32),
            pltpu.VMEM((128, FQ), F32),
            pltpu.VMEM((1, KC // 2, QB), U32),
            pltpu.VMEM((1, KC // 2, QB), U32),
            pltpu.VMEM((1, KC // 2, QB), U32),
            pltpu.VMEM((1, KC // 2, QB), U32),
            pltpu.SemaphoreType.DMA((D // 128,)),
            pltpu.SemaphoreType.DMA((S // KB + 1,)),
            pltpu.SemaphoreType.DMA((5,)),
            pltpu.SemaphoreType.DMA((S // OB,)),
        ],
        compiler_params=pltpu.CompilerParams(vmem_limit_bytes=110 * 1024 * 1024),
        name="interleaved_attention_stack",
    )(x, A_wqkv, A_wo, B_wqkv, B_wo)
    return out.reshape(1, S, D)
```

```python
import functools
import math

import jax
import jax.numpy as jnp
from jax import lax
import jax.experimental.pallas as pl
import jax.experimental.pallas.tpu as pltpu

S = 2048
D = 1024
H = 32
DH = D // H
NT = D // 128
HPT = 128 // DH
WIN = 8
DIL = 2
HALO = 16
EPS = 1e-5
LOG2E = math.log2(math.e)
QSCALE = (DH ** -0.5) * LOG2E
MASKED = -1e9 * LOG2E

BM = 256
KB = 512
CM = 128
RG = 16
KC = 512
QB = 1024
OS = 128
OB = 128
FQ = 128

SPLIT1 = 12
SPLIT2 = 16
LAG_T = 6
LAG_K = 2
LAG_LN, STEP_LN = 4, 0.6
LAG_SM, STEP_SM = 6, 1

L_LO = 2.0 ** -40
L_HI = 2.0 ** 90
O_HI = 3.0e38

F32 = jnp.float32
BF16 = jnp.bfloat16
U32 = jnp.uint32


def _layernorm(x):
    mu = jnp.mean(x, axis=-1, keepdims=True)
    xc = x - mu
    var = jnp.mean(xc * xc, axis=-1, keepdims=True)
    return xc * lax.rsqrt(var + EPS)


def _permute_cols(w32):
    rows = w32.shape[0]
    lane = lax.broadcasted_iota(jnp.int32, (rows, 128), 1)
    tiles = [w32[:, t * 128:(t + 1) * 128] for t in range(NT)]
    for b in range(3):
        sh = 4 << b
        low = (lane & sh) == 0
        for a in range(NT):
            if a & (1 << b):
                continue
            c = a | (1 << b)
            ta, tc = tiles[a], tiles[c]
            tiles[a] = jnp.where(low, ta, pltpu.roll(tc, sh, 1))
            tiles[c] = jnp.where(low, pltpu.roll(ta, 128 - sh, 1), tc)
    return jnp.concatenate(tiles, axis=1)


def _permute_rows(w32):
    ncols = w32.shape[1]
    nv = D // 16
    v = [w32[i * 8:(i + 1) * 8, :] for i in range(nv)]
    sub = lax.broadcasted_iota(jnp.int32, (8, ncols), 0)
    for vb, sh in ((8, 2), (16, 4)):
        low = (sub & sh) == 0
        for a in range(nv):
            if a & vb:
                continue
            c = a | vb
            ta, tc = v[a], v[c]
            v[a] = jnp.where(low, ta, pltpu.roll(tc, sh, 0))
            v[c] = jnp.where(low, pltpu.roll(ta, 8 - sh, 0), tc)
    def src(i):
        b0, b5 = i & 1, (i >> 5) & 1
        return (i & ~33) | (b0 << 5) | b5
    return jnp.concatenate([v[src(i)] for i in range(nv)], axis=0)


def _group_sum4(x, lane):
    b0 = (lane & 1) == 0
    x = x + jnp.where(b0, pltpu.roll(x, 127, 1), pltpu.roll(x, 1, 1))
    b1 = (lane & 2) == 0
    return x + jnp.where(b1, pltpu.roll(x, 126, 1), pltpu.roll(x, 2, 1))


def _pack(x):
    return pltpu.bitcast(x.astype(BF16), U32)


def _unpack(x):
    return pltpu.bitcast(x, BF16)


def _kernel(x_hbm, wa_hbm, woa_hbm, wb_hbm, wob_hbm, out_hbm,
            xio, xres, xsave, wst, wost, wst2, wost2, wak, wvq, woa, wb, wob, hb, hall, h2b, ob,
            qbuf0, qbuf1, zref, zvec, kall, kbuf, vbuf, qs, ks, vt, ots, pb0, pb1, pb2, pb3,
            wsems, xsems, sems, osems):
    nblk = S // BM
    qbuf = (qbuf0, qbuf1)
    pbufs = (pb0, pb1, pb2, pb3)
    zref[0] = 0
    zvec[...] = jnp.zeros(zvec.shape, U32)
    pr = 128
    nwc = D // pr
    sec_q, sec_k, sec_v = 0, 1, 2

    def wak_copy(c):
        r = pl.multiple_of(c * pr, pr)
        return pltpu.make_async_copy(wa_hbm.at[pl.ds(r, pr), pl.ds(sec_k * D, D)],
                                     wst.at[pl.ds(r, pr), pl.ds(sec_k * D, D)], wsems.at[c])

    x_cuts = [0, CM] + [min(CM + (j + 1) * KB, S) for j in range(S // KB)]
    cp_x = [pltpu.make_async_copy(x_hbm.at[pl.ds(lo, hi - lo), :], xio.at[pl.ds(lo, hi - lo), :],
                                  xsems.at[k])
            for k, (lo, hi) in enumerate(zip(x_cuts[:-1], x_cuts[1:]))]

    def sec_copy(sec, k):
        return pltpu.make_async_copy(wa_hbm.at[:, pl.ds(sec * D, D)], wst.at[:, pl.ds(sec * D, D)],
                                     sems.at[k])

    cp_wav = sec_copy(sec_v, 0)
    cp_waq = sec_copy(sec_q, 1)
    cp_woa = pltpu.make_async_copy(woa_hbm, wost, sems.at[2])
    cp_wb = pltpu.make_async_copy(wb_hbm, wst2, sems.at[3])
    cp_wob = pltpu.make_async_copy(wob_hbm, wost2, sems.at[4])
    ahead = 3
    for c in range(ahead):
        wak_copy(c).start()

    for t in range(NT):
        kall[t, 0:HALO, :] = jnp.zeros((HALO, 128), F32)
        vbuf[t, BM:BM + HALO, :] = jnp.zeros((HALO, 128), F32)

    def perm_body(c, carry):
        wak_copy(c).wait()

        @pl.when(c + ahead < nwc)
        def _():
            wak_copy(jnp.minimum(c + ahead, nwc - 1)).start()

        for k, cp in enumerate((cp_x[0], cp_x[1], cp_wav)):
            @pl.when(c + ahead == nwc + k)
            def _(cp=cp):
                cp.start()

        r = pl.multiple_of(c * pr, pr)
        r2 = pl.multiple_of(c * (pr // 2), pr // 2)
        w32 = _pack(wst[pl.ds(r, pr), sec_k * D:(sec_k + 1) * D])
        wak[pl.ds(r2, pr // 2), :] = _permute_cols(w32)
        return carry

    with jax.named_scope("perm_cols"):
        lax.fori_loop(0, nwc, perm_body, 0)

    def repack(src, dst):
        step = 64

        def body(i, carry):
            r = pl.multiple_of(i * step, step)
            r2 = pl.multiple_of(i * (step // 2), step // 2)
            dst[pl.ds(r2, step // 2), :] = _pack(src[pl.ds(r, step), :])
            return carry

        lax.fori_loop(0, D // step, body, 0)

    def permo_body(t, carry):
        c0 = pl.multiple_of(t * 128, 128)
        woa[:, pl.ds(c0, 128)] = _permute_rows(_pack(wost[:, pl.ds(c0, 128)]))
        return carry

    lane = lax.broadcasted_iota(jnp.int32, (RG, 128), 1)
    rowi = lax.broadcasted_iota(jnp.int32, (RG, 128), 0)

    ties = []

    def tile_dot(lhs_ref, w_ref, n):
        lhs = lhs_ref[...]
        for e in ties:
            e[0] -= 1
        due = [e[1] for e in ties if e[0] <= 0]
        ties[:] = [e for e in ties if e[0] > 0]
        if due:
            first = functools.reduce(lambda u, v: u | v, due, lhs[0:8, 0:128])
            top = jnp.concatenate([first, lhs[0:8, 128:]], axis=1)
            lhs = jnp.concatenate([top, lhs[8:, :]], axis=0)
        return jnp.dot(_unpack(lhs), _unpack(w_ref[:, n * 128:(n + 1) * 128]),
                       preferred_element_type=F32)

    def add_tie(lag, x32):
        vregs = [x32[j * 8:(j + 1) * 8, c * 128:(c + 1) * 128]
                 for j in range(x32.shape[0] // 8) for c in range(x32.shape[1] // 128)]
        ties.append([lag, functools.reduce(lambda u, v: u | v, vregs) & zvec[...]])

    def pack_t(val):
        pt = _pack(val.T)
        add_tie(LAG_T, pt)
        return pt

    def local_vq(h_ref, off, i, lo=0, hi=2 * NT):
        for n in range(lo, hi):
            slot, t = divmod(n, NT)
            val = tile_dot(h_ref, wvq.at[slot], t)
            if slot == 1:
                qbuf[off // CM][t, 0:CM, :] = val
            else:
                vbuf[t, HALO + off:HALO + off + CM, :] = val
                if off == 0:
                    first = jnp.broadcast_to(val[0:1, :], (HALO, 128))
                    vbuf[t, 0:HALO, :] = jnp.where(i == 0, first, vbuf[t, 0:HALO, :])

    def local_attn(o_ref, off, i, paced):
        zero = zref[0]
        for g in range(CM // RG):
            base = HALO + off + g * RG
            qg = [qbuf[off // CM][t, pl.ds(pl.multiple_of(zero + g * RG, RG), RG), :] for t in range(NT)]
            logit = []
            for w in range(WIN):
                a = base - DIL * w
                part = qg[0] * kbuf[0, a:a + RG, :]
                for t in range(1, NT):
                    part = part + qg[t] * kbuf[t, a:a + RG, :]
                lg = _group_sum4(part, lane) * QSCALE
                if off == 0 and g == 0 and w > 0:
                    lg = jnp.where(rowi + i * BM >= DIL * w, lg, MASKED)
                logit.append(lg)
            m = functools.reduce(jnp.maximum, logit)
            p = [jnp.exp2(lg - m) for lg in logit]
            inv = 1.0 / functools.reduce(lambda u, v: u + v, p)
            if paced:
                add_tie(int(LAG_SM + g * STEP_SM), pltpu.bitcast(inv, U32))
            for t in range(NT):
                acc = p[0] * vbuf[t, base:base + RG, :]
                for w in range(1, WIN):
                    a = base - DIL * w
                    acc = acc + p[w] * vbuf[t, a:a + RG, :]
                o_ref[g * RG // 2:(g + 1) * RG // 2, t * 128:(t + 1) * 128] = _pack(acc * inv)

    def full_qkv(h_ref, r, secs, lo=0, hi=3 * NT):
        r2 = pl.multiple_of(r >> 1, CM // 2)
        for sec, t in [(sec, t) for sec in secs for t in range(NT)][lo:hi]:
            val = tile_dot(h_ref, wb, sec * NT + t)
            if sec == sec_q:
                qs[t * 64:(t + 1) * 64, pl.ds(r, CM)] = pack_t(val * QSCALE)
            elif sec == sec_k:
                ks[t, pl.ds(r2, CM // 2), :] = _pack(val)
            else:
                vt[t * 64:(t + 1) * 64, pl.ds(r, CM)] = pack_t(val)

    def normalize(pair, r, ch, paced):
        x = jnp.where(pair == 0, xio[pl.ds(r, CM), :].astype(F32), xres[pl.ds(r, CM), :])
        xres[pl.ds(r, CM), :] = x
        if paced:
            gate = pltpu.bitcast(pltpu.bitcast(kall[0, 0:8, :], U32) & zvec[...], F32)
            head = x[:, 0:128] + jnp.concatenate([gate] * (CM // 8), axis=0)
            x = jnp.concatenate([head, x[:, 128:]], axis=1)
            hs = []
            for j in range(CM // RG):
                hs.append(_pack(_layernorm(x[j * RG:(j + 1) * RG, :])))
                add_tie(int(LAG_LN + j * STEP_LN), hs[-1])
            h = jnp.concatenate(hs, axis=0)
        else:
            h = _pack(_layernorm(x))
        hb[ch] = h
        hall[pl.ds(pl.multiple_of(r >> 1, CM // 2), CM // 2), :] = h

    def key_phase(pair):
        @pl.when(pair == 0)
        def _():
            cp_x[0].wait()
            cp_x[2].start()

        normalize(pair, 0, 0, False)

        def body(j, c):
            @pl.when(pair == 0)
            def _():
                @pl.when(j == 0)
                def _():
                    cp_x[1].wait()
                    cp_waq.start()
                    cp_woa.start(priority=1)
                    cp_wb.start(priority=1)

                @pl.when(j == 1)
                def _():
                    cp_x[3].start()
                    cp_x[4].start()
                    cp_x[2].wait()
                    cp_wav.wait()

                @pl.when(j == 2)
                def _():
                    cp_wob.start(priority=1)
                    cp_x[3].wait()
                    cp_waq.wait()

                @pl.when(j == 3)
                def _():
                    cp_x[4].wait()

            r0 = pl.multiple_of(j * KB, KB)
            nsub = KB // CM
            rows = [pl.multiple_of(r0 + u * CM, CM) for u in range(nsub)]
            rows.append(pl.multiple_of(jnp.minimum(r0 + KB, S - CM), CM))

            sec = jnp.where(j == 0, sec_k, jnp.where(j == 1, sec_v, sec_q))
            c0 = pl.multiple_of(sec * D, D)
            for u in range(nsub):
                normalize(pair, rows[u + 1], (u + 1) % 2, True)
                for cc in range(u * nwc // nsub, (u + 1) * nwc // nsub):
                    w32 = _pack(wst[cc * pr:(cc + 1) * pr, pl.ds(c0, D)])
                    wvq[j >> 1, cc * pr // 2:(cc + 1) * pr // 2, :] = _permute_cols(w32)
                for t in range(NT):
                    kall[t, pl.ds(pl.multiple_of(HALO + rows[u], 8), CM), :] = tile_dot(
                        hb.at[u % 2], wak, t)
            assert not ties
            return c

        with jax.named_scope("key_phase"):
            lax.fori_loop(0, S // KB, body, 0)

        @pl.when(pair == 0)
        def _():
            cp_woa.wait()
            lax.fori_loop(0, NT, permo_body, 0)
            cp_wb.wait()
            repack(wst2, wb)

    def row_phase(pair):
        def body(i, c):
            @pl.when(jnp.logical_and(pair == 0, i == 1))
            def _():
                cp_wob.wait()
                repack(wost2, wob)

            r0 = pl.multiple_of(i * BM, BM)
            rs = [r0, pl.multiple_of(r0 + CM, CM)]
            hs = [hall.at[pl.ds(pl.multiple_of(r >> 1, CM // 2), CM // 2), :] for r in rs]

            def local_out(ch):
                y = jnp.concatenate([tile_dot(ob.at[ch], woa, n) for n in range(NT)], axis=1)
                x2 = xres[pl.ds(rs[ch], CM), :] + y
                xres[pl.ds(rs[ch], CM), :] = x2
                xsave[pl.ds(rs[ch], CM), :] = x2
                h2b[ch] = _pack(_layernorm(x2))

            for t in range(NT):
                vbuf[t, 0:HALO, :] = vbuf[t, BM:BM + HALO, :]
            local_vq(hs[0], 0, i, 0, 1)
            for t in range(NT):
                kt = kall[t, pl.ds(r0, HALO + BM), :]
                kbuf[t] = kt
                add_tie(LAG_K + t, pltpu.bitcast(kt, U32))
            local_vq(hs[0], 0, i, 1)
            local_vq(hs[1], CM, i, 0, SPLIT1)
            local_attn(ob.at[0], 0, i, False)
            local_out(0)
            local_vq(hs[1], CM, i, SPLIT1)
            local_attn(ob.at[1], CM, i, True)
            full_qkv(h2b.at[0], rs[0], (sec_k, sec_v, sec_q), 0, SPLIT2)
            local_out(1)
            full_qkv(h2b.at[0], rs[0], (sec_k, sec_v, sec_q), SPLIT2)
            full_qkv(h2b.at[1], rs[1], (sec_v, sec_q, sec_k))
            assert not ties
            return c

        with jax.named_scope("row_phase"):
            lax.fori_loop(0, nblk, body, 0)

    early = QB // OB

    def out_copy(i):
        r0 = pl.multiple_of(i * OB, OB)
        return pltpu.make_async_copy(xio.at[pl.ds(r0, OB), :], out_hbm.at[pl.ds(r0, OB), :],
                                     osems.at[i])

    def write_out(lo, hi):
        def body(i, c):
            r0 = pl.multiple_of(i * OB, OB)
            xio[pl.ds(r0, OB), :] = xres[pl.ds(r0, OB), :].astype(BF16)
            out_copy(i).start()
            return c

        lax.fori_loop(lo, hi, body, 0)

    def masked_q(q32, hp):
        head = lax.broadcasted_iota(jnp.int32, q32.shape, 0) >> (DH.bit_length() - 2)
        return _unpack(jnp.where(head == hp, q32, jnp.uint32(0)))

    def padded_qt(g, hp, q0, nq):
        hr = DH // 2
        qt = qs[pl.ds(pl.multiple_of(g * 64 + hp * hr, hr), hr), pl.ds(q0, nq)]
        parts = [jnp.zeros((hp * hr, nq), U32), qt, jnp.zeros(((HPT - 1 - hp) * hr, nq), U32)]
        return _unpack(jnp.concatenate([x for x in parts if x.shape[0]], axis=0))

    def add_oproj(ot, g, q0, nq):
        g64 = pl.multiple_of(g * 64, 64)
        for j in range(nq // OS):
            y = jnp.dot(ot[:, j * OS:(j + 1) * OS].T.astype(BF16), _unpack(wob[pl.ds(g64, 64), :]),
                        preferred_element_type=F32)
            r = pl.multiple_of(q0 + j * OS, OS)
            xres[pl.ds(r, OS), :] = xres[pl.ds(r, OS), :] + y

    def full_attn(pair):
        nqb = S // QB

        def body(it, bad):
            @pl.when(jnp.logical_and(pair == 1, it == NT))
            def _():
                write_out(0, early)

            g = it & (NT - 1)
            qh = it >> (NT.bit_length() - 1)
            q0 = pl.multiple_of(qh * QB, QB)
            zero = zref[0]
            acc = [None] * HPT
            l8 = [None] * HPT

            def pv(hp, t, buf):
                r0 = pl.multiple_of(g * 64 + hp * (DH // 2), DH // 2)
                vc = _unpack(vt[pl.ds(r0, DH // 2), t * KC:(t + 1) * KC])
                a = jnp.dot(vc, _unpack(buf[zero]), preferred_element_type=F32)
                acc[hp] = a if acc[hp] is None else acc[hp] + a

            pending = None
            for hp in range(HPT):
                w = padded_qt(g, hp, q0, QB)
                for t in range(S // KC):
                    kc = _unpack(ks[g, t * KC // 2:(t + 1) * KC // 2, :])
                    p = jnp.exp2(jnp.dot(kc, w, preferred_element_type=F32))
                    part = jnp.sum(p.reshape(KC // 8, 8, QB), axis=0)
                    l8[hp] = part if l8[hp] is None else l8[hp] + part
                    buf = pbufs[(hp * (S // KC) + t) % len(pbufs)]
                    buf[0] = _pack(p)
                    if pending is not None:
                        pv(*pending)
                    pending = (hp, t, buf)
            pv(*pending)
            outs = []
            for hp in range(HPT):
                l = jnp.sum(l8[hp], axis=0, keepdims=True)
                o = acc[hp] * (1.0 / l)
                outs.append(o)
                ok = (jnp.abs(o) < O_HI) & (l > L_LO) & (l < L_HI)
                nbad = jnp.where(ok, 0.0, 1.0)
                nbad = jnp.max(nbad.reshape(DH // 8, 8, QB), axis=0)
                for j in range(QB // 128):
                    bad = jnp.maximum(bad, nbad[:, j * 128:(j + 1) * 128])
            add_oproj(jnp.concatenate(outs, axis=0), g, q0, QB)
            return bad

        with jax.named_scope("full_attn"):
            bad = lax.fori_loop(0, NT * nqb, body, jnp.zeros((8, 128), F32))

        @pl.when(jnp.max(bad) > 0.0)
        def _():
            nq = S // FQ

            def restore(i, c):
                r = pl.multiple_of(i * 32, 32)
                xres[pl.ds(r, 32), :] = xsave[pl.ds(r, 32), :]
                return c

            lax.fori_loop(0, S // 32, restore, 0)

            def fb_body(it, c):
                g = it // nq
                q0 = pl.multiple_of((it % nq) * FQ, FQ)
                q32 = qs[pl.ds(pl.multiple_of(g * 64, 64), 64), pl.ds(q0, FQ)]

                def head_body(hp, c2):
                    r0 = pl.multiple_of(g * 64 + hp * (DH // 2), DH // 2)
                    s = jnp.dot(_unpack(ks[g]), masked_q(q32, hp), preferred_element_type=F32)
                    p = jnp.exp2(s - jnp.max(s, axis=0, keepdims=True))
                    l = jnp.sum(p, axis=0, keepdims=True)
                    acc = jnp.dot(_unpack(vt[pl.ds(r0, DH // 2), :]), p.astype(BF16),
                                  preferred_element_type=F32)
                    ots[pl.ds(pl.multiple_of(hp * DH, DH), DH), :] = acc * (1.0 / l)
                    return c2

                lax.fori_loop(0, HPT, head_body, 0)
                add_oproj(ots[...], g, q0, FQ)
                return c

            lax.fori_loop(0, NT * nq, fb_body, 0)

            @pl.when(pair == 1)
            def _():
                for i in range(early):
                    out_copy(i).wait()
                write_out(0, early)

    def pair_body(pair, c):
        key_phase(pair)
        row_phase(pair)
        full_attn(pair)
        return c

    with jax.named_scope("pairs"):
        lax.fori_loop(0, 2, pair_body, 0)

    with jax.named_scope("out_phase"):
        write_out(early, S // OB)
        for i in range(S // OB):
            out_copy(i).wait()


@jax.jit
def pallas_interleave_layers__sliding_local_dilated__softmax_full_mha__prompt_kernel(
    A_x: jax.Array,
    A_wqkv: jax.Array,
    A_wo: jax.Array,
    B_x: jax.Array,
    B_wqkv: jax.Array,
    B_wo: jax.Array,
):
    del B_x
    x = A_x.reshape(S, D)
    hbm = pl.BlockSpec(memory_space=pl.ANY)
    out = pl.pallas_call(
        _kernel,
        out_shape=jax.ShapeDtypeStruct((S, D), BF16),
        in_specs=[hbm] * 5,
        out_specs=hbm,
        scratch_shapes=[
            pltpu.VMEM((S, D), BF16),
            pltpu.VMEM((S, D), F32),
            pltpu.VMEM((S, D), F32),
            pltpu.VMEM((D, 3 * D), BF16),
            pltpu.VMEM((D, D), BF16),
            pltpu.VMEM((D, 3 * D), BF16),
            pltpu.VMEM((D, D), BF16),
            pltpu.VMEM((D // 2, D), U32),
            pltpu.VMEM((2, D // 2, D), U32),
            pltpu.VMEM((D // 2, D), U32),
            pltpu.VMEM((D // 2, 3 * D), U32),
            pltpu.VMEM((D // 2, D), U32),
            pltpu.VMEM((BM // CM, CM // 2, D), U32),
            pltpu.VMEM((S // 2, D), U32),
            pltpu.VMEM((BM // CM, CM // 2, D), U32),
            pltpu.VMEM((BM // CM, CM // 2, D), U32),
            pltpu.VMEM((NT, CM + 8, 128), F32),
            pltpu.VMEM((NT, CM + 8, 128), F32),
            pltpu.SMEM((1,), jnp.int32),
            pltpu.VMEM((8, 128), U32),
            pltpu.VMEM((NT, HALO + S, 128), F32),
            pltpu.VMEM((NT, HALO + BM, 128), F32),
            pltpu.VMEM((NT, HALO + BM, 128), F32),
            pltpu.VMEM((D // 2, S), U32),
            pltpu.VMEM((NT, S // 2, 128), U32),
            pltpu.VMEM((D // 2, S), U32),
            pltpu.VMEM((128, FQ), F32),
            pltpu.VMEM((1, KC // 2, QB), U32),
            pltpu.VMEM((1, KC // 2, QB), U32),
            pltpu.VMEM((1, KC // 2, QB), U32),
            pltpu.VMEM((1, KC // 2, QB), U32),
            pltpu.SemaphoreType.DMA((D // 128,)),
            pltpu.SemaphoreType.DMA((S // KB + 1,)),
            pltpu.SemaphoreType.DMA((5,)),
            pltpu.SemaphoreType.DMA((S // OB,)),
        ],
        compiler_params=pltpu.CompilerParams(vmem_limit_bytes=110 * 1024 * 1024),
        name="interleaved_attention_stack",
    )(x, A_wqkv, A_wo, B_wqkv, B_wo)
    return out.reshape(1, S, D)
```

```python
import functools
import math

import jax
import jax.numpy as jnp
from jax import lax
import jax.experimental.pallas as pl
import jax.experimental.pallas.tpu as pltpu

S = 2048
D = 1024
H = 32
DH = D // H
NT = D // 128
HPT = 128 // DH
WIN = 8
DIL = 2
HALO = 16
EPS = 1e-5
LOG2E = math.log2(math.e)
QSCALE = (DH ** -0.5) * LOG2E
MASKED = -1e9 * LOG2E

BM = 256
KB = 512
CM = 128
RG = 16
KC = 512
QB = 1024
OS = 128
FQ = 128

SPLIT1 = 12
SPLIT2 = 16
LAG_T = 6
LAG_K = 2
LAG_LN, STEP_LN = 4, 0.6
LAG_SM, STEP_SM = 6, 1

L_LO = 2.0 ** -40
L_HI = 2.0 ** 90
O_HI = 3.0e38

F32 = jnp.float32
BF16 = jnp.bfloat16
U32 = jnp.uint32


def _layernorm(x):
    mu = jnp.mean(x, axis=-1, keepdims=True)
    xc = x - mu
    var = jnp.mean(xc * xc, axis=-1, keepdims=True)
    return xc * lax.rsqrt(var + EPS)


def _permute_cols(w32):
    rows = w32.shape[0]
    lane = lax.broadcasted_iota(jnp.int32, (rows, 128), 1)
    tiles = [w32[:, t * 128:(t + 1) * 128] for t in range(NT)]
    for b in range(3):
        sh = 4 << b
        low = (lane & sh) == 0
        for a in range(NT):
            if a & (1 << b):
                continue
            c = a | (1 << b)
            ta, tc = tiles[a], tiles[c]
            tiles[a] = jnp.where(low, ta, pltpu.roll(tc, sh, 1))
            tiles[c] = jnp.where(low, pltpu.roll(ta, 128 - sh, 1), tc)
    return jnp.concatenate(tiles, axis=1)


def _permute_rows(w32):
    ncols = w32.shape[1]
    nv = D // 16
    v = [w32[i * 8:(i + 1) * 8, :] for i in range(nv)]
    sub = lax.broadcasted_iota(jnp.int32, (8, ncols), 0)
    for vb, sh in ((8, 2), (16, 4)):
        low = (sub & sh) == 0
        for a in range(nv):
            if a & vb:
                continue
            c = a | vb
            ta, tc = v[a], v[c]
            v[a] = jnp.where(low, ta, pltpu.roll(tc, sh, 0))
            v[c] = jnp.where(low, pltpu.roll(ta, 8 - sh, 0), tc)
    def src(i):
        b0, b5 = i & 1, (i >> 5) & 1
        return (i & ~33) | (b0 << 5) | b5
    return jnp.concatenate([v[src(i)] for i in range(nv)], axis=0)


def _group_sum4(x, lane):
    b0 = (lane & 1) == 0
    x = x + jnp.where(b0, pltpu.roll(x, 127, 1), pltpu.roll(x, 1, 1))
    b1 = (lane & 2) == 0
    return x + jnp.where(b1, pltpu.roll(x, 126, 1), pltpu.roll(x, 2, 1))


def _pack(x):
    return pltpu.bitcast(x.astype(BF16), U32)


def _unpack(x):
    return pltpu.bitcast(x, BF16)


def _kernel(x_hbm, wa_hbm, woa_hbm, wb_hbm, wob_hbm, out_hbm,
            xio, xres, xsave, wst, wost, wst2, wost2, wak, wvq, woa, wb, wob, hb, hall, h2b, ob,
            qbuf0, qbuf1, zref, zvec, kall, kbuf, vbuf, qs, ks, vt, ots, pb0, pb1, pb2, pb3,
            wsems, xsems, sems, osems):
    nblk = S // BM
    qbuf = (qbuf0, qbuf1)
    pbufs = (pb0, pb1, pb2, pb3)
    zref[0] = 0
    zvec[...] = jnp.zeros(zvec.shape, U32)
    pr = 128
    nwc = D // pr
    sec_q, sec_k, sec_v = 0, 1, 2

    def wak_copy(c):
        r = pl.multiple_of(c * pr, pr)
        return pltpu.make_async_copy(wa_hbm.at[pl.ds(r, pr), pl.ds(sec_k * D, D)],
                                     wst.at[pl.ds(r, pr), pl.ds(sec_k * D, D)], wsems.at[c])

    x_cuts = [0, CM] + [min(CM + (j + 1) * KB, S) for j in range(S // KB)]
    cp_x = [pltpu.make_async_copy(x_hbm.at[pl.ds(lo, hi - lo), :], xio.at[pl.ds(lo, hi - lo), :],
                                  xsems.at[k])
            for k, (lo, hi) in enumerate(zip(x_cuts[:-1], x_cuts[1:]))]

    def sec_copy(sec, k):
        return pltpu.make_async_copy(wa_hbm.at[:, pl.ds(sec * D, D)], wst.at[:, pl.ds(sec * D, D)],
                                     sems.at[k])

    cp_wav = sec_copy(sec_v, 0)
    cp_waq = sec_copy(sec_q, 1)
    cp_woa = pltpu.make_async_copy(woa_hbm, wost, sems.at[2])
    cp_wb = pltpu.make_async_copy(wb_hbm, wst2, sems.at[3])
    cp_wob = pltpu.make_async_copy(wob_hbm, wost2, sems.at[4])
    ahead = 3
    for c in range(ahead):
        wak_copy(c).start()

    for t in range(NT):
        kall[t, 0:HALO, :] = jnp.zeros((HALO, 128), F32)
        vbuf[t, BM:BM + HALO, :] = jnp.zeros((HALO, 128), F32)

    def perm_body(c, carry):
        wak_copy(c).wait()

        @pl.when(c + ahead < nwc)
        def _():
            wak_copy(jnp.minimum(c + ahead, nwc - 1)).start()

        for k, cp in enumerate((cp_x[0], cp_x[1], cp_wav)):
            @pl.when(c + ahead == nwc + k)
            def _(cp=cp):
                cp.start()

        r = pl.multiple_of(c * pr, pr)
        r2 = pl.multiple_of(c * (pr // 2), pr // 2)
        w32 = _pack(wst[pl.ds(r, pr), sec_k * D:(sec_k + 1) * D])
        wak[pl.ds(r2, pr // 2), :] = _permute_cols(w32)
        return carry

    with jax.named_scope("perm_cols"):
        lax.fori_loop(0, nwc, perm_body, 0)

    def repack(src, dst):
        step = 64

        def body(i, carry):
            r = pl.multiple_of(i * step, step)
            r2 = pl.multiple_of(i * (step // 2), step // 2)
            dst[pl.ds(r2, step // 2), :] = _pack(src[pl.ds(r, step), :])
            return carry

        lax.fori_loop(0, D // step, body, 0)

    def relayout_body(t, carry):
        c0 = pl.multiple_of(t * 128, 128)
        woa[:, pl.ds(c0, 128)] = _permute_rows(_pack(wost[:, pl.ds(c0, 128)]))
        wb[pl.ds(pl.multiple_of(t * 64, 64), 64), :] = _pack(wst2[pl.ds(c0, 128), :])
        return carry

    lane = lax.broadcasted_iota(jnp.int32, (RG, 128), 1)
    rowi = lax.broadcasted_iota(jnp.int32, (RG, 128), 0)

    ties = []

    def tile_dot(lhs_ref, w_ref, n):
        lhs = lhs_ref[...]
        for e in ties:
            e[0] -= 1
        due = [e[1] for e in ties if e[0] <= 0]
        ties[:] = [e for e in ties if e[0] > 0]
        if due:
            first = functools.reduce(lambda u, v: u | v, due, lhs[0:8, 0:128])
            top = jnp.concatenate([first, lhs[0:8, 128:]], axis=1)
            lhs = jnp.concatenate([top, lhs[8:, :]], axis=0)
        return jnp.dot(_unpack(lhs), _unpack(w_ref[:, n * 128:(n + 1) * 128]),
                       preferred_element_type=F32)

    def add_tie(lag, x32):
        vregs = [x32[j * 8:(j + 1) * 8, c * 128:(c + 1) * 128]
                 for j in range(x32.shape[0] // 8) for c in range(x32.shape[1] // 128)]
        ties.append([lag, functools.reduce(lambda u, v: u | v, vregs) & zvec[...]])

    def pack_t(val):
        pt = _pack(val.T)
        add_tie(LAG_T, pt)
        return pt

    def local_vq(h_ref, off, i, lo=0, hi=2 * NT):
        for n in range(lo, hi):
            slot, t = divmod(n, NT)
            val = tile_dot(h_ref, wvq.at[slot], t)
            if slot == 1:
                qbuf[off // CM][t, 0:CM, :] = val
            else:
                vbuf[t, HALO + off:HALO + off + CM, :] = val
                if off == 0:
                    first = jnp.broadcast_to(val[0:1, :], (HALO, 128))
                    vbuf[t, 0:HALO, :] = jnp.where(i == 0, first, vbuf[t, 0:HALO, :])

    def local_attn(o_ref, off, i, paced):
        zero = zref[0]
        for g in range(CM // RG):
            base = HALO + off + g * RG
            qg = [qbuf[off // CM][t, pl.ds(pl.multiple_of(zero + g * RG, RG), RG), :] for t in range(NT)]
            logit = []
            for w in range(WIN):
                a = base - DIL * w
                part = qg[0] * kbuf[0, a:a + RG, :]
                for t in range(1, NT):
                    part = part + qg[t] * kbuf[t, a:a + RG, :]
                lg = _group_sum4(part, lane) * QSCALE
                if off == 0 and g == 0 and w > 0:
                    lg = jnp.where(rowi + i * BM >= DIL * w, lg, MASKED)
                logit.append(lg)
            m = functools.reduce(jnp.maximum, logit)
            p = [jnp.exp2(lg - m) for lg in logit]
            inv = 1.0 / functools.reduce(lambda u, v: u + v, p)
            if paced:
                add_tie(int(LAG_SM + g * STEP_SM), pltpu.bitcast(inv, U32))
            for t in range(NT):
                acc = p[0] * vbuf[t, base:base + RG, :]
                for w in range(1, WIN):
                    a = base - DIL * w
                    acc = acc + p[w] * vbuf[t, a:a + RG, :]
                o_ref[g * RG // 2:(g + 1) * RG // 2, t * 128:(t + 1) * 128] = _pack(acc * inv)

    def full_qkv(h_ref, r, secs, lo=0, hi=3 * NT):
        r2 = pl.multiple_of(r >> 1, CM // 2)
        for sec, t in [(sec, t) for sec in secs for t in range(NT)][lo:hi]:
            val = tile_dot(h_ref, wb, sec * NT + t)
            if sec == sec_q:
                qs[t * 64:(t + 1) * 64, pl.ds(r, CM)] = pack_t(val * QSCALE)
            elif sec == sec_k:
                ks[t, pl.ds(r2, CM // 2), :] = _pack(val)
            else:
                vt[t * 64:(t + 1) * 64, pl.ds(r, CM)] = pack_t(val)

    def normalize(pair, r, ch, paced):
        x = jnp.where(pair == 0, xio[pl.ds(r, CM), :].astype(F32), xres[pl.ds(r, CM), :])
        xres[pl.ds(r, CM), :] = x
        if paced:
            gate = pltpu.bitcast(pltpu.bitcast(kall[0, 0:8, :], U32) & zvec[...], F32)
            head = x[:, 0:128] + jnp.concatenate([gate] * (CM // 8), axis=0)
            x = jnp.concatenate([head, x[:, 128:]], axis=1)
            hs = []
            for j in range(CM // RG):
                hs.append(_pack(_layernorm(x[j * RG:(j + 1) * RG, :])))
                add_tie(int(LAG_LN + j * STEP_LN), hs[-1])
            h = jnp.concatenate(hs, axis=0)
        else:
            h = _pack(_layernorm(x))
        hb[ch] = h
        hall[pl.ds(pl.multiple_of(r >> 1, CM // 2), CM // 2), :] = h

    def key_phase(pair):
        @pl.when(pair == 0)
        def _():
            cp_x[0].wait()
            cp_x[2].start()

        normalize(pair, 0, 0, False)

        def body(j, c):
            @pl.when(pair == 0)
            def _():
                @pl.when(j == 0)
                def _():
                    cp_x[1].wait()
                    cp_waq.start()
                    cp_woa.start(priority=1)
                    cp_wb.start(priority=1)

                @pl.when(j == 1)
                def _():
                    cp_x[3].start()
                    cp_x[4].start()
                    cp_x[2].wait()
                    cp_wav.wait()

                @pl.when(j == 2)
                def _():
                    cp_wob.start(priority=1)
                    cp_x[3].wait()
                    cp_waq.wait()

                @pl.when(j == 3)
                def _():
                    cp_x[4].wait()

            r0 = pl.multiple_of(j * KB, KB)
            nsub = KB // CM
            rows = [pl.multiple_of(r0 + u * CM, CM) for u in range(nsub)]
            rows.append(pl.multiple_of(jnp.minimum(r0 + KB, S - CM), CM))

            sec = jnp.where(j == 0, sec_k, jnp.where(j == 1, sec_v, sec_q))
            c0 = pl.multiple_of(sec * D, D)
            for u in range(nsub):
                normalize(pair, rows[u + 1], (u + 1) % 2, True)
                for cc in range(u * nwc // nsub, (u + 1) * nwc // nsub):
                    w32 = _pack(wst[cc * pr:(cc + 1) * pr, pl.ds(c0, D)])
                    wvq[j >> 1, cc * pr // 2:(cc + 1) * pr // 2, :] = _permute_cols(w32)
                for t in range(NT):
                    kall[t, pl.ds(pl.multiple_of(HALO + rows[u], 8), CM), :] = tile_dot(
                        hb.at[u % 2], wak, t)
            assert not ties
            return c

        with jax.named_scope("key_phase"):
            lax.fori_loop(0, S // KB, body, 0)

        @pl.when(pair == 0)
        def _():
            cp_woa.wait()
            cp_wb.wait()
            lax.fori_loop(0, NT, relayout_body, 0)

    def row_phase(pair):
        def body(i, c):
            @pl.when(jnp.logical_and(pair == 0, i == 1))
            def _():
                cp_wob.wait()
                repack(wost2, wob)

            r0 = pl.multiple_of(i * BM, BM)
            rs = [r0, pl.multiple_of(r0 + CM, CM)]
            hs = [hall.at[pl.ds(pl.multiple_of(r >> 1, CM // 2), CM // 2), :] for r in rs]

            def local_out(ch):
                y = jnp.concatenate([tile_dot(ob.at[ch], woa, n) for n in range(NT)], axis=1)
                x2 = xres[pl.ds(rs[ch], CM), :] + y
                xres[pl.ds(rs[ch], CM), :] = x2
                xsave[pl.ds(rs[ch], CM), :] = x2
                h2b[ch] = _pack(_layernorm(x2))

            for t in range(NT):
                vbuf[t, 0:HALO, :] = vbuf[t, BM:BM + HALO, :]
            local_vq(hs[0], 0, i, 0, 1)
            for t in range(NT):
                kt = kall[t, pl.ds(r0, HALO + BM), :]
                kbuf[t] = kt
                add_tie(LAG_K + t, pltpu.bitcast(kt, U32))
            local_vq(hs[0], 0, i, 1)
            local_vq(hs[1], CM, i, 0, SPLIT1)
            local_attn(ob.at[0], 0, i, False)
            local_out(0)
            local_vq(hs[1], CM, i, SPLIT1)
            local_attn(ob.at[1], CM, i, True)
            full_qkv(h2b.at[0], rs[0], (sec_k, sec_v, sec_q), 0, SPLIT2)
            local_out(1)
            full_qkv(h2b.at[0], rs[0], (sec_k, sec_v, sec_q), SPLIT2)
            full_qkv(h2b.at[1], rs[1], (sec_v, sec_q, sec_k))
            assert not ties
            return c

        with jax.named_scope("row_phase"):
            lax.fori_loop(0, nblk, body, 0)

    def out_copy(i):
        r0 = pl.multiple_of(i * OS, OS)
        return pltpu.make_async_copy(xio.at[pl.ds(r0, OS), :], out_hbm.at[pl.ds(r0, OS), :],
                                     osems.at[i])

    def write_out():
        def body(i, c):
            r0 = pl.multiple_of(i * OS, OS)
            xio[pl.ds(r0, OS), :] = xres[pl.ds(r0, OS), :].astype(BF16)
            out_copy(i).start()
            return c

        lax.fori_loop(0, S // OS, body, 0)

    def masked_q(q32, hp):
        head = lax.broadcasted_iota(jnp.int32, q32.shape, 0) >> (DH.bit_length() - 2)
        return _unpack(jnp.where(head == hp, q32, jnp.uint32(0)))

    def padded_qt(g, hp, q0, nq):
        hr = DH // 2
        qt = qs[pl.ds(pl.multiple_of(g * 64 + hp * hr, hr), hr), pl.ds(q0, nq)]
        parts = [jnp.zeros((hp * hr, nq), U32), qt, jnp.zeros(((HPT - 1 - hp) * hr, nq), U32)]
        return _unpack(jnp.concatenate([x for x in parts if x.shape[0]], axis=0))

    def add_oproj(ot, g, q0, nq, final=None):
        g64 = pl.multiple_of(g * 64, 64)
        for j in range(nq // OS):
            y = jnp.dot(ot[:, j * OS:(j + 1) * OS].T.astype(BF16), _unpack(wob[pl.ds(g64, 64), :]),
                        preferred_element_type=F32)
            r = pl.multiple_of(q0 + j * OS, OS)
            xn = xres[pl.ds(r, OS), :] + y
            xres[pl.ds(r, OS), :] = xn
            if final is not None:
                xio[pl.ds(r, OS), :] = xn.astype(BF16)

                @pl.when(final)
                def _():
                    out_copy((q0 >> (OS.bit_length() - 1)) + j).start()

    def full_attn(pair):
        nqb = S // QB

        def body(it, bad):
            g = it & (NT - 1)
            qh = it >> (NT.bit_length() - 1)
            q0 = pl.multiple_of(qh * QB, QB)
            zero = zref[0]
            acc = [None] * HPT
            l8 = [None] * HPT

            def pv(hp, t, buf):
                r0 = pl.multiple_of(g * 64 + hp * (DH // 2), DH // 2)
                vc = _unpack(vt[pl.ds(r0, DH // 2), t * KC:(t + 1) * KC])
                a = jnp.dot(vc, _unpack(buf[zero]), preferred_element_type=F32)
                acc[hp] = a if acc[hp] is None else acc[hp] + a

            pending = None
            for hp in range(HPT):
                w = padded_qt(g, hp, q0, QB)
                for t in range(S // KC):
                    kc = _unpack(ks[g, t * KC // 2:(t + 1) * KC // 2, :])
                    p = jnp.exp2(jnp.dot(kc, w, preferred_element_type=F32))
                    part = jnp.sum(p.reshape(KC // 8, 8, QB), axis=0)
                    l8[hp] = part if l8[hp] is None else l8[hp] + part
                    buf = pbufs[(hp * (S // KC) + t) % len(pbufs)]
                    buf[0] = _pack(p)
                    if pending is not None:
                        pv(*pending)
                    pending = (hp, t, buf)
            pv(*pending)
            outs = []
            for hp in range(HPT):
                l = jnp.sum(l8[hp], axis=0, keepdims=True)
                o = acc[hp] * (1.0 / l)
                outs.append(o)
                ok = (jnp.abs(o) < O_HI) & (l > L_LO) & (l < L_HI)
                nbad = jnp.where(ok, 0.0, 1.0)
                nbad = jnp.max(nbad.reshape(DH // 8, 8, QB), axis=0)
                for j in range(QB // 128):
                    bad = jnp.maximum(bad, nbad[:, j * 128:(j + 1) * 128])
            add_oproj(jnp.concatenate(outs, axis=0), g, q0, QB,
                      jnp.logical_and(pair == 1, g == NT - 1))
            return bad

        with jax.named_scope("full_attn"):
            bad = lax.fori_loop(0, NT * nqb, body, jnp.zeros((8, 128), F32))

        @pl.when(jnp.max(bad) > 0.0)
        def _():
            nq = S // FQ

            def restore(i, c):
                r = pl.multiple_of(i * 32, 32)
                xres[pl.ds(r, 32), :] = xsave[pl.ds(r, 32), :]
                return c

            lax.fori_loop(0, S // 32, restore, 0)

            def fb_body(it, c):
                g = it // nq
                q0 = pl.multiple_of((it % nq) * FQ, FQ)
                q32 = qs[pl.ds(pl.multiple_of(g * 64, 64), 64), pl.ds(q0, FQ)]

                def head_body(hp, c2):
                    r0 = pl.multiple_of(g * 64 + hp * (DH // 2), DH // 2)
                    s = jnp.dot(_unpack(ks[g]), masked_q(q32, hp), preferred_element_type=F32)
                    p = jnp.exp2(s - jnp.max(s, axis=0, keepdims=True))
                    l = jnp.sum(p, axis=0, keepdims=True)
                    acc = jnp.dot(_unpack(vt[pl.ds(r0, DH // 2), :]), p.astype(BF16),
                                  preferred_element_type=F32)
                    ots[pl.ds(pl.multiple_of(hp * DH, DH), DH), :] = acc * (1.0 / l)
                    return c2

                lax.fori_loop(0, HPT, head_body, 0)
                add_oproj(ots[...], g, q0, FQ)
                return c

            lax.fori_loop(0, NT * nq, fb_body, 0)

            @pl.when(pair == 1)
            def _():
                for i in range(S // OS):
                    out_copy(i).wait()
                write_out()

    def pair_body(pair, c):
        key_phase(pair)
        row_phase(pair)
        full_attn(pair)
        return c

    with jax.named_scope("pairs"):
        lax.fori_loop(0, 2, pair_body, 0)

    with jax.named_scope("out_phase"):
        for i in range(S // OS):
            out_copy(i).wait()


@jax.jit
def pallas_interleave_layers__sliding_local_dilated__softmax_full_mha__prompt_kernel(
    A_x: jax.Array,
    A_wqkv: jax.Array,
    A_wo: jax.Array,
    B_x: jax.Array,
    B_wqkv: jax.Array,
    B_wo: jax.Array,
):
    del B_x
    x = A_x.reshape(S, D)
    hbm = pl.BlockSpec(memory_space=pl.ANY)
    out = pl.pallas_call(
        _kernel,
        out_shape=jax.ShapeDtypeStruct((S, D), BF16),
        in_specs=[hbm] * 5,
        out_specs=hbm,
        scratch_shapes=[
            pltpu.VMEM((S, D), BF16),
            pltpu.VMEM((S, D), F32),
            pltpu.VMEM((S, D), F32),
            pltpu.VMEM((D, 3 * D), BF16),
            pltpu.VMEM((D, D), BF16),
            pltpu.VMEM((D, 3 * D), BF16),
            pltpu.VMEM((D, D), BF16),
            pltpu.VMEM((D // 2, D), U32),
            pltpu.VMEM((2, D // 2, D), U32),
            pltpu.VMEM((D // 2, D), U32),
            pltpu.VMEM((D // 2, 3 * D), U32),
            pltpu.VMEM((D // 2, D), U32),
            pltpu.VMEM((BM // CM, CM // 2, D), U32),
            pltpu.VMEM((S // 2, D), U32),
            pltpu.VMEM((BM // CM, CM // 2, D), U32),
            pltpu.VMEM((BM // CM, CM // 2, D), U32),
            pltpu.VMEM((NT, CM + 8, 128), F32),
            pltpu.VMEM((NT, CM + 8, 128), F32),
            pltpu.SMEM((1,), jnp.int32),
            pltpu.VMEM((8, 128), U32),
            pltpu.VMEM((NT, HALO + S, 128), F32),
            pltpu.VMEM((NT, HALO + BM, 128), F32),
            pltpu.VMEM((NT, HALO + BM, 128), F32),
            pltpu.VMEM((D // 2, S), U32),
            pltpu.VMEM((NT, S // 2, 128), U32),
            pltpu.VMEM((D // 2, S), U32),
            pltpu.VMEM((128, FQ), F32),
            pltpu.VMEM((1, KC // 2, QB), U32),
            pltpu.VMEM((1, KC // 2, QB), U32),
            pltpu.VMEM((1, KC // 2, QB), U32),
            pltpu.VMEM((1, KC // 2, QB), U32),
            pltpu.SemaphoreType.DMA((D // 128,)),
            pltpu.SemaphoreType.DMA((S // KB + 1,)),
            pltpu.SemaphoreType.DMA((5,)),
            pltpu.SemaphoreType.DMA((S // OS,)),
        ],
        compiler_params=pltpu.CompilerParams(vmem_limit_bytes=110 * 1024 * 1024,
                                             disable_bounds_checks=True),
        name="interleaved_attention_stack",
    )(x, A_wqkv, A_wo, B_wqkv, B_wo)
    return out.reshape(1, S, D)
```

```python
import functools
import math

import jax
import jax.numpy as jnp
from jax import lax
import jax.experimental.pallas as pl
import jax.experimental.pallas.tpu as pltpu

S = 2048
D = 1024
H = 32
DH = D // H
NT = D // 128
HPT = 128 // DH
WIN = 8
DIL = 2
HALO = 16
EPS = 1e-5
LOG2E = math.log2(math.e)
QSCALE = (DH ** -0.5) * LOG2E
MASKED = -1e9 * LOG2E

BM = 256
KB = 512
CM = 128
RG = 16
KC = 512
QB = 1024
OS = 128
FQ = 128

SPLIT1 = 12
SPLIT2 = 16
LAG_T = 6
LAG_K = 2
LAG_LN, STEP_LN = 4, 0.6
LAG_SM, STEP_SM = 6, 1

L_LO = 2.0 ** -40
L_HI = 2.0 ** 90
O_HI = 3.0e38

F32 = jnp.float32
BF16 = jnp.bfloat16
U32 = jnp.uint32


def _layernorm(x):
    mu = jnp.mean(x, axis=-1, keepdims=True)
    xc = x - mu
    var = jnp.mean(xc * xc, axis=-1, keepdims=True)
    return xc * lax.rsqrt(var + EPS)


def _permute_cols(w32):
    rows = w32.shape[0]
    lane = lax.broadcasted_iota(jnp.int32, (rows, 128), 1)
    tiles = [w32[:, t * 128:(t + 1) * 128] for t in range(NT)]
    for b in range(3):
        sh = 4 << b
        low = (lane & sh) == 0
        for a in range(NT):
            if a & (1 << b):
                continue
            c = a | (1 << b)
            ta, tc = tiles[a], tiles[c]
            tiles[a] = jnp.where(low, ta, pltpu.roll(tc, sh, 1))
            tiles[c] = jnp.where(low, pltpu.roll(ta, 128 - sh, 1), tc)
    return jnp.concatenate(tiles, axis=1)


def _permute_rows(w32):
    ncols = w32.shape[1]
    nv = D // 16
    v = [w32[i * 8:(i + 1) * 8, :] for i in range(nv)]
    sub = lax.broadcasted_iota(jnp.int32, (8, ncols), 0)
    for vb, sh in ((8, 2), (16, 4)):
        low = (sub & sh) == 0
        for a in range(nv):
            if a & vb:
                continue
            c = a | vb
            ta, tc = v[a], v[c]
            v[a] = jnp.where(low, ta, pltpu.roll(tc, sh, 0))
            v[c] = jnp.where(low, pltpu.roll(ta, 8 - sh, 0), tc)
    def src(i):
        b0, b5 = i & 1, (i >> 5) & 1
        return (i & ~33) | (b0 << 5) | b5
    return jnp.concatenate([v[src(i)] for i in range(nv)], axis=0)


def _group_sum4(x, lane):
    b0 = (lane & 1) == 0
    x = x + jnp.where(b0, pltpu.roll(x, 127, 1), pltpu.roll(x, 1, 1))
    b1 = (lane & 2) == 0
    return x + jnp.where(b1, pltpu.roll(x, 126, 1), pltpu.roll(x, 2, 1))


def _pack(x):
    return pltpu.bitcast(x.astype(BF16), U32)


def _unpack(x):
    return pltpu.bitcast(x, BF16)


def _kernel(x_hbm, wa_hbm, woa_hbm, wb_hbm, wob_hbm, out_hbm,
            xio, xres, xsave, wst, wost, wb, wob, wak, wvq, woa, hb, hall, h2b, ob,
            qbuf0, qbuf1, zref, zvec, kall, kbuf, vbuf, qs, ks, vt, ots, pb0, pb1, pb2, pb3,
            wsems, xsems, sems, osems):
    nblk = S // BM
    qbuf = (qbuf0, qbuf1)
    pbufs = (pb0, pb1, pb2, pb3)
    zref[0] = 0
    zvec[...] = jnp.zeros(zvec.shape, U32)
    pr = 128
    nwc = D // pr
    sec_q, sec_k, sec_v = 0, 1, 2

    def wak_copy(c):
        r = pl.multiple_of(c * pr, pr)
        return pltpu.make_async_copy(wa_hbm.at[pl.ds(r, pr), pl.ds(sec_k * D, D)],
                                     wst.at[pl.ds(r, pr), pl.ds(sec_k * D, D)], wsems.at[c])

    x_cuts = [0, CM] + [min(CM + (j + 1) * KB, S) for j in range(S // KB)]
    cp_x = [pltpu.make_async_copy(x_hbm.at[pl.ds(lo, hi - lo), :], xio.at[pl.ds(lo, hi - lo), :],
                                  xsems.at[k])
            for k, (lo, hi) in enumerate(zip(x_cuts[:-1], x_cuts[1:]))]

    def sec_copy(sec, k):
        return pltpu.make_async_copy(wa_hbm.at[:, pl.ds(sec * D, D)], wst.at[:, pl.ds(sec * D, D)],
                                     sems.at[k])

    cp_wav = sec_copy(sec_v, 0)
    cp_waq = sec_copy(sec_q, 1)
    cp_woa = pltpu.make_async_copy(woa_hbm, wost, sems.at[2])
    cp_wb = pltpu.make_async_copy(wb_hbm, wb, sems.at[3])
    cp_wob = pltpu.make_async_copy(wob_hbm, wob, sems.at[4])
    ahead = 5
    for c in range(ahead):
        wak_copy(c).start()

    for t in range(NT):
        kall[t, 0:HALO, :] = jnp.zeros((HALO, 128), F32)
        vbuf[t, BM:BM + HALO, :] = jnp.zeros((HALO, 128), F32)

    def perm_body(c, carry):
        wak_copy(c).wait()

        @pl.when(c + ahead < nwc)
        def _():
            wak_copy(jnp.minimum(c + ahead, nwc - 1)).start()

        for k, cp in enumerate((cp_x[0], cp_x[1], cp_wav)):
            @pl.when(c + ahead == nwc + k)
            def _(cp=cp):
                cp.start()

        r = pl.multiple_of(c * pr, pr)
        r2 = pl.multiple_of(c * (pr // 2), pr // 2)
        w32 = _pack(wst[pl.ds(r, pr), sec_k * D:(sec_k + 1) * D])
        wak[pl.ds(r2, pr // 2), :] = _permute_cols(w32)
        return carry

    with jax.named_scope("perm_cols"):
        lax.fori_loop(0, nwc, perm_body, 0)

    def permo_body(t, carry):
        c0 = pl.multiple_of(t * 128, 128)
        woa[:, pl.ds(c0, 128)] = _permute_rows(_pack(wost[:, pl.ds(c0, 128)]))
        return carry

    lane = lax.broadcasted_iota(jnp.int32, (RG, 128), 1)
    rowi = lax.broadcasted_iota(jnp.int32, (RG, 128), 0)

    ties = []

    def tile_dot(lhs_ref, w_ref, n):
        lhs = lhs_ref[...]
        for e in ties:
            e[0] -= 1
        due = [e[1] for e in ties if e[0] <= 0]
        ties[:] = [e for e in ties if e[0] > 0]
        if due:
            first = functools.reduce(lambda u, v: u | v, due, lhs[0:8, 0:128])
            top = jnp.concatenate([first, lhs[0:8, 128:]], axis=1)
            lhs = jnp.concatenate([top, lhs[8:, :]], axis=0)
        w = w_ref[:, n * 128:(n + 1) * 128]
        return jnp.dot(_unpack(lhs), w if w.dtype == BF16 else _unpack(w),
                       preferred_element_type=F32)

    def add_tie(lag, x32):
        vregs = [x32[j * 8:(j + 1) * 8, c * 128:(c + 1) * 128]
                 for j in range(x32.shape[0] // 8) for c in range(x32.shape[1] // 128)]
        ties.append([lag, functools.reduce(lambda u, v: u | v, vregs) & zvec[...]])

    def pack_t(val):
        pt = _pack(val.T)
        add_tie(LAG_T, pt)
        return pt

    def local_vq(h_ref, off, i, lo=0, hi=2 * NT):
        for n in range(lo, hi):
            slot, t = divmod(n, NT)
            val = tile_dot(h_ref, wvq.at[slot], t)
            if slot == 1:
                qbuf[off // CM][t, 0:CM, :] = val
            else:
                vbuf[t, HALO + off:HALO + off + CM, :] = val
                if off == 0:
                    first = jnp.broadcast_to(val[0:1, :], (HALO, 128))
                    vbuf[t, 0:HALO, :] = jnp.where(i == 0, first, vbuf[t, 0:HALO, :])

    def local_attn(o_ref, off, i, paced):
        zero = zref[0]
        for g in range(CM // RG):
            base = HALO + off + g * RG
            qg = [qbuf[off // CM][t, pl.ds(pl.multiple_of(zero + g * RG, RG), RG), :] for t in range(NT)]
            logit = []
            for w in range(WIN):
                a = base - DIL * w
                part = qg[0] * kbuf[0, a:a + RG, :]
                for t in range(1, NT):
                    part = part + qg[t] * kbuf[t, a:a + RG, :]
                lg = _group_sum4(part, lane) * QSCALE
                if off == 0 and g == 0 and w > 0:
                    lg = jnp.where(rowi + i * BM >= DIL * w, lg, MASKED)
                logit.append(lg)
            m = functools.reduce(jnp.maximum, logit)
            p = [jnp.exp2(lg - m) for lg in logit]
            inv = 1.0 / functools.reduce(lambda u, v: u + v, p)
            if paced:
                add_tie(int(LAG_SM + g * STEP_SM), pltpu.bitcast(inv, U32))
            for t in range(NT):
                acc = p[0] * vbuf[t, base:base + RG, :]
                for w in range(1, WIN):
                    a = base - DIL * w
                    acc = acc + p[w] * vbuf[t, a:a + RG, :]
                o_ref[g * RG // 2:(g + 1) * RG // 2, t * 128:(t + 1) * 128] = _pack(acc * inv)

    def full_qkv(h_ref, r, secs, lo=0, hi=3 * NT):
        r2 = pl.multiple_of(r >> 1, CM // 2)
        for sec, t in [(sec, t) for sec in secs for t in range(NT)][lo:hi]:
            val = tile_dot(h_ref, wb, sec * NT + t)
            if sec == sec_q:
                qs[t * 64:(t + 1) * 64, pl.ds(r, CM)] = pack_t(val * QSCALE)
            elif sec == sec_k:
                ks[t, pl.ds(r2, CM // 2), :] = _pack(val)
            else:
                vt[t * 64:(t + 1) * 64, pl.ds(r, CM)] = pack_t(val)

    def normalize(pair, r, ch, paced):
        x = jnp.where(pair == 0, xio[pl.ds(r, CM), :].astype(F32), xres[pl.ds(r, CM), :])
        xres[pl.ds(r, CM), :] = x
        if paced:
            gate = pltpu.bitcast(pltpu.bitcast(kall[0, 0:8, :], U32) & zvec[...], F32)
            head = x[:, 0:128] + jnp.concatenate([gate] * (CM // 8), axis=0)
            x = jnp.concatenate([head, x[:, 128:]], axis=1)
            hs = []
            for j in range(CM // RG):
                hs.append(_pack(_layernorm(x[j * RG:(j + 1) * RG, :])))
                add_tie(int(LAG_LN + j * STEP_LN), hs[-1])
            h = jnp.concatenate(hs, axis=0)
        else:
            h = _pack(_layernorm(x))
        hb[ch] = h
        hall[pl.ds(pl.multiple_of(r >> 1, CM // 2), CM // 2), :] = h

    def key_phase(pair):
        @pl.when(pair == 0)
        def _():
            cp_x[0].wait()
            cp_x[2].start()

        normalize(pair, 0, 0, False)

        def body(j, c):
            @pl.when(pair == 0)
            def _():
                @pl.when(j == 0)
                def _():
                    cp_x[1].wait()
                    cp_waq.start()
                    cp_woa.start(priority=1)
                    cp_wb.start(priority=1)

                @pl.when(j == 1)
                def _():
                    cp_x[3].start()
                    cp_x[4].start()
                    cp_x[2].wait()
                    cp_wav.wait()

                @pl.when(j == 2)
                def _():
                    cp_wob.start(priority=1)
                    cp_x[3].wait()
                    cp_waq.wait()

                @pl.when(j == 3)
                def _():
                    cp_x[4].wait()

            r0 = pl.multiple_of(j * KB, KB)
            nsub = KB // CM
            rows = [pl.multiple_of(r0 + u * CM, CM) for u in range(nsub)]
            rows.append(pl.multiple_of(jnp.minimum(r0 + KB, S - CM), CM))

            sec = jnp.where(j == 0, sec_k, jnp.where(j == 1, sec_v, sec_q))
            c0 = pl.multiple_of(sec * D, D)
            for u in range(nsub):
                normalize(pair, rows[u + 1], (u + 1) % 2, True)
                for cc in range(u * nwc // nsub, (u + 1) * nwc // nsub):
                    w32 = _pack(wst[cc * pr:(cc + 1) * pr, pl.ds(c0, D)])
                    wvq[j >> 1, cc * pr // 2:(cc + 1) * pr // 2, :] = _permute_cols(w32)
                for t in range(NT):
                    kall[t, pl.ds(pl.multiple_of(HALO + rows[u], 8), CM), :] = tile_dot(
                        hb.at[u % 2], wak, t)
            assert not ties
            return c

        with jax.named_scope("key_phase"):
            lax.fori_loop(0, S // KB, body, 0)

        @pl.when(pair == 0)
        def _():
            cp_woa.wait()
            lax.fori_loop(0, NT, permo_body, 0)
            cp_wb.wait()

    def row_phase(pair):
        def body(i, c):
            r0 = pl.multiple_of(i * BM, BM)
            rs = [r0, pl.multiple_of(r0 + CM, CM)]
            hs = [hall.at[pl.ds(pl.multiple_of(r >> 1, CM // 2), CM // 2), :] for r in rs]

            def local_out(ch):
                y = jnp.concatenate([tile_dot(ob.at[ch], woa, n) for n in range(NT)], axis=1)
                x2 = xres[pl.ds(rs[ch], CM), :] + y
                xres[pl.ds(rs[ch], CM), :] = x2
                xsave[pl.ds(rs[ch], CM), :] = x2
                h2b[ch] = _pack(_layernorm(x2))

            for t in range(NT):
                vbuf[t, 0:HALO, :] = vbuf[t, BM:BM + HALO, :]
            local_vq(hs[0], 0, i, 0, 1)
            for t in range(NT):
                kt = kall[t, pl.ds(r0, HALO + BM), :]
                kbuf[t] = kt
                add_tie(LAG_K + t, pltpu.bitcast(kt, U32))
            local_vq(hs[0], 0, i, 1)
            local_vq(hs[1], CM, i, 0, SPLIT1)
            local_attn(ob.at[0], 0, i, False)
            local_out(0)
            local_vq(hs[1], CM, i, SPLIT1)
            local_attn(ob.at[1], CM, i, True)
            full_qkv(h2b.at[0], rs[0], (sec_k, sec_v, sec_q), 0, SPLIT2)
            local_out(1)
            full_qkv(h2b.at[0], rs[0], (sec_k, sec_v, sec_q), SPLIT2)
            full_qkv(h2b.at[1], rs[1], (sec_v, sec_q, sec_k))
            assert not ties
            return c

        with jax.named_scope("row_phase"):
            lax.fori_loop(0, nblk, body, 0)

    def out_copy(i):
        r0 = pl.multiple_of(i * OS, OS)
        return pltpu.make_async_copy(xio.at[pl.ds(r0, OS), :], out_hbm.at[pl.ds(r0, OS), :],
                                     osems.at[i])

    def write_out():
        def body(i, c):
            r0 = pl.multiple_of(i * OS, OS)
            xio[pl.ds(r0, OS), :] = xres[pl.ds(r0, OS), :].astype(BF16)
            out_copy(i).start()
            return c

        lax.fori_loop(0, S // OS, body, 0)

    def masked_q(q32, hp):
        head = lax.broadcasted_iota(jnp.int32, q32.shape, 0) >> (DH.bit_length() - 2)
        return _unpack(jnp.where(head == hp, q32, jnp.uint32(0)))

    def padded_qt(g, hp, q0, nq):
        hr = DH // 2
        qt = qs[pl.ds(pl.multiple_of(g * 64 + hp * hr, hr), hr), pl.ds(q0, nq)]
        parts = [jnp.zeros((hp * hr, nq), U32), qt, jnp.zeros(((HPT - 1 - hp) * hr, nq), U32)]
        return _unpack(jnp.concatenate([x for x in parts if x.shape[0]], axis=0))

    def add_oproj(ot, g, q0, nq, final=None):
        g128 = pl.multiple_of(g * 128, 128)
        for j in range(nq // OS):
            y = jnp.dot(ot[:, j * OS:(j + 1) * OS].T.astype(BF16), wob[pl.ds(g128, 128), :],
                        preferred_element_type=F32)
            r = pl.multiple_of(q0 + j * OS, OS)
            xn = xres[pl.ds(r, OS), :] + y
            xres[pl.ds(r, OS), :] = xn
            if final is not None:
                xio[pl.ds(r, OS), :] = xn.astype(BF16)

                @pl.when(final)
                def _():
                    out_copy((q0 >> (OS.bit_length() - 1)) + j).start()

    def full_attn(pair):
        nqb = S // QB

        @pl.when(pair == 0)
        def _():
            cp_wob.wait()

        def body(it, bad):
            g = it & (NT - 1)
            qh = it >> (NT.bit_length() - 1)
            q0 = pl.multiple_of(qh * QB, QB)
            zero = zref[0]
            acc = [None] * HPT
            l8 = [None] * HPT

            def pv(hp, t, buf):
                r0 = pl.multiple_of(g * 64 + hp * (DH // 2), DH // 2)
                vc = _unpack(vt[pl.ds(r0, DH // 2), t * KC:(t + 1) * KC])
                a = jnp.dot(vc, _unpack(buf[zero]), preferred_element_type=F32)
                acc[hp] = a if acc[hp] is None else acc[hp] + a

            pending = None
            for hp in range(HPT):
                w = padded_qt(g, hp, q0, QB)
                for t in range(S // KC):
                    kc = _unpack(ks[g, t * KC // 2:(t + 1) * KC // 2, :])
                    p = jnp.exp2(jnp.dot(kc, w, preferred_element_type=F32))
                    part = jnp.sum(p.reshape(KC // 8, 8, QB), axis=0)
                    l8[hp] = part if l8[hp] is None else l8[hp] + part
                    buf = pbufs[(hp * (S // KC) + t) % len(pbufs)]
                    buf[0] = _pack(p)
                    if pending is not None:
                        pv(*pending)
                    pending = (hp, t, buf)
            pv(*pending)
            outs = []
            for hp in range(HPT):
                l = jnp.sum(l8[hp], axis=0, keepdims=True)
                o = acc[hp] * (1.0 / l)
                outs.append(o)
                ok = (jnp.abs(o) < O_HI) & (l > L_LO) & (l < L_HI)
                nbad = jnp.where(ok, 0.0, 1.0)
                nbad = jnp.max(nbad.reshape(DH // 8, 8, QB), axis=0)
                for j in range(QB // 128):
                    bad = jnp.maximum(bad, nbad[:, j * 128:(j + 1) * 128])
            add_oproj(jnp.concatenate(outs, axis=0), g, q0, QB,
                      jnp.logical_and(pair == 1, g == NT - 1))
            return bad

        with jax.named_scope("full_attn"):
            bad = lax.fori_loop(0, NT * nqb, body, jnp.zeros((8, 128), F32))

        @pl.when(jnp.max(bad) > 0.0)
        def _():
            nq = S // FQ

            def restore(i, c):
                r = pl.multiple_of(i * 32, 32)
                xres[pl.ds(r, 32), :] = xsave[pl.ds(r, 32), :]
                return c

            lax.fori_loop(0, S // 32, restore, 0)

            def fb_body(it, c):
                g = it // nq
                q0 = pl.multiple_of((it % nq) * FQ, FQ)
                q32 = qs[pl.ds(pl.multiple_of(g * 64, 64), 64), pl.ds(q0, FQ)]

                def head_body(hp, c2):
                    r0 = pl.multiple_of(g * 64 + hp * (DH // 2), DH // 2)
                    s = jnp.dot(_unpack(ks[g]), masked_q(q32, hp), preferred_element_type=F32)
                    p = jnp.exp2(s - jnp.max(s, axis=0, keepdims=True))
                    l = jnp.sum(p, axis=0, keepdims=True)
                    acc = jnp.dot(_unpack(vt[pl.ds(r0, DH // 2), :]), p.astype(BF16),
                                  preferred_element_type=F32)
                    ots[pl.ds(pl.multiple_of(hp * DH, DH), DH), :] = acc * (1.0 / l)
                    return c2

                lax.fori_loop(0, HPT, head_body, 0)
                add_oproj(ots[...], g, q0, FQ)
                return c

            lax.fori_loop(0, NT * nq, fb_body, 0)

            @pl.when(pair == 1)
            def _():
                for i in range(S // OS):
                    out_copy(i).wait()
                write_out()

    def pair_body(pair, c):
        key_phase(pair)
        row_phase(pair)
        full_attn(pair)
        return c

    with jax.named_scope("pairs"):
        lax.fori_loop(0, 2, pair_body, 0)

    with jax.named_scope("out_phase"):
        for i in range(S // OS):
            out_copy(i).wait()


@jax.jit
def pallas_interleave_layers__sliding_local_dilated__softmax_full_mha__prompt_kernel(
    A_x: jax.Array,
    A_wqkv: jax.Array,
    A_wo: jax.Array,
    B_x: jax.Array,
    B_wqkv: jax.Array,
    B_wo: jax.Array,
):
    del B_x
    x = A_x.reshape(S, D)
    hbm = pl.BlockSpec(memory_space=pl.ANY)
    out = pl.pallas_call(
        _kernel,
        out_shape=jax.ShapeDtypeStruct((S, D), BF16),
        in_specs=[hbm] * 5,
        out_specs=hbm,
        scratch_shapes=[
            pltpu.VMEM((S, D), BF16),
            pltpu.VMEM((S, D), F32),
            pltpu.VMEM((S, D), F32),
            pltpu.VMEM((D, 3 * D), BF16),
            pltpu.VMEM((D, D), BF16),
            pltpu.VMEM((D, 3 * D), BF16),
            pltpu.VMEM((D, D), BF16),
            pltpu.VMEM((D // 2, D), U32),
            pltpu.VMEM((2, D // 2, D), U32),
            pltpu.VMEM((D // 2, D), U32),
            pltpu.VMEM((BM // CM, CM // 2, D), U32),
            pltpu.VMEM((S // 2, D), U32),
            pltpu.VMEM((BM // CM, CM // 2, D), U32),
            pltpu.VMEM((BM // CM, CM // 2, D), U32),
            pltpu.VMEM((NT, CM + 8, 128), F32),
            pltpu.VMEM((NT, CM + 8, 128), F32),
            pltpu.SMEM((1,), jnp.int32),
            pltpu.VMEM((8, 128), U32),
            pltpu.VMEM((NT, HALO + S, 128), F32),
            pltpu.VMEM((NT, HALO + BM, 128), F32),
            pltpu.VMEM((NT, HALO + BM, 128), F32),
            pltpu.VMEM((D // 2, S), U32),
            pltpu.VMEM((NT, S // 2, 128), U32),
            pltpu.VMEM((D // 2, S), U32),
            pltpu.VMEM((128, FQ), F32),
            pltpu.VMEM((1, KC // 2, QB), U32),
            pltpu.VMEM((1, KC // 2, QB), U32),
            pltpu.VMEM((1, KC // 2, QB), U32),
            pltpu.VMEM((1, KC // 2, QB), U32),
            pltpu.SemaphoreType.DMA((D // 128,)),
            pltpu.SemaphoreType.DMA((S // KB + 1,)),
            pltpu.SemaphoreType.DMA((5,)),
            pltpu.SemaphoreType.DMA((S // OS,)),
        ],
        compiler_params=pltpu.CompilerParams(vmem_limit_bytes=110 * 1024 * 1024,
                                             disable_bounds_checks=True),
        name="interleaved_attention_stack",
    )(x, A_wqkv, A_wo, B_wqkv, B_wo)
    return out.reshape(1, S, D)
```
